```python
import jax
import jax.numpy as jnp

def _softmax(x, axis=-1):
    return jax.nn.softmax(x, axis=axis)

def _gelu(x):
    return jax.nn.gelu(x, approximate=True)

def _silu(x):
    return jax.nn.silu(x)

def _sigmoid(x):
    return jax.nn.sigmoid(x)

def _layernorm(x, axis=-1, eps=1e-05):
    m = jnp.mean(x, axis=axis, keepdims=True)
    v = jnp.var(x, axis=axis, keepdims=True)
    return (x - m) / jnp.sqrt(v + eps)

def _scatter_add(tgt, idx, src, axis=0):
    return tgt.at[idx].add(src)

def _segment_sum(src, seg, n):
    return jax.ops.segment_sum(src, seg, n)

class _Rng:

    def __init__(self, key):
        self._k = key

    def _next(self):
        self._k, sub = jax.random.split(self._k)
        return sub

    def normal(self, shape):
        return jax.random.normal(self._next(), shape, dtype=jnp.bfloat16)

    def randint(self, lo, hi, shape):
        return jax.random.randint(self._next(), shape, lo, hi, dtype=jnp.int32)

    def uniform(self, shape, lo=0.0, hi=1.0):
        return jax.random.uniform(self._next(), shape, jnp.bfloat16, lo, hi)

    def permutation(self, n):
        return jax.random.permutation(self._next(), n)
kernel_name = 'concat_heads__ssm_conv_h3__memory_aug_infini_attn__prompt'

def setup_inputs():
    _rng = _Rng(jax.random.key(int.from_bytes(__import__("os").urandom(4), "little")))
    _w = lambda a: (lambda t: t.astype(jnp.bfloat16) if jnp.issubdtype(t.dtype, jnp.floating) else t)(jnp.asarray(a))

    def _A_setup():
        B, S, D = (1, 2048, 640)
        ks = 4
        return {'q': _w((lambda *s: _rng.normal(s) * 0.05)(B, S, D)), 'k': _w((lambda *s: _rng.normal(s) * 0.05)(B, S, D)), 'v': _w((lambda *s: _rng.normal(s) * 0.05)(B, S, D)), 'shift_k': _w((lambda *s: _rng.normal(s) * 0.05)(D, ks) * 0.5), 'ssm_k': _w((lambda *s: _rng.normal(s) * 0.05)(D, S) * (1.0 / S ** 0.5)), 'ssm_D': _w((lambda *s: _rng.normal(s) * 0.05)(D))}
    _A_in = _A_setup()

    def _B_setup():
        B, S, D, H = (1, 2048, 640, 32)
        N = 4
        L = max(1, S // N)
        sc = D ** (-0.5)
        return {'x': _w((lambda *s: _rng.normal(s) * 0.05)(B, N * L, D)), 'wq': _w((lambda *s: _rng.normal(s) * 0.05)(D, D) * sc), 'wk': _w((lambda *s: _rng.normal(s) * 0.05)(D, D) * sc), 'wv': _w((lambda *s: _rng.normal(s) * 0.05)(D, D) * sc), 'wo': _w((lambda *s: _rng.normal(s) * 0.05)(D, D) * sc), 'beta': _w((lambda *s: _rng.normal(s) * 0.05)(H))}
    _B_in = _B_setup()
    return {'A_q': _A_in['q'], 'A_k': _A_in['k'], 'A_v': _A_in['v'], 'A_shift_k': _A_in['shift_k'], 'A_ssm_k': _A_in['ssm_k'], 'A_ssm_D': _A_in['ssm_D'], 'B_x': _B_in['x'], 'B_wq': _B_in['wq'], 'B_wk': _B_in['wk'], 'B_wv': _B_in['wv'], 'B_wo': _B_in['wo'], 'B_beta': _B_in['beta']}

def reference(A_q, A_k, A_v, A_shift_k, A_ssm_k, A_ssm_D, B_x, B_wq, B_wk, B_wv, B_wo, B_beta):

    def _A_ref(q, k, v, shift_k, ssm_k, ssm_D):
        B, S, D = q.shape
        ks = shift_k.shape[-1]
        k_pad = jnp.pad(k, ((0, 0), (ks - 1, 0), (0, 0)))
        k_shift = jnp.zeros_like(k)
        for t in range(ks):
            k_shift = k_shift + k_pad[:, t:t + S, :] * shift_k[:, ks - 1 - t][None, None, :]
        kv = k_shift * v
        L = 2 * S
        kv_pad = jnp.pad(kv, ((0, 0), (0, S), (0, 0)))
        kf_pad = jnp.pad(ssm_k, ((0, 0), (0, S)))
        kv_f = (lambda x, axes=(-2, -1): jnp.fft.rfft2(x.astype(jnp.float32), axes=axes))(kv_pad[:, None, :, :], axes=(1, 2))
        kf_f = (lambda x, axes=(-2, -1): jnp.fft.rfft2(x.astype(jnp.float32), axes=axes))(kf_pad[:, None, :], axes=(1, 2))
        kf_f = (lambda x, *d: x.transpose(*d))(kf_f, 1, 2, 0)
        y_f = kv_f * kf_f[None, :, :, :]
        y = (lambda x, s, axes=(-2, -1): jnp.fft.irfft2(x, s=s, axes=axes).astype(jnp.bfloat16))(y_f, (1, L), axes=(1, 2))[:, 0, :S, :]
        y = y + kv * ssm_D[None, None, :]
        return q * y

    def _B_ref(x, wq, wk, wv, wo, beta):
        B, S, D = x.shape
        H = 32
        Dh = D // H
        N = 4
        L = S // N
        q = (lambda x, *d: x.transpose(*d))((x @ wq).reshape(B, S, H, Dh), 0, 2, 1, 3).reshape(B, H, N, L, Dh)
        k = (lambda x, *d: x.transpose(*d))((x @ wk).reshape(B, S, H, Dh), 0, 2, 1, 3).reshape(B, H, N, L, Dh)
        v = (lambda x, *d: x.transpose(*d))((x @ wv).reshape(B, S, H, Dh), 0, 2, 1, 3).reshape(B, H, N, L, Dh)
        phi = lambda t: jnp.where(t > 0, t + 1.0, jnp.exp(t))
        scale = Dh ** (-0.5)
        ar = jnp.arange(L)
        mask = (lambda x, dt: x.astype(dt))(ar[:, None] < ar[None, :], x.dtype) * -1000000000.0
        g = _sigmoid(beta).reshape(1, H, 1, 1)
        M = jnp.einsum('bhd,bhe->bhde', q[:, :, 0, 0, :] * 0.0, q[:, :, 0, 0, :] * 0.0)
        z = q[:, :, 0, 0, :] * 0.0
        outs = []
        for s in range(N):
            qs, ks, vs = (q[:, :, s].copy(), k[:, :, s].copy(), v[:, :, s].copy())
            logits = jnp.einsum('bhqd,bhkd->bhqk', qs, ks) * scale + mask
            p = _softmax(logits, axis=-1)
            a_dot = jnp.einsum('bhqk,bhkd->bhqd', p, vs)
            pq = phi(qs)
            num = jnp.einsum('bhld,bhde->bhle', pq, M)
            den = jnp.einsum('bhld,bhd->bhl', pq, z)[..., None] + 1e-06
            a_mem = num / den
            o = g * a_mem + (1.0 - g) * a_dot
            outs.append(o)
            pk = phi(ks)
            M = M + jnp.einsum('bhld,bhle->bhde', pk, vs)
            z = z + jnp.einsum('bhld->bhd', pk)
        o = (lambda x, *d: x.transpose(*d))(jnp.stack(outs, 2).reshape(B, H, S, Dh), 0, 2, 1, 3).reshape(B, S, D)
        return o @ wo
    a = _A_ref(A_q, A_k, A_v, A_shift_k, A_ssm_k, A_ssm_D)
    b = _B_ref(B_x, B_wq, B_wk, B_wv, B_wo, B_beta)
    return jnp.concatenate([a, b], axis=-1)
```

```python
import math

import numpy as np
import jax
import jax.numpy as jnp
from jax import lax
from jax.experimental import pallas as pl
from jax.experimental.pallas import tpu as pltpu

S, D = 2048, 640
H, DH, NSEG, L = 32, 20, 4, 512
T = 128
NC = D // T
NB = S // T
UH = 4
UD = UH * DH
NU = H // UH
UR = L // NU
BF, F32 = jnp.bfloat16, jnp.float32
LOG2E = math.log2(math.e)


def _dft_matrix():
    m = np.arange(T, dtype=np.float64)[:, None]
    b = np.arange(T, dtype=np.float64)[None, :]
    ang = np.pi * np.mod((4 * m + 1) * b, 512) / 256
    f = np.stack([np.cos(ang).reshape(NB, 8, T), -np.sin(ang).reshape(NB, 8, T)], 1)
    return f.reshape(2 * T, T).astype(np.float32)


_F = _dft_matrix()
_FWD = _F.astype(BF)
_INV = np.stack([_F[:T].T / T, _F[T:].T / T]).astype(BF)


def _dot(a, b):
    return jnp.dot(a, b, preferred_element_type=F32)


def _dot_nt(a, b):
    return lax.dot_general(a, b, (((1,), (1,)), ((), ())), preferred_element_type=F32)


def _phi(t):
    return jnp.where(t > 0, t + 1.0, jnp.exp(t))


def _iota(shape, dim):
    return lax.broadcasted_iota(jnp.int32, shape, dim)


def _kernel(q_hbm, k_hbm, v_hbm, shift_ref, h_hbm, d_ref, x_hbm, wq_hbm, wk_hbm, wv_hbm,
            wo_hbm, beta_ref, fwd_ref, inv_ref, out_hbm,
            q_v, k_v, v_v, h_v, x_v, w_v, wo_v, wt_s, kf_s, kv_s, xf_s, gf_s, hp_s, y_s,
            outa_s, outb_s, ot_s, mem_s, gate_s, bias_s,
            sem_w, sem_x, sem_a, sem_q, sem_oa, sem_ob):

    def w_copy(i):
        return pltpu.make_async_copy((wq_hbm, wk_hbm, wv_hbm)[i], w_v.at[i], sem_w.at[i])

    def wo_copy(n):
        return pltpu.make_async_copy(wo_hbm.at[:, pl.ds(n * T, T)], wo_v.at[n], sem_w.at[3 + n])

    def x_copy(s, c):
        return pltpu.make_async_copy(x_hbm.at[pl.ds(s * L, L), pl.ds(c * T, T)],
                                     x_v.at[c, pl.ds(s * L, L)], sem_x.at[s * NC + c])

    def a_copies(u):
        r = pl.ds(pl.multiple_of(u * 2 * T, 2 * T), 2 * T)
        return (pltpu.make_async_copy(k_hbm.at[r], k_v.at[r], sem_a.at[3 * u]),
                pltpu.make_async_copy(v_hbm.at[r], v_v.at[r], sem_a.at[3 * u + 1]),
                pltpu.make_async_copy(h_hbm.at[:, r], h_v.at[u], sem_a.at[3 * u + 2]))

    def q_copy():
        return pltpu.make_async_copy(q_hbm, q_v, sem_q)

    def oa_copy(u):
        r = pl.ds(pl.multiple_of(u * 2 * T, 2 * T), 2 * T)
        c = pl.ds(0, (NC - 1) * T)
        return pltpu.make_async_copy(outa_s.at[r, c], out_hbm.at[r, c], sem_oa.at[u])

    def oa_last_copy(i):
        r = pl.ds(i * L, L)
        c = pl.ds((NC - 1) * T, T)
        return pltpu.make_async_copy(outa_s.at[r, c], out_hbm.at[r, c], sem_oa.at[NU + i])

    def ob_copy(i):
        r = pl.ds(pl.multiple_of(i * UR, UR), UR)
        return pltpu.make_async_copy(outb_s.at[r], out_hbm.at[r, pl.ds(D, D)], sem_ob.at[i])

    for i in range(3):
        w_copy(i).start()
    for c in range(NC):
        x_copy(0, c).start()
    for cp in a_copies(0):
        cp.start()

    def start_rest(u, _):
        for cp in a_copies(u):
            cp.start()
    lax.fori_loop(1, NU, start_rest, None)
    for s in range(1, NSEG):
        for c in range(NC):
            x_copy(s, c).start()
    for n in range(NC):
        wo_copy(n).start()
    q_copy().start()

    shift = shift_ref[...].astype(F32)
    dskip = d_ref[...].astype(F32).reshape(1, D)
    g = jax.nn.sigmoid(beta_ref[...].astype(F32).reshape(1, H))
    rr = _iota((D, H), 0)
    hh = _iota((D, H), 1) * DH
    gate = jnp.sum(jnp.where((rr >= hh) & (rr < hh + DH), g, 0.0), axis=1, keepdims=True)
    gate_s[...] = jnp.broadcast_to(gate, (D, T))
    bias_s[...] = jnp.where(_iota((T, T), 0) > _iota((T, T), 1), -1e9 * LOG2E, 0.0).astype(F32)
    mem_s[...] = jnp.zeros(mem_s.shape, F32)
    hp_s[...] = jnp.zeros(hp_s.shape, F32)
    for c in range(NC):
        kf_s[c, 0:8, :] = jnp.zeros((8, T), F32)

    for i in range(3):
        w_copy(i).wait()
        for c in range(NC):
            for t in range(NC):
                wt = w_v[i, c * T:(c + 1) * T, t * T:(t + 1) * T].T
                for r in range(T // 16):
                    grp = t * (T // 16) + r
                    row = (grp // 5) * 3 * UD + i * UD + (grp % 5) * 16
                    wt_s[c, row:row + 16, :] = wt[r * 16:(r + 1) * 16, :]

    def conv_forward(u, j, c):
        a = 2 * u + j
        r0 = pl.multiple_of(a * T, T)
        lanes = slice(c * T, (c + 1) * T)
        kf = k_v[pl.ds(r0, T), lanes].astype(F32)
        kf_s[c, pl.ds(pl.multiple_of(r0 + 8, 8), T), :] = kf
        ks = kf * shift[0:1, lanes]
        for t in range(1, 4):
            ks = ks + kf_s[c, pl.ds(r0 + 8 - t, T), :] * shift[t:t + 1, lanes]
        kv = (ks * v_v[pl.ds(r0, T), lanes].astype(F32)).astype(BF)
        kv_s[c, pl.ds(r0, T), :] = kv
        xf_s[c, a] = _dot(fwd_ref[...], kv)
        hf = _dot_nt(fwd_ref[...], h_v[u, lanes, j * T:(j + 1) * T])
        hp = hp_s[c]
        hp_s[c] = hf
        parts = []
        for f in range(NB):
            re, im = slice(16 * f, 16 * f + 8), slice(16 * f + 8, 16 * f + 16)
            parts += [hf[re] - hp[im], hf[im] + hp[re]]
        gf_s[c, a] = jnp.concatenate(parts, axis=0)

    def conv_mac(c, f):
        r0 = pl.multiple_of(f * 16, 16)
        re, im = pl.ds(r0, 8), pl.ds(pl.multiple_of(r0 + 8, 8), 8)
        for a in range(NB):
            yr = yi = None
            for b in range(a + 1):
                xr, xi = xf_s[c, b, re, :], xf_s[c, b, im, :]
                gr, gi = gf_s[c, a - b, re, :], gf_s[c, a - b, im, :]
                pr, pi = xr * gr - xi * gi, xr * gi + xi * gr
                yr, yi = (pr, pi) if yr is None else (yr + pr, yi + pi)
            y_s[c, a, pl.ds(r0, 16), :] = jnp.concatenate([yr, yi], axis=0).astype(BF)

    def conv_inverse(c, a):
        r0 = pl.multiple_of(a * T, T)
        lanes = slice(c * T, (c + 1) * T)
        y = _dot(inv_ref[0], y_s[c, a, 0:T, :]) + _dot(inv_ref[1], y_s[c, a, T:2 * T, :])
        y = y + kv_s[c, pl.ds(r0, T), :].astype(F32) * dskip[:, lanes]
        outa_s[pl.ds(r0, T), lanes] = (q_v[pl.ds(r0, T), lanes].astype(F32) * y).astype(BF)

    def out_proj(s, u):
        o = jnp.concatenate(
            [ot_s[s % 2, u, c * T:(c + 1) * T, :].T for c in range(NC)], axis=1)
        wo = jnp.concatenate([wo_v[n] for n in range(NC)], axis=1)
        outb_s[pl.ds(pl.multiple_of(s * L + u * UR, UR), UR), :] = _dot(o, wo).astype(BF)

    def unit(s, u, fillers):
        fillers = list(fillers)

        def fill(n=1):
            for _ in range(n):
                if fillers:
                    fillers.pop(0)()

        w0 = pl.multiple_of(u * 3 * UD, 16)
        w = jnp.concatenate([wt_s[c, pl.ds(w0, 3 * UD), :] for c in range(NC)], axis=1)
        x = jnp.concatenate([x_v[c, s * L:(s + 1) * L, :] for c in range(NC)], axis=1)
        qkv = _dot_nt(w, x)
        qt, kt, vt = qkv[0:UD], qkv[UD:2 * UD], qkv[2 * UD:3 * UD]
        fill(2)
        pad = jnp.zeros((T - UD, L), F32)
        kn = jnp.concatenate([kt, pad], axis=0).T.astype(BF)
        qs = qt * (DH ** -0.5 * LOG2E)

        if s < NSEG - 1:
            pk = jnp.concatenate([_phi(kt), pad], axis=0).astype(BF)
            va = jnp.concatenate([vt, jnp.ones((16, L), F32)], axis=0).astype(BF)
            upd = _dot_nt(va, pk)
        if s > 0:
            mem = mem_s[u]
            lane = _iota((UD, T), 1)
            row = _iota((UD, T), 0)
            same = functools_reduce_or(
                [(row >= DH * i) & (row < DH * (i + 1)) & (lane >= DH * i) & (lane < DH * (i + 1))
                 for i in range(UH)])
            lane8 = _iota((8, T), 1)
            lhs = [jnp.where(same, mem[0:UD], 0.0)]
            for i in range(UH):
                lhs.append(jnp.where((lane8 >= DH * i) & (lane8 < DH * (i + 1)), mem[UD:UD + 8], 0.0))
            pq = jnp.concatenate([_phi(qt), pad], axis=0).astype(BF)
            ret = _dot(jnp.concatenate(lhs, axis=0).astype(BF), pq)
        if s < NSEG - 1:
            mem_s[u] = upd if s == 0 else mem + upd

        row32 = _iota((32, L), 0)
        low4 = _iota((8, T), 0) < 4
        heads = []
        for i in range(UH):
            mine = (row32 >= 4 * i) & (row32 < 4 * i + DH)
            win = slice(16 * i, 16 * i + 32)
            rq = jnp.where(mine, qs[win], 0.0).astype(BF)
            blocks = [rq]
            if i > 0:
                blocks.insert(0, jnp.zeros((16 * i, L), BF))
            blocks.append(jnp.zeros((T - 32 - 16 * i, L), BF))
            rq = jnp.concatenate(blocks, axis=0)
            va = jnp.where(mine, vt[win], 1.0).astype(BF)
            den_rows = slice(24, 32) if i < 2 else slice(0, 8)
            val_rows = slice(0, 24) if i < 2 else slice(8, 32)
            cols = []
            for j in range(L // T):
                n = (j + 1) * T
                sc = _dot(kn[0:n], rq[:, j * T:(j + 1) * T])
                diag = sc[n - T:n] + bias_s[...]
                sc = diag if j == 0 else jnp.concatenate([sc[0:n - T], diag], axis=0)
                p = jnp.exp2(sc - jnp.max(sc, axis=0, keepdims=True)).astype(BF)
                acc = _dot(va[:, 0:n], p)
                inv = 1.0 / acc[den_rows]
                cols.append(acc[val_rows] * jnp.concatenate([inv] * 3, axis=0))
            heads.append(jnp.concatenate(cols, axis=1))
            fill(2)
        low4 = _iota((8, L), 0) < 4
        att = jnp.concatenate([
            heads[0][0:16], jnp.where(low4, heads[0][16:24], heads[1][0:8]), heads[1][8:24],
            heads[2][0:16], jnp.where(low4, heads[2][16:24], heads[3][0:8]), heads[3][8:24]], axis=0)
        gt = gate_s[pl.ds(pl.multiple_of(u * UD, 8), UD), :]
        gt = jnp.concatenate([gt] * (L // T), axis=1)
        o = (1.0 - gt) * att
        if s > 0:
            rd = [1.0 / (ret[UD + 8 * i:UD + 8 * i + 8] + 1e-6) for i in range(UH)]
            rden = jnp.concatenate([
                rd[0], rd[0], jnp.where(low4, rd[0], rd[1]), rd[1], rd[1],
                rd[2], rd[2], jnp.where(low4, rd[2], rd[3]), rd[3], rd[3]], axis=0)
            o = o + gt * (ret[0:UD] * rden)
        o = o.astype(BF)
        for r in range(NU):
            ot_s[s % 2, r, pl.ds(pl.multiple_of(u * UD, 16), UD), :] = o[:, r * UR:(r + 1) * UR]
        fill(len(fillers))

    for c in range(NC):
        x_copy(0, c).wait()

    def seg0(u, _):
        for cp in a_copies(u):
            cp.wait()
        unit(0, u, [lambda j=j, c=c: conv_forward(u, j, c) for j in range(2) for c in range(NC)])
    lax.fori_loop(0, NU, seg0, None)

    for n in range(NC):
        wo_copy(n).wait()

    for s in (1, 2):
        for c in range(NC):
            x_copy(s, c).wait()

        def seg(u, _, s=s):
            fl = [lambda c=c, j=j: conv_mac(2 * (s - 1) + c, 2 * u + j)
                  for c in range(2) for j in range(2)]
            fl.insert(0, lambda: out_proj(s - 1, u))
            unit(s, u, fl)
            ob_copy((s - 1) * NU + u).start()
        lax.fori_loop(0, NU, seg, None)

    for c in range(NC):
        x_copy(3, c).wait()
    q_copy().wait()

    def seg3(u, _):
        fl = [lambda: out_proj(2, u)]
        fl += [lambda j=j: conv_mac(NC - 1, 2 * u + j) for j in range(2)]
        fl += [lambda j=j, c=c: conv_inverse(c, 2 * u + j) for j in range(2) for c in range(NC - 1)]
        unit(3, u, fl)
        ob_copy(2 * NU + u).start()
        oa_copy(u).start()
    lax.fori_loop(0, NU, seg3, None)

    def tail(u, _):
        out_proj(3, u)
        for j in range(2):
            conv_inverse(NC - 1, 2 * u + j)
        ob_copy(3 * NU + u).start()

        @pl.when(u % 2 == 1)
        def _():
            r = pl.ds(pl.multiple_of((u // 2) * L, L), L)
            c = pl.ds((NC - 1) * T, T)
            pltpu.make_async_copy(outa_s.at[r, c], out_hbm.at[r, c], sem_oa.at[NU + u // 2]).start()
    lax.fori_loop(0, NU, tail, None)

    def wait_b(i, _):
        ob_copy(i).wait()
    lax.fori_loop(0, NSEG * NU, wait_b, None)

    def wait_a(u, _):
        oa_copy(u).wait()
    lax.fori_loop(0, NU, wait_a, None)
    for i in range(NSEG):
        oa_last_copy(i).wait()


def functools_reduce_or(xs):
    r = xs[0]
    for x in xs[1:]:
        r = r | x
    return r


@jax.jit
def pallas_concat_heads__ssm_conv_h3__memory_aug_infini_attn__prompt_kernel(
    A_q, A_k, A_v, A_shift_k, A_ssm_k, A_ssm_D, B_x, B_wq, B_wk, B_wv, B_wo, B_beta,
):
    hbm = pl.BlockSpec(memory_space=pl.ANY)
    vmem = pl.BlockSpec(memory_space=pltpu.VMEM)
    dma = pltpu.SemaphoreType.DMA
    out = pl.pallas_call(
        _kernel,
        out_shape=jax.ShapeDtypeStruct((S, 2 * D), BF),
        in_specs=[hbm, hbm, hbm, vmem, hbm, vmem, hbm, hbm, hbm, hbm, hbm, vmem, vmem, vmem],
        out_specs=hbm,
        scratch_shapes=[
            pltpu.VMEM((S, D), BF),
            pltpu.VMEM((S, D), BF),
            pltpu.VMEM((S, D), BF),
            pltpu.VMEM((NU, D, 2 * T), BF),
            pltpu.VMEM((NC, S, T), BF),
            pltpu.VMEM((3, D, D), BF),
            pltpu.VMEM((NC, D, T), BF),
            pltpu.VMEM((NC, 3 * D, T), BF),
            pltpu.VMEM((NC, S + 8, T), F32),
            pltpu.VMEM((NC, S, T), BF),
            pltpu.VMEM((NC, NB, 2 * T, T), F32),
            pltpu.VMEM((NC, NB, 2 * T, T), F32),
            pltpu.VMEM((NC, 2 * T, T), F32),
            pltpu.VMEM((NC, NB, 2 * T, T), BF),
            pltpu.VMEM((S, D), BF),
            pltpu.VMEM((S, D), BF),
            pltpu.VMEM((2, NU, D, UR), BF),
            pltpu.VMEM((NU, UD + 16, T), F32),
            pltpu.VMEM((D, T), F32),
            pltpu.VMEM((T, T), F32),
            dma((3 + NC,)), dma((NSEG * NC,)), dma((3 * NU,)), dma(()),
            dma((NU + NSEG,)), dma((NSEG * NU,)),
        ],
        compiler_params=pltpu.CompilerParams(vmem_limit_bytes=100 * 1024 * 1024),
        name="h3_infini",
    )(A_q.reshape(S, D), A_k.reshape(S, D), A_v.reshape(S, D), A_shift_k.T, A_ssm_k, A_ssm_D,
      B_x.reshape(S, D), B_wq, B_wk, B_wv, B_wo, B_beta, _FWD, _INV)
    return out.reshape(1, S, 2 * D)
```

```python
import math, os

import numpy as np
import jax
import jax.numpy as jnp
from jax import lax
from jax.experimental import pallas as pl
from jax.experimental.pallas import tpu as pltpu

OPT = os.environ.get('OPT', '')
ONLY = os.environ.get('ONLY', '')
ENV = os.environ.get

S, D = 2048, 640
H, DH, NSEG, L = 32, 20, 4, 512
T = 128
NC = D // T
NB = S // T
NQ = L // T
UH = 4
UD = UH * DH
NU = H // UH
UR = L // NU
BF, F32 = jnp.bfloat16, jnp.float32
LOG2E = math.log2(math.e)


def _dft_matrix():
    m = np.arange(T, dtype=np.float64)[:, None]
    b = np.arange(T, dtype=np.float64)[None, :]
    ang = np.pi * np.mod((4 * m + 1) * b, 512) / 256
    f = np.stack([np.cos(ang).reshape(NB, 8, T), -np.sin(ang).reshape(NB, 8, T)], 1)
    return f.reshape(2 * T, T).astype(np.float32)


_F = _dft_matrix()
_DFT = np.stack([_F[:T], _F[T:], _F[:T].T / T, _F[T:].T / T]).astype(BF)


def _dot(a, b):
    return jnp.dot(a, b, preferred_element_type=F32)


def _dot_nt(a, b):
    return lax.dot_general(a, b, (((1,), (1,)), ((), ())), preferred_element_type=F32)


def _phi(t):
    return jnp.where(t > 0, t + 1.0, jnp.exp(t))


def _iota(shape, dim):
    return lax.broadcasted_iota(jnp.int32, shape, dim)


def _head_of(z):
    return sum((z >= DH * i).astype(jnp.int32) for i in range(1, UH))


def _kernel(q_hbm, k_hbm, v_hbm, shift_ref, h_hbm, d_ref, x_hbm, wq_hbm, wk_hbm, wv_hbm,
            wo_hbm, beta_ref, dft_ref, out_hbm,
            q_v, k_v, v_v, h_v, x_v, w_v, wo_v, wt_s, dft_s, kf_s, kv_s, xg_s, hp_s, y_s,
            outa_s, outb_s, ot0_s, ot1_s, mem_s, meml_s, gate_s, bias_s,
            kn_s, rq_s, pk_s, pq_s, vt_s, va_s, s_s, p_s, m_s, ret_s, zero_s,
            sem_w, sem_x, sem_a, sem_q, sem_oa, sem_ob):
    ot_s = (ot0_s, ot1_s)

    def w_copy(i, t):
        cols = pl.ds(t * T, T)
        return pltpu.make_async_copy((wq_hbm, wk_hbm, wv_hbm)[i].at[:, cols], w_v.at[i, t],
                                     sem_w.at[i * NC + t])

    def wo_copy(n):
        return pltpu.make_async_copy(wo_hbm.at[:, pl.ds(n * T, T)], wo_v.at[n],
                                     sem_w.at[3 * NC + n])

    def x_copy(s, c):
        return pltpu.make_async_copy(x_hbm.at[pl.ds(s * L, L), pl.ds(c * T, T)],
                                     x_v.at[c, pl.ds(s * L, L)], sem_x.at[s * NC + c])

    def a_copies(u):
        r = pl.ds(pl.multiple_of(u * 2 * T, 2 * T), 2 * T)
        return (pltpu.make_async_copy(k_hbm.at[r], k_v.at[r], sem_a.at[3 * u]),
                pltpu.make_async_copy(v_hbm.at[r], v_v.at[r], sem_a.at[3 * u + 1]),
                pltpu.make_async_copy(h_hbm.at[:, r], h_v.at[u], sem_a.at[3 * u + 2]))

    def q_copy():
        return pltpu.make_async_copy(q_hbm, q_v, sem_q)

    def oa_copy(u):
        r = pl.ds(pl.multiple_of(u * 2 * T, 2 * T), 2 * T)
        c = pl.ds(0, (NC - 1) * T)
        return pltpu.make_async_copy(outa_s.at[r, c], out_hbm.at[r, c], sem_oa.at[u])

    def oa_last_copy(i):
        r = pl.ds(i * L, L)
        c = pl.ds((NC - 1) * T, T)
        return pltpu.make_async_copy(outa_s.at[r, c], out_hbm.at[r, c], sem_oa.at[NU + i])

    def ob_copy(i):
        r = pl.ds(pl.multiple_of(i * UR, UR), UR)
        return pltpu.make_async_copy(outb_s.at[r], out_hbm.at[r, pl.ds(D, D)], sem_ob.at[i])

    def ob_last_copy(j):
        r = pl.ds((NSEG - 1) * L + j * T, T)
        return pltpu.make_async_copy(outb_s.at[r], out_hbm.at[r, pl.ds(D, D)],
                                     sem_ob.at[(NSEG - 1) * NU + j])

    def conv_forward(u, c):
        r0 = pl.multiple_of(u * 2 * T, 2 * T)
        lanes = slice(c * T, (c + 1) * T)
        kf = k_v[pl.ds(r0, 2 * T), lanes].astype(F32)
        kf_s[c, 8:8 + 2 * T, :] = kf
        ks = kf * shift_ref[0:1, lanes].astype(F32)
        for t in range(1, 4):
            ks = ks + kf_s[c, 8 - t:8 - t + 2 * T, :] * shift_ref[t:t + 1, lanes].astype(F32)
        kf_s[c, 0:8, :] = kf[2 * T - 8:2 * T]
        kv = (ks * v_v[pl.ds(r0, 2 * T), lanes].astype(F32)).astype(BF)
        kv_s[c, pl.ds(r0, 2 * T), :] = kv
        fwd = jnp.concatenate([dft_s[0], dft_s[1]], axis=0)
        hf = [_dot_nt(fwd, h_v[u, lanes, j * T:(j + 1) * T]) for j in range(2)]
        for j in range(2):
            xg_s[c, 2 * u + j] = _dot(fwd, kv[j * T:(j + 1) * T])
        prev = [hp_s[c], hf[0]]
        hp_s[c] = hf[1]
        for j in range(2):
            parts = []
            for f in range(NB):
                re, im = slice(16 * f, 16 * f + 8), slice(16 * f + 8, 16 * f + 16)
                parts += [hf[j][re] - prev[j][im], hf[j][im] + prev[j][re]]
            xg_s[NC + c, 2 * u + j] = jnp.concatenate(parts, axis=0)

    def conv_mac(items, w=2):
        for c, f in items:
            for k in range(NB // w):
                outs = range(k * w, (k + 1) * w)
                r0 = pl.multiple_of((f + zero_s[k]) * 16, 16)
                re, im = pl.ds(r0, 8), pl.ds(pl.multiple_of(r0 + 8, 8), 8)
                acc, g = {}, {}
                for b in range(max(outs) + 1):
                    xr, xi = xg_s[c, b, re, :], xg_s[c, b, im, :]
                    cost = 0
                    for a in outs:
                        if b > a:
                            continue
                        if a - b not in g:
                            g[a - b] = (xg_s[NC + c, a - b, re, :], xg_s[NC + c, a - b, im, :])
                        gr, gi = g[a - b]
                        p = (xr * gr - xi * gi, xr * gi + xi * gr)
                        acc[a] = p if a not in acc else (acc[a][0] + p[0], acc[a][1] + p[1])
                        cost += 1
                        if a == b:
                            y_s[c, a, pl.ds(r0, 16), :] = jnp.concatenate(acc[a], axis=0).astype(BF)
                    yield cost

    class Filler:
        def __init__(self):
            self.gen, self.credit = None, 0.0

        def pin(self, value, amount):
            if self.gen is None or amount == 0:
                return
            xg_s[0, NB, 0:8, :] = value
            self.credit += amount
            while self.gen is not None and self.credit > 0:
                cost = next(self.gen, None)
                if cost is None:
                    self.gen = None
                else:
                    self.credit -= cost

        def drain(self):
            if self.gen is not None:
                for _ in self.gen:
                    pass
            self.gen = None

    filler = Filler()

    def conv_inverse(u, c):
        r0 = pl.multiple_of(u * 2 * T, 2 * T)
        lanes = slice(c * T, (c + 1) * T)
        for j in range(2):
            a = 2 * u + j
            rows = pl.ds(pl.multiple_of(r0 + j * T, T), T)
            y = _dot(dft_s[2], y_s[c, a, 0:T, :]) + _dot(dft_s[3], y_s[c, a, T:2 * T, :])
            y = y + kv_s[c, rows, :].astype(F32) * d_row[:, lanes]
            outa_s[rows, lanes] = (q_v[rows, lanes].astype(F32) * y).astype(BF)

    def out_proj(s, u):
        o = jnp.concatenate(
            [ot_s[s % 2][u, c * T:(c + 1) * T, :].T for c in range(NC)], axis=1)
        wo = jnp.concatenate([wo_v[n] for n in range(NC)], axis=1)
        outb_s[pl.ds(pl.multiple_of(s * L + u * UR, UR), UR), :] = _dot(o, wo).astype(BF)

    def project(n, amount):
        s, u = n // NU, n % NU
        w0 = pl.multiple_of(u * 3 * UD, 16)
        x0 = pl.multiple_of(s * L, L)
        qkv = None
        for c in range(NC):
            part = _dot_nt(wt_s[c, pl.ds(w0, 3 * UD), :], x_v[c, pl.ds(x0, L), :])
            for r in range(0, 3 * UD, 24):
                filler.pin(part[r:r + 8, 0:T], amount[c] / 10)
            qkv = part if qkv is None else qkv + part
            yield c
        slot = n % 3
        row32 = _iota((32, T), 0)
        pad = jnp.zeros((T - UD, T), F32)
        for j in range(NQ):
            cols = slice(j * T, (j + 1) * T)
            qt, kt, vt = qkv[0:UD, cols], qkv[UD:2 * UD, cols], qkv[2 * UD:3 * UD, cols]
            kn_s[cols, :] = jnp.concatenate([kt, pad], axis=0).T.astype(BF)
            pk_s[slot, j] = _phi(kt).astype(BF)
            pq_s[slot, j] = _phi(qt).astype(BF)
            vt_s[slot, j] = vt.astype(BF)
            qs = qt * (DH ** -0.5 * LOG2E)
            for i in range(UH):
                mine = (row32 >= 4 * i) & (row32 < 4 * i + DH)
                win = slice(16 * i, 16 * i + 32)
                rq_s[j, i, win, :] = jnp.where(mine, qs[win], 0.0).astype(BF)
                va_s[slot, i, j] = jnp.where(mine, vt[win], 1.0).astype(BF)

    def s_off(j, i, t):
        return pl.ds((2 * j * (j + 1) + i * (j + 1) + t) * T, T)

    def scores(j, t, top, amount):
        rq = jnp.concatenate([rq_s[j, i] for i in range(UH)], axis=1)
        sc = _dot(kn_s[t * T:(t + 1) * T, :], rq)
        for i in range(UH):
            si = sc[:, i * T:(i + 1) * T]
            if t == j:
                si = si + bias_s[...]
            s_s[s_off(j, i, t), :] = si
            if i == 0:
                for r in range(0, T, 32):
                    filler.pin(si[r:r + 8], amount / 4)
            m = jnp.max(si.reshape(T // 8, 8, T), axis=0)
            top[i] = m if t == 0 else jnp.maximum(top[i], m)
            if t == j:
                m_s[j, i] = jnp.broadcast_to(jnp.max(top[i], axis=0, keepdims=True), (8, T))

    def softmax(j, t):
        for i in range(UH):
            m = jnp.concatenate([m_s[j, i]] * (T // 8), axis=0)
            p_s[s_off(j, i, t), :] = jnp.exp2(s_s[s_off(j, i, t), :] - m).astype(BF)

    def spread(a, b):
        low4 = _iota(a.shape, 0) < 4
        ar, br = pltpu.roll(a, 4, 0), pltpu.roll(b, 4, 0)
        r0, r1 = jnp.where(low4, a, ar), jnp.where(low4, ar, a)
        r2, r3 = jnp.where(low4, b, br), jnp.where(low4, br, b)
        return jnp.concatenate([r0, r0, a, r1, r1, r2, r2, b, r3, r3], axis=0)

    def retrieve(n):
        u, slot = n % NU, n % 3
        zpad = jnp.zeros((T - UD, T), BF)
        pq = jnp.concatenate(
            [jnp.concatenate([pq_s[slot, j], zpad], axis=0) for j in range(NQ)], axis=1)
        ret = _dot(meml_s[u], pq)
        rd = 1.0 / (ret[UD:UD + 16] + 1e-6)
        ret_s[...] = ret[0:UD] * spread(rd[0:8], rd[8:16])

    def update(n, s):
        u, slot = n % NU, n % 3
        zpad = jnp.zeros((T - UD, T), BF)
        va = jnp.concatenate(
            [jnp.concatenate([vt_s[slot, j], jnp.ones((16, T), BF)], axis=0) for j in range(NQ)],
            axis=1)
        pk = jnp.concatenate(
            [jnp.concatenate([pk_s[slot, j], zpad], axis=0) for j in range(NQ)], axis=1)
        mem = _dot_nt(va, pk)
        if s > 0:
            mem = mem_s[u] + mem
        if s < NSEG - 2:
            mem_s[u] = mem
        row = _iota((UD + 16, T), 0)
        row_head = jnp.where(row < UD, _head_of(row), (row - UD) >> 2)
        meml_s[u] = jnp.where(row_head == _head_of(_iota((UD + 16, T), 1)), mem, 0.0).astype(BF)

    def values(n, s, j, t, acc):
        u, slot = n % NU, n % 3
        for i in range(UH):
            part = _dot(va_s[slot, i, t], p_s[s_off(j, i, t), :])
            acc[i] = part if t == 0 else acc[i] + part
        if t < j:
            return
        heads = []
        for i in range(UH):
            den = acc[i][24:32] if i < 2 else acc[i][0:8]
            val = acc[i][0:24] if i < 2 else acc[i][8:32]
            heads.append(val * jnp.concatenate([1.0 / den] * 3, axis=0))
        low4 = _iota((8, T), 0) < 4
        att = jnp.concatenate([
            heads[0][0:16], jnp.where(low4, heads[0][16:24], heads[1][0:8]), heads[1][8:24],
            heads[2][0:16], jnp.where(low4, heads[2][16:24], heads[3][0:8]), heads[3][8:24]], axis=0)
        rows = pl.ds(pl.multiple_of(u * UD, 16), UD)
        gt = gate_s[rows, :]
        o = (1.0 - gt) * att
        if s > 0:
            o = o + gt * ret_s[:, j * T:(j + 1) * T]
        o = o.astype(BF)
        ot_s[s % 2][2 * j, rows, :] = o[:, 0:UR]
        ot_s[s % 2][2 * j + 1, rows, :] = o[:, UR:T]

    ORDER = ENV('ORDER', 'R Q30 Q31 V30 Q32 V31 Q33 V32 Q20 V33 Q21 V20 Q22 V21 Q10 V22 Q11 V10 Q00 V11 '
                         'P X V00 P X P X P X P U X X O X X X').split()
    PQK, PPR = float(ENV('PQK', '0.27')), float(ENV('PPR', '0.73'))

    def step(n, s, jobs=(), out=None, mac=(), do_proj=True, do_scores=True, do_values=True):
        jobs = list(jobs)
        total = 136 * len(mac)
        filler.gen, filler.credit = (conv_mac(mac) if mac else None), 0.0
        proj = project(n + 2, [total * PPR / NC] * NC)
        top, acc, nproj = [None] * UH, [None] * UH, 0
        for tok in ORDER:
            if tok[0] == 'Q':
                j, t = int(tok[1]), int(tok[2])
                if do_values:
                    softmax(j, t)
                if do_scores:
                    scores(j, t, top, total * PQK / 10)
            elif tok[0] == 'V':
                if do_values:
                    values(n, s, int(tok[1]), int(tok[2]), acc)
            elif tok == 'P':
                if do_proj:
                    next(proj)
                    nproj += 1
                    if nproj == NC:
                        next(proj, None)
            elif tok == 'R':
                if do_values and s > 0:
                    retrieve(n)
            elif tok == 'U':
                if do_values and s < NSEG - 1:
                    update(n, s)
            elif tok == 'O':
                if out is not None:
                    out()
            elif tok == 'X':
                if jobs:
                    jobs.pop(0)()
        assert not jobs
        filler.drain()

    def seg_step(s, u, **kw):
        if s == 0:
            step(u, 0, jobs=[lambda c=c: conv_forward(u, c) for c in range(NC)])
        elif s < NSEG - 1:
            step(s * NU + u, s, out=lambda: out_proj(s - 1, u),
                 mac=[(2 * (s - 1) + c, 2 * u + j) for c in range(2) for j in range(2)])
        else:
            step(s * NU + u, s, out=lambda: out_proj(s - 1, u),
                 jobs=[lambda c=c: conv_inverse(u, c) for c in range(NC - 1)],
                 mac=[(NC - 1, 2 * u + j) for j in range(2)], **kw)

    def transpose_weights(t):
        for i in range(3):
            for c in range(NC):
                wt = w_v[i, t, c * T:(c + 1) * T, :].T
                for r in range(T // 16):
                    grp = t * (T // 16) + r
                    row = (grp // 5) * 3 * UD + i * UD + (grp % 5) * 16
                    wt_s[c, row:row + 16, :] = wt[r * 16:(r + 1) * 16, :]

    d_row = d_ref[...].astype(F32).reshape(1, D)

    if ONLY:
        lax.fori_loop(0, NU, lambda u, _: seg_step(int(ONLY), u), None)

        def fin(i, _):
            z = (y_s[i, i, 0:16, :].astype(F32) + ot0_s[i, 0:16, 0:1] + ot1_s[i, 0:16, 0:1] + mem_s[i, 0:16, :]
                 + xg_s[i, i, 0:16, :] + meml_s[i, 0:16, :] + kv_s[i, 0:16, :] + p_s[pl.ds(i * 16, 16), :] + s_s[pl.ds(i * 16, 16), :])
            outa_s[0:16, 0:T] = z.astype(BF)
            cp = pltpu.make_async_copy(outa_s, out_hbm.at[:, pl.ds(0, D)], sem_q); cp.start(); cp.wait()
            cp = pltpu.make_async_copy(outb_s, out_hbm.at[:, pl.ds(D, D)], sem_q); cp.start(); cp.wait()
        lax.fori_loop(0, 4, fin, None)
        return

    for i in range(3):
        w_copy(i, 0).start()
    for c in range(NC):
        x_copy(0, c).start()
    for t in range(1, NC):
        for i in range(3):
            w_copy(i, t).start()

    g = jax.nn.sigmoid(beta_ref[...].astype(F32).reshape(1, H))
    rr = _iota((D, H), 0)
    hh = _iota((D, H), 1) * DH
    gate = jnp.sum(jnp.where((rr >= hh) & (rr < hh + DH), g, 0.0), axis=1, keepdims=True)
    gate_s[...] = jnp.broadcast_to(gate, (D, T))
    bias_s[...] = jnp.where(_iota((T, T), 0) > _iota((T, T), 1), -1e9 * LOG2E, 0.0).astype(F32)
    hp_s[...] = jnp.zeros(hp_s.shape, F32)
    rq_s[...] = jnp.zeros(rq_s.shape, BF)
    dft_s[...] = dft_ref[...]
    for c in range(NC):
        kf_s[c, 0:8, :] = jnp.zeros((8, T), F32)
    for k in range(NB):
        zero_s[k] = 0

    for i in range(3):
        w_copy(i, 0).wait()
    transpose_weights(0)
    for c in range(NC):
        x_copy(0, c).wait()

    for cp in a_copies(0):
        cp.start()

    def start_rest(u, _):
        for cp in a_copies(u):
            cp.start()
    lax.fori_loop(1, NU, start_rest, None)
    for s in range(1, NSEG):
        for c in range(NC):
            x_copy(s, c).start()
    for n in range(NC):
        wo_copy(n).start()
    q_copy().start()

    with jax.named_scope("pro"):
        for t in range(1, NC):
            for i in range(3):
                w_copy(i, t).wait()
        transpose_weights(1)
        for _ in project(0, [0] * NC):
            pass
        step(-1, 0, do_values=False)
        for t in range(2, NC):
            transpose_weights(t)
    for c in range(NC):
        x_copy(1, c).wait()

    def seg0(u, _):
        for cp in a_copies(u):
            cp.wait()
        seg_step(0, u)
    with jax.named_scope("seg0"):
        lax.fori_loop(0, NU, seg0, None)

    for n in range(NC):
        wo_copy(n).wait()

    for s in (1, 2):
        for c in range(NC):
            x_copy(s + 1, c).wait()

        def seg(u, _, s=s):
            seg_step(s, u)
            ob_copy((s - 1) * NU + u).start()
        with jax.named_scope(f"seg{s}"):
            lax.fori_loop(0, NU, seg, None)

    q_copy().wait()

    def seg3(u, _, **kw):
        seg_step(3, u, **kw)
        ob_copy(2 * NU + u).start()
        oa_copy(u).start()
    with jax.named_scope("seg3"):
        lax.fori_loop(0, NU - 2, seg3, None)
    with jax.named_scope("seg3e"):
        seg3(NU - 2, None, do_proj=False)
        seg3(NU - 1, None, do_proj=False, do_scores=False)

    with jax.named_scope("tail"):
        wo = jnp.concatenate([wo_v[n] for n in range(NC)], axis=1)
        for j in range(NQ):
            conv_inverse(2 * j, NC - 1)
            conv_inverse(2 * j + 1, NC - 1)
            oa_last_copy(j).start()
        for j in range(NQ):
            o = jnp.concatenate(
                [jnp.concatenate([ot1_s[2 * j + r, c * T:(c + 1) * T, :].T for r in range(2)], axis=0)
                 for c in range(NC)], axis=1)
            r0 = (NSEG - 1) * L + j * T
            outb_s[r0:r0 + T, :] = _dot(o, wo).astype(BF)
            ob_last_copy(j).start()

    def wait_b(i, _):
        ob_copy(i).wait()
    lax.fori_loop(0, (NSEG - 1) * NU, wait_b, None)

    def wait_a(u, _):
        oa_copy(u).wait()
    lax.fori_loop(0, NU, wait_a, None)
    for i in range(NQ):
        oa_last_copy(i).wait()
        ob_last_copy(i).wait()


@jax.jit
def pallas_concat_heads__ssm_conv_h3__memory_aug_infini_attn__prompt_kernel(
    A_q, A_k, A_v, A_shift_k, A_ssm_k, A_ssm_D, B_x, B_wq, B_wk, B_wv, B_wo, B_beta,
):
    hbm = pl.BlockSpec(memory_space=pl.ANY)
    vmem = pl.BlockSpec(memory_space=pltpu.VMEM)
    dma = pltpu.SemaphoreType.DMA
    out = pl.pallas_call(
        _kernel,
        out_shape=jax.ShapeDtypeStruct((S, 2 * D), BF),
        in_specs=[hbm, hbm, hbm, vmem, hbm, vmem, hbm, hbm, hbm, hbm, hbm, vmem, vmem],
        out_specs=hbm,
        scratch_shapes=[
            pltpu.VMEM((S, D), BF),
            pltpu.VMEM((S, D), BF),
            pltpu.VMEM((S, D), BF),
            pltpu.VMEM((NU, D, 2 * T), BF),
            pltpu.VMEM((NC, S, T), BF),
            pltpu.VMEM((3, NC, D, T), BF),
            pltpu.VMEM((NC, D, T), BF),
            pltpu.VMEM((NC, 3 * D, T), BF),
            pltpu.VMEM((4, T, T), BF),
            pltpu.VMEM((NC, 2 * T + 8, T), F32),
            pltpu.VMEM((NC, S, T), BF),
            pltpu.VMEM((2 * NC, NB + 1, 2 * T, T), F32),
            pltpu.VMEM((NC, 2 * T, T), F32),
            pltpu.VMEM((NC, NB, 2 * T, T), BF),
            pltpu.VMEM((S, D), BF),
            pltpu.VMEM((S, D), BF),
            pltpu.VMEM((NU, D, UR), BF),
            pltpu.VMEM((NU, D, UR), BF),
            pltpu.VMEM((NU, UD + 16, T), F32),
            pltpu.VMEM((NU, UD + 16, T), BF),
            pltpu.VMEM((D, T), F32),
            pltpu.VMEM((T, T), F32),
            pltpu.VMEM((L, T), BF),
            pltpu.VMEM((NQ, UH, T, T), BF),
            pltpu.VMEM((3, NQ, UD, T), BF),
            pltpu.VMEM((3, NQ, UD, T), BF),
            pltpu.VMEM((3, NQ, UD, T), BF),
            pltpu.VMEM((3, UH, NQ, 32, T), BF),
            pltpu.VMEM((40 * T, T), F32),
            pltpu.VMEM((40 * T, T), BF),
            pltpu.VMEM((NQ, UH, 8, T), F32),
            pltpu.VMEM((UD, L), F32),
            pltpu.SMEM((NB,), jnp.int32),
            dma((4 * NC,)), dma((NSEG * NC,)), dma((3 * NU,)), dma(()),
            dma((NU + NQ,)), dma((NSEG * NU,)),
        ],
        compiler_params=pltpu.CompilerParams(
            vmem_limit_bytes=100 * 1024 * 1024,
            flags=({'XLA_TPU_EVENLY_DISTRIBUTE_CRITICAL_NODES': True} if 'EV' in OPT else None)),
        name="h3_infini",
    )(A_q.reshape(S, D), A_k.reshape(S, D), A_v.reshape(S, D), A_shift_k.T, A_ssm_k, A_ssm_D,
      B_x.reshape(S, D), B_wq, B_wk, B_wv, B_wo, B_beta, _DFT)
    return out.reshape(1, S, 2 * D)
```

```python
import math, os

import numpy as np
import jax
import jax.numpy as jnp
from jax import lax
from jax.experimental import pallas as pl
from jax.experimental.pallas import tpu as pltpu

OPT = os.environ.get('OPT', '')
ONLY = os.environ.get('ONLY', '')
ENV = os.environ.get

S, D = 2048, 640
H, DH, NSEG, L = 32, 20, 4, 512
T = 128
NC = D // T
CB = 2 * T
NB = S // CB
NF = T // 8
NQ = L // T
UH = 4
UD = UH * DH
NU = H // UH
UR = L // NU
BF, F32 = jnp.bfloat16, jnp.float32
LOG2E = math.log2(math.e)


def _dft_matrices():
    m = np.arange(T)[:, None]
    r = np.arange(T)[None, :]

    def rows(power):
        ang = np.pi * np.mod((4 * m + 1) * power, 1024) / 512
        f = np.stack([np.cos(ang).reshape(NF, 8, T), -np.sin(ang).reshape(NF, 8, T)], 1)
        return f.reshape(2 * T, T)

    even, odd = rows(2 * r), rows(2 * r + 1)
    lane = np.arange(T)
    even_h = even[:, lane // 2 + (T // 2) * (lane % 2)]
    odd_h = odd[:, lane // 2 + (T // 2) * (1 - lane % 2)]
    inverse = [np.concatenate([f[:T].T, f[T:].T]) / (2 * T) for f in (even, odd)]
    return np.stack([even, odd, even_h, odd_h] + inverse).astype(np.float32).astype(BF)


_DFT = _dft_matrices()


def _halves(x):
    w = pltpu.bitcast(x, jnp.uint32)
    return (lax.bitcast_convert_type(w << 16, F32),
            lax.bitcast_convert_type(w & np.uint32(0xFFFF0000), F32))


def _interleave(even, odd):
    e, o = (lax.bitcast_convert_type(v.astype(BF).astype(F32), jnp.uint32) for v in (even, odd))
    return pltpu.bitcast((e >> 16) | o, BF)


def _dot(a, b):
    return jnp.dot(a, b, preferred_element_type=F32)


def _dot_nt(a, b):
    return lax.dot_general(a, b, (((1,), (1,)), ((), ())), preferred_element_type=F32)


def _phi(t):
    return jnp.where(t > 0, t + 1.0, jnp.exp(t))


def _iota(shape, dim):
    return lax.broadcasted_iota(jnp.int32, shape, dim)


def _head_of(z):
    return sum((z >= DH * i).astype(jnp.int32) for i in range(1, UH))


def _kernel(q_hbm, k_hbm, v_hbm, shift_ref, h_hbm, d_ref, x_hbm, wq_hbm, wk_hbm, wv_hbm,
            wo_hbm, beta_ref, dft_ref, out_hbm,
            q_v, k_v, v_v, h_v, x_v, w_v, wo_v, wt_s, dft_s, kf_s, kv_s, xg_s, y_s, yl_s,
            outa_s, outb_s, ot0_s, ot1_s, mem_s, meml_s, gate_s, bias_s,
            kn_s, rq_s, pk_s, pq_s, vt_s, va_s, vc_s, s_s, p_s, m_s, ret_s, e_s, zero_s,
            sem_w, sem_x, sem_a, sem_q, sem_oa, sem_ob):
    ot_s = (ot0_s, ot1_s)

    def y_of(c):
        return yl_s if c == NC - 1 else y_s.at[c]

    def w_copy(i, t):
        cols = pl.ds(t * T, T)
        return pltpu.make_async_copy((wq_hbm, wk_hbm, wv_hbm)[i].at[:, cols], w_v.at[i, t],
                                     sem_w.at[i * NC + t])

    def wo_copy(n):
        return pltpu.make_async_copy(wo_hbm.at[:, pl.ds(n * T, T)], wo_v.at[n],
                                     sem_w.at[3 * NC + n])

    def x_copy(s, c):
        return pltpu.make_async_copy(x_hbm.at[pl.ds(s * L, L), pl.ds(c * T, T)],
                                     x_v.at[c, pl.ds(s * L, L)], sem_x.at[s * NC + c])

    def kv_copies(u):
        r = pl.ds(pl.multiple_of(u * 2 * T, 2 * T), 2 * T)
        return (pltpu.make_async_copy(k_hbm.at[r], k_v.at[r], sem_a.at[3 * u]),
                pltpu.make_async_copy(v_hbm.at[r], v_v.at[r], sem_a.at[3 * u + 1]))

    def h_copy(u):
        r = pl.ds(pl.multiple_of(u * 2 * T, 2 * T), 2 * T)
        return pltpu.make_async_copy(h_hbm.at[:, r], h_v.at[u], sem_a.at[3 * u + 2])

    def q_copy():
        return pltpu.make_async_copy(q_hbm, q_v, sem_q)

    def oa_copy(rows, lanes):
        return pltpu.make_async_copy(outa_s.at[rows, lanes], out_hbm.at[rows, lanes], sem_oa)

    def ob_copy(rows):
        return pltpu.make_async_copy(outb_s.at[rows], out_hbm.at[rows, pl.ds(D, D)], sem_ob)

    def gate_kv(u, half):
        src = pl.multiple_of(jnp.minimum(u, NB - 1) * CB, CB)
        for c in range(NC):
            lanes = slice(c * T, (c + 1) * T)
            taps = [shift_ref[t:t + 1, lanes].astype(F32) for t in range(4)]
            pe, po = kf_s[c, 0], kf_s[c, 1]
            for r in range(0, T, 16):
                rows = pl.ds(pl.multiple_of(src + 2 * r, 32), 32)
                ke, ko = _halves(k_v[rows, lanes])
                ve, vo = _halves(v_v[rows, lanes])
                e1 = pltpu.roll(jnp.concatenate([pe, ke], axis=0), 1, 0)[8:24]
                odd = jnp.concatenate([po, ko], axis=0)
                o1, o2 = pltpu.roll(odd, 1, 0)[8:24], pltpu.roll(odd, 2, 0)[8:24]
                se = ke * taps[0] + o1 * taps[1] + e1 * taps[2] + o2 * taps[3]
                so = ko * taps[0] + ke * taps[1] + o1 * taps[2] + e1 * taps[3]
                kv_s[half, c, r:r + 16, :] = (se * ve).astype(BF)
                kv_s[half, c, T + r:T + r + 16, :] = (so * vo).astype(BF)
                pe, po = ke[8:16], ko[8:16]
                yield 1
            kf_s[c, 0] = pe
            kf_s[c, 1] = po

    def conv_forward(u, half, c):
        lanes = slice(c * T, (c + 1) * T)
        h0, h1 = (pltpu.bitcast(h_v[u, lanes, j * T:(j + 1) * T], jnp.uint32) for j in range(2))
        even = (_iota(h0.shape, 1) & 1) == 0
        he = pltpu.bitcast(jnp.where(even, h0, pltpu.roll(h1, 1, 1)), BF)
        ho = pltpu.bitcast(jnp.where(even, pltpu.roll(h1, T - 1, 1), h0), BF)
        for base, a, b in (
                (c, _dot(dft_s[0], kv_s[half, c, 0:T, :]), _dot(dft_s[1], kv_s[half, c, T:CB, :])),
                (NC + c, _dot_nt(dft_s[2], he), _dot_nt(dft_s[3], ho))):
            xg_s[base, u, 0:CB, :] = a + b
            xg_s[base, u, CB:2 * CB, :] = a - b

    def conv_mac(items, w=2):
        for c, f in items:
            for k in range(NB // w):
                outs = range(k * w, (k + 1) * w)
                r0 = pl.multiple_of((f + zero_s[k]) * 16, 16)
                plus = {}
                for sign in range(2):
                    re = pl.ds(pl.multiple_of(r0 + sign * CB, 8), 8)
                    im = pl.ds(pl.multiple_of(r0 + sign * CB + 8, 8), 8)
                    acc, g, h = {}, {}, {}

                    def filt(n):
                        if n not in g:
                            for m in (n, n - 1):
                                if m >= 0 and m not in h:
                                    h[m] = (xg_s[NC + c, m, re, :], xg_s[NC + c, m, im, :])
                            if n == 0:
                                g[n] = (h[0][0] + d_row[:, c * T:(c + 1) * T], h[0][1])
                            else:
                                g[n] = (h[n][0] - h[n - 1][1], h[n][1] + h[n - 1][0])
                        return g[n]

                    for b in range(max(outs) + 1):
                        xr, xi = xg_s[c, b, re, :], xg_s[c, b, im, :]
                        cost = 0
                        for a in outs:
                            if b > a:
                                continue
                            gr, gi = filt(a - b)
                            p = (xr * gr - xi * gi, xr * gi + xi * gr)
                            acc[a] = p if a not in acc else (acc[a][0] + p[0], acc[a][1] + p[1])
                            cost += 1
                            if a == b and sign == 0:
                                plus[a] = jnp.concatenate(acc[a], axis=0)
                            elif a == b:
                                minus = jnp.concatenate(acc[a], axis=0)
                                y_of(c)[a, pl.ds(r0, 16), :] = (plus[a] + minus).astype(BF)
                                y_of(c)[a, pl.ds(pl.multiple_of(r0 + CB, 16), 16), :] = (
                                    plus[a] - minus).astype(BF)
                        yield cost

    class Filler:
        def __init__(self):
            self.gen, self.credit, self.in_k = None, 0.0, False

        def pin(self, value, amount):
            if self.gen is None or amount == 0:
                return
            if self.in_k:
                k_v[S:S + 16, 0:T] = jnp.concatenate([value, value], axis=0).astype(BF)
            else:
                xg_s[2 * NC, 0, 0:8, :] = value
            self.credit += amount
            while self.gen is not None and self.credit > 0:
                cost = next(self.gen, None)
                if cost is None:
                    self.gen = None
                else:
                    self.credit -= cost

        def drain(self):
            if self.gen is not None:
                for _ in self.gen:
                    pass
            self.gen = None

    filler = Filler()

    def conv_inverse(u, c):
        r0 = pl.multiple_of(u * CB, CB)
        lanes = slice(c * T, (c + 1) * T)
        qs = _halves(q_v[pl.ds(r0, CB), lanes])
        out = []
        for j in range(2):
            inv = jnp.concatenate([dft_s[4 + j, 0:T, :], dft_s[4 + j, T:CB, :]], axis=1)
            y = _dot(inv, y_of(c)[u, j * CB:(j + 1) * CB, :])
            out.append(qs[j] * y)
        outa_s[pl.ds(r0, CB), lanes] = _interleave(*out)

    def out_proj(o, rows, amount):
        m = o[0].shape[0]
        last = NC - 1
        head = jnp.concatenate(o[0:last], axis=1)

        def pin(part):
            for r in range(0, m, 32):
                filler.pin(part[r:r + 8, 0:T], amount * 32 / (6 * m))

        edge = _dot(o[last], jnp.concatenate(
            [wo_v[n, last * T:D, :] for n in range(last)], axis=1))
        pin(edge)
        yield
        corner = _dot(o[last], wo_v[last, last * T:D, :])
        for n in reversed(range(NC)):
            part = _dot(head, wo_v[n, 0:last * T, :])
            pin(part)
            part = part + (corner if n == last else edge[:, n * T:(n + 1) * T])
            outb_s[rows, n * T:(n + 1) * T] = part.astype(BF)
            yield

    def own_rows(x, i, fill):
        low4 = _iota((8, T), 0) < 4
        full = jnp.full((8, T), fill, F32)
        g0 = 5 * (i // 2)
        if i % 2 == 0:
            body = [x[8 * g0:8 * g0 + 16], jnp.where(low4, x[8 * g0 + 16:8 * g0 + 24], fill)]
        else:
            body = [jnp.where(low4, fill, x[8 * g0 + 16:8 * g0 + 24]), x[8 * g0 + 24:8 * g0 + 40]]
        return jnp.concatenate(body + [full] if i < 2 else [full] + body, axis=0).astype(BF)

    def project(n, amount, need_q=True, need_k=True):
        s, u = n // NU, n % NU
        w0 = pl.multiple_of(u * UD, 16)
        x0 = pl.multiple_of(s * L, L)
        slot = n % 3
        pad = jnp.zeros((T - UD, T), F32)

        def finish(j, qkv):
            cols = slice(j * T, (j + 1) * T)
            qt, kt, vt = qkv[0:UD], qkv[UD:2 * UD], qkv[2 * UD:3 * UD]
            kn_s[cols, :] = jnp.concatenate([kt, pad], axis=0).T.astype(BF)
            qs = qt * (DH ** -0.5 * LOG2E)
            low4 = _iota((8, T), 0) < 4
            left = _iota((8, T), 1) < T // 2
            zero = jnp.zeros((8, T), F32)
            for pr in range(UH // 2):
                qa = [qs[40 * pr + 8 * r:40 * pr + 8 * r + 8] for r in range(3)]
                qb = [pltpu.roll(qs[40 * pr + 8 * r:40 * pr + 8 * r + 8], T // 2, 1) for r in (2, 3, 4)]
                ra = [qa[0], qa[1], jnp.where(low4, qa[2], 0.0)]
                rb = [jnp.where(low4, 0.0, qb[0]), qb[1], qb[2]]
                rh = [jnp.where(left, 0.0, qa[0]), jnp.where(left, 0.0, qa[1]),
                      jnp.where(left, rb[0], ra[2]),
                      jnp.where(left, qb[1], 0.0), jnp.where(left, qb[2], 0.0)]
                for i, rows in ((2 * pr, ra), (2 * pr + 1, rb)):
                    rows = rows + [zero] if pr == 0 else [zero] + rows
                    rq_s[j, i, 16 * i:16 * i + 32, :] = jnp.concatenate(rows, axis=0).astype(BF)
                rows = rh + [zero] if pr == 0 else [zero] + rh
                rq_s[j, UH + pr, 32 * pr:32 * pr + 48, :] = jnp.concatenate(rows, axis=0).astype(BF)
            for i in range(UH):
                va_s[slot, i, j] = own_rows(vt, i, 1.0)
            if need_q:
                pq_s[slot, j] = _phi(qt).astype(BF)
            if need_k:
                pk_s[slot, j] = _phi(kt).astype(BF)
                vt_s[slot, j] = vt.astype(BF)

        if 'pc' in OPT:
            qkv = None
            for c in range(NC):
                w = jnp.concatenate([wt_s[c, i, pl.ds(w0, UD), :] for i in range(3)], axis=0)
                part = _dot_nt(w, x_v[c, pl.ds(x0, L), :])
                for r in range(0, 3 * UD, 24):
                    filler.pin(part[r:r + 8, 0:T], amount / (10 * NC))
                qkv = part if qkv is None else qkv + part
                yield c
            for j in range(NQ):
                finish(j, qkv[:, j * T:(j + 1) * T])
            return
        if 'pj' in OPT:
            acc = None
            for job in range(NQ * NC):
                j, c = divmod(job, NC)
                j = NQ - 1 - j
                w = jnp.concatenate([wt_s[c, i, pl.ds(w0, UD), :] for i in range(3)], axis=0)
                part = _dot_nt(w, x_v[c, pl.ds(pl.multiple_of(x0 + j * T, T), T), :])
                if job % 4 == 0:
                    for r in range(0, 3 * UD, 24):
                        filler.pin(part[r:r + 8], amount / (10 * NC))
                acc = part if c == 0 else acc + part
                if c == NC - 1:
                    finish(j, acc)
                if job % 4 == 3:
                    yield job
            return
        w = [jnp.concatenate([wt_s[c, i, pl.ds(w0, UD), :] for i in range(3)], axis=0)
             for c in range(NC)]
        part = _dot_nt(w[NC - 1], x_v[NC - 1, pl.ds(x0, L), :])
        for j in range(NQ):
            e_s[j] = part[:, j * T:(j + 1) * T]
        for r in range(0, 3 * UD, 24):
            filler.pin(part[r:r + 8, 0:T], amount / (10 * NC))
        yield
        w = jnp.concatenate(w[0:NC - 1], axis=1)
        for j in reversed(range(NQ)):
            rows = pl.ds(pl.multiple_of(x0 + j * T, T), T)
            part = _dot_nt(w, jnp.concatenate([x_v[c, rows, :] for c in range(NC - 1)], axis=1))
            for r in range(0, 3 * UD, 24):
                filler.pin(part[r:r + 8], amount / (10 * NC))
            finish(j, part + e_s[j])
            yield

    HALF = T // 2

    def s_off(j, i, t, n=T):
        return pl.ds((2 * j * (j + 1) + i * (j + 1) + t) * T, n)

    def hi_off(j, pr):
        return pl.ds((2 * j * (j + 1) + 2 * pr * (j + 1) + j) * T + HALF, HALF)

    def col_max(x):
        return jnp.max(x.reshape(x.shape[0] // 8, 8, T), axis=0)

    def scores(j, t, top, amount):
        rq = jnp.concatenate([rq_s[j, i] for i in range(UH)], axis=1)
        n = T if t < j else HALF
        sc = _dot(kn_s[t * T:t * T + n, :], rq)
        if t == j:
            rh = jnp.concatenate([rq_s[j, UH + pr] for pr in range(2)], axis=1)
            hi = _dot(kn_s[t * T + HALF:(t + 1) * T, :], rh)
        for i in range(UH):
            si = sc[:, i * T:(i + 1) * T]
            if t == j:
                si = si + bias_s[i % 2]
            s_s[s_off(j, i, t, n), :] = si
            if i == 0:
                for r in range(0, n, 32):
                    filler.pin(si[r:r + 8], amount * 32 / n)
            top[i] = col_max(si) if t == 0 else jnp.maximum(top[i], col_max(si))
        if t < j:
            return
        left = _iota((8, T), 1) < HALF
        for pr in range(2):
            si = hi[:, pr * T:(pr + 1) * T] + bias_s[2]
            s_s[hi_off(j, pr), :] = si
            mh = col_max(si)
            ma = jnp.maximum(top[2 * pr], jnp.where(left, -jnp.inf, mh))
            mb = jnp.maximum(top[2 * pr + 1], jnp.where(left, mh, -jnp.inf))
            ma = jnp.broadcast_to(jnp.max(ma, axis=0, keepdims=True), (8, T))
            mb = jnp.broadcast_to(jnp.max(mb, axis=0, keepdims=True), (8, T))
            m_s[j, 2 * pr] = ma
            m_s[j, 2 * pr + 1] = mb
            m_s[j, UH + pr] = jnp.where(left, mb, ma)

    def weights(rows, j, i):
        sc = s_s[rows, :]
        m = jnp.concatenate([m_s[j, i]] * (sc.shape[0] // 8), axis=0)
        return jnp.exp2(sc - m).astype(BF)

    def softmax(j, t):
        n = T if t < j else HALF
        for i in range(UH):
            p_s[s_off(j, i, t, n), :] = weights(s_off(j, i, t, n), j, i)
        if t < j:
            return
        left = _iota((HALF // 2, T), 1) < HALF
        none = jnp.zeros((HALF // 2, T), jnp.uint32)
        for pr in range(2):
            p = pltpu.bitcast(weights(hi_off(j, pr), j, UH + pr), jnp.uint32)
            for i, part in ((2 * pr, jnp.where(left, none, p)), (2 * pr + 1, jnp.where(left, p, none))):
                p_s[pl.ds(s_off(j, i, t).start + HALF, HALF), :] = pltpu.bitcast(part, BF)

    def spread(a, b):
        low4 = _iota(a.shape, 0) < 4
        ar, br = pltpu.roll(a, 4, 0), pltpu.roll(b, 4, 0)
        r0, r1 = jnp.where(low4, a, ar), jnp.where(low4, ar, a)
        r2, r3 = jnp.where(low4, b, br), jnp.where(low4, br, b)
        return jnp.concatenate([r0, r0, a, r1, r1, r2, r2, b, r3, r3], axis=0)

    def retrieve(n):
        u, slot = n % NU, n % 3
        zpad = jnp.zeros((T - UD, T), BF)
        pq = jnp.concatenate(
            [jnp.concatenate([pq_s[slot, j], zpad], axis=0) for j in range(NQ)], axis=1)
        ret = _dot(meml_s[u], pq)
        rd = 1.0 / (ret[UD:UD + 16] + 1e-6)
        ret_s[...] = ret[0:UD] * spread(rd[0:8], rd[8:16])

    def update(n, s):
        u, slot = n % NU, n % 3
        zpad = jnp.zeros((T - UD, T), BF)
        va = jnp.concatenate(
            [jnp.concatenate([vt_s[slot, j], jnp.ones((16, T), BF)], axis=0) for j in range(NQ)],
            axis=1)
        pk = jnp.concatenate(
            [jnp.concatenate([pk_s[slot, j], zpad], axis=0) for j in range(NQ)], axis=1)
        mem = _dot_nt(va, pk)
        if s > 0:
            mem = mem_s[u] + mem
        if s < NSEG - 2:
            mem_s[u] = mem
        row = _iota((UD + 16, T), 0)
        row_head = jnp.where(row < UD, _head_of(row), (row - UD) >> 2)
        meml_s[u] = jnp.where(row_head == _head_of(_iota((UD + 16, T), 1)), mem, 0.0).astype(BF)

    def values(n, s, j, t, acc):
        u, slot = n % NU, n % 3
        for i in range(UH):
            part = _dot(vc_s[i, t], p_s[s_off(j, i, t), :])
            acc[i] = part if t == 0 else acc[i] + part
        if t < j:
            return
        heads = []
        for i in range(UH):
            den = acc[i][24:32] if i < 2 else acc[i][0:8]
            val = acc[i][0:24] if i < 2 else acc[i][8:32]
            val = val * jnp.concatenate([1.0 / den] * 3, axis=0)
            heads.append(pltpu.roll(val, HALF, 1) if i % 2 else val)
        low4 = _iota((8, T), 0) < 4
        att = jnp.concatenate([
            heads[0][0:16], jnp.where(low4, heads[0][16:24], heads[1][0:8]), heads[1][8:24],
            heads[2][0:16], jnp.where(low4, heads[2][16:24], heads[3][0:8]), heads[3][8:24]], axis=0)
        rows = pl.ds(pl.multiple_of(u * UD, 16), UD)
        gt = gate_s[rows, :]
        o = (1.0 - gt) * att
        if s > 0:
            o = o + gt * ret_s[:, j * T:(j + 1) * T]
        o = o.astype(BF)
        ot_s[s % 2][j, rows, :] = o

    ATT = 'R U P Q30 Q31 Q32 Q33 P V30 V31 Q20 V32 Q21 V33 Q22 P V20 Q10 V21 Q11 V22 P Q00 V10 V11 P V00 '
    ATX = 'R U P Q30 Q31 Q32 Q33 P V30 X V31 Q20 V32 Q21 V33 Q22 P V20 X Q10 V21 Q11 V22 P X Q00 V10 V11 P V00 '
    ORDERS = [
        ENV('ORD0', ATX + 'X X / ' + ATX + 'X X'),
        ENV('ORD1', ATT + '/ ' + ATT + 'O O O O O O'),
        ENV('ORD1', ATT + '/ ' + ATT + 'O O O O O O'),
        ENV('ORD3', ATX + 'X / ' + ATX + 'X O O O O O O'),
    ]
    ORDERS = [[half.split() for half in order.split('/')] for order in ORDERS]
    SHARE = [[float(v) for v in ENV(k, d).split(',')] for k, d in
             (('SH0', '0.4,0.6,0'), ('SH1', '0.4,0.5,0.1'), ('SH1', '0.4,0.5,0.1'), ('SH3', '0.3,0.6,0.1'))]

    def step(n, s, order, total, jobs=(), oproj=None, do_proj=True, do_scores=True,
             do_values=True, need_q=True):
        jobs = list(jobs)
        share = SHARE[s]
        proj = project(n + 2, total * share[1], need_q=need_q, need_k=s < NSEG - 1)
        top, acc = [None] * UH, {}
        if do_values:
            vc_s[...] = va_s[n % 3]
        for tok in order:
            if tok[0] == 'Q':
                j, t = int(tok[1]), int(tok[2])
                if do_values:
                    softmax(j, t)
                if do_scores:
                    scores(j, t, top, total * share[0] / 10)
            elif tok[0] == 'V':
                if do_values:
                    values(n, s, int(tok[1]), int(tok[2]), acc.setdefault(tok[1], [None] * UH))
            elif tok == 'P':
                if do_proj:
                    next(proj)
            elif tok == 'R':
                if do_values and s > 0:
                    retrieve(n)
            elif tok == 'U':
                if do_values and s < NSEG - 1:
                    update(n, s)
            elif tok == 'O':
                if oproj is not None:
                    next(oproj)
            elif tok == 'X':
                if jobs:
                    jobs.pop(0)()
        assert not jobs

    def out_tiles(s, j):
        return [ot_s[s % 2][j, c * T:(c + 1) * T, :].T for c in range(NC)]

    def pair_step(s, j, last=False, between=lambda half: None):
        us = (2 * j, 2 * j + 1)
        stream, total, oproj = None, 0, None
        if s == 0:
            total = 8 * NC
        elif 'nomac' not in OPT:
            tiles = (2 * (s - 1), 2 * s - 1) if s < NSEG - 1 else (NC - 1,)
            total = 72 * 2 * len(tiles)
            stream = conv_mac([(c, 2 * u + r) for u in us for c in tiles for r in range(2)], int(ENV('W', '2')))
        filler.gen, filler.credit, filler.in_k = stream, 0.0, s == 0
        if s > 0:
            rows = pl.ds(pl.multiple_of((s - 1) * L + j * T, T), T)
            oproj = out_proj(out_tiles(s - 1, j), rows, 2 * total * SHARE[s][2])
        for half, u in enumerate(us):
            jobs = []
            if s == 0:
                between(half)
                filler.drain()
                filler.gen, filler.credit = gate_kv(u + 1, 1 - half), 0.0
                jobs = [lambda c=c, u=u, half=half: conv_forward(u, half, c) for c in range(NC)]
            elif s == NSEG - 1:
                jobs = [lambda c=c, u=u: conv_inverse(u, c) for c in range(NC - 1)]
            step(s * NU + u, s, ORDERS[s][half], total, jobs, oproj, do_proj=not last,
                 do_scores=not (last and half == 1))
        filler.drain()

    def transpose_weights(t):
        for i in range(3):
            for c in range(NC):
                wt_s[c, i, t * T:(t + 1) * T, :] = w_v[i, t, c * T:(c + 1) * T, :].T

    d_row = d_ref[...].astype(F32).reshape(1, D)

    if ONLY:
        for k in range(NB):
            zero_s[k] = 0
        with jax.named_scope('loop'):
            lax.fori_loop(0, NQ, lambda j, _: pair_step(int(ONLY), j), None)

        def fin(i, _):
            z = (y_s[i, i, 0:16, :].astype(F32) + yl_s[i, 0:16, :] + ot0_s[i, 0:16, :] + ot1_s[i, 0:16, :] + mem_s[i, 0:16, :]
                 + xg_s[i, i, 0:16, :] + meml_s[i, 0:16, :] + kv_s[0, i, 0:16, :] + p_s[pl.ds(i * 16, 16), :] + s_s[pl.ds(i * 16, 16), :])
            outa_s[0:16, 0:T] = z.astype(BF)
            cp = pltpu.make_async_copy(outa_s, out_hbm.at[:, pl.ds(0, D)], sem_q); cp.start(); cp.wait()
            cp = pltpu.make_async_copy(outb_s, out_hbm.at[:, pl.ds(D, D)], sem_q); cp.start(); cp.wait()
        lax.fori_loop(0, 4, fin, None)
        return

    for i in range(3):
        w_copy(i, 0).start()
    for c in range(NC):
        x_copy(0, c).start()

    sc_setup = jax.named_scope('setup')
    sc_setup.__enter__()
    g = jax.nn.sigmoid(beta_ref[...].astype(F32).reshape(1, H))
    rr = _iota((D, H), 0)
    hh = _iota((D, H), 1) * DH
    gate = jnp.sum(jnp.where((rr >= hh) & (rr < hh + DH), g, 0.0), axis=1, keepdims=True)
    gate_s[...] = jnp.broadcast_to(gate, (D, T))
    key, lane = _iota((T // 2, T), 0), _iota((T // 2, T), 1)
    for b, query in enumerate((lane, lane ^ (T // 2), lane & (T // 2 - 1))):
        bias_s[b] = jnp.where(key > query, -1e9 * LOG2E, 0.0).astype(F32)
    rq_s[...] = jnp.zeros(rq_s.shape, BF)
    dft_s[...] = dft_ref[...]
    kf_s[...] = jnp.zeros(kf_s.shape, F32)
    for k in range(NB):
        zero_s[k] = 0

    sc_setup.__exit__(None, None, None)
    with jax.named_scope("w0"):
        for i in range(3):
            w_copy(i, 0).wait()
        for i in range(3):
            w_copy(i, 1).start()
    with jax.named_scope("t0"):
        transpose_weights(0)
    with jax.named_scope("x0"):
        for c in range(NC):
            x_copy(0, c).wait()
        for i in range(3):
            w_copy(i, 2).start()
    with jax.named_scope("p0"):
        for _ in project(0, 0, need_q=False):
            pass
    with jax.named_scope("w1"):
        for i in range(3):
            w_copy(i, 1).wait()
        for t in range(3, NC):
            for i in range(3):
                w_copy(i, t).start()
        for cp in kv_copies(0):
            cp.start()
    with jax.named_scope("p1"):
        transpose_weights(1)
        step(-1, 0, ORDERS[0][0], 0, do_values=False, need_q=False)
    with jax.named_scope("w2"):
        for t in range(2, NC):
            for i in range(3):
                w_copy(i, t).wait()
        for cp in kv_copies(0):
            cp.wait()
        h_copy(0).start()
        for cp in kv_copies(1):
            cp.start()
    with jax.named_scope("p2"):
        for t in range(2, NC):
            transpose_weights(t)
        for _ in gate_kv(0, 0):
            pass
    h_copy(1).start()
    for cp in kv_copies(2):
        cp.start()

    def seg0(j, _):
        def between(half):
            u = 2 * j + half
            h_copy(u).wait()
            if half == 0:
                for cp in kv_copies(u + 1):
                    cp.wait()
                return

            @pl.when(j == 0)
            def _():
                for later in range(2, NB):
                    h_copy(later).start()
                    if later + 1 < NB:
                        for cp in kv_copies(later + 1):
                            cp.start()
                    if later == 3:
                        for c in range(NC):
                            x_copy(1, c).start()
                for n in range(NC):
                    wo_copy(n).start()
                for s in range(2, NSEG):
                    for c in range(NC):
                        x_copy(s, c).start()
                q_copy().start()

            @pl.when(j < NQ - 1)
            def _():
                for cp in kv_copies(u + 1):
                    cp.wait()

            @pl.when(j == NQ - 1)
            def _():
                for c in range(NC):
                    x_copy(1, c).wait()
        pair_step(0, j, between=between)
    with jax.named_scope("seg0"):
        lax.fori_loop(0, NQ, seg0, None)

    for n in range(NC):
        wo_copy(n).wait()

    for s in (1, 2):
        for c in range(NC):
            x_copy(s + 1, c).wait()
        with jax.named_scope(f"seg{s}"):
            lax.fori_loop(0, NQ, lambda j, _, s=s: pair_step(s, j), None)
        ob_copy(pl.ds((s - 1) * L, L)).start()

    q_copy().wait()

    first = pl.ds(0, (NC - 1) * T)
    with jax.named_scope("seg3"):
        lax.fori_loop(0, NQ - 1, lambda j, _: pair_step(3, j), None)
    oa_copy(pl.ds(0, S - L), first).start()
    ob_copy(pl.ds(2 * L, L - T)).start()
    with jax.named_scope("seg3e"):
        pair_step(3, NQ - 1, last=True)
    oa_copy(pl.ds(S - L, L), first).start()
    ob_copy(pl.ds(3 * L - T, T)).start()

    with jax.named_scope("tail"):
        for u in range(NB):
            conv_inverse(u, NC - 1)
        oa_copy(pl.ds(0, S), pl.ds((NC - 1) * T, T)).start()
        for j in range(NQ):
            rows = pl.ds((NSEG - 1) * L + j * T, T)
            for _ in out_proj(out_tiles(NSEG - 1, j), rows, 0):
                pass
            ob_copy(rows).start()

    oa_copy(pl.ds(0, S), pl.ds(0, D)).wait()
    ob_copy(pl.ds(0, S)).wait()


@jax.jit
def pallas_concat_heads__ssm_conv_h3__memory_aug_infini_attn__prompt_kernel(
    A_q, A_k, A_v, A_shift_k, A_ssm_k, A_ssm_D, B_x, B_wq, B_wk, B_wv, B_wo, B_beta,
):
    hbm = pl.BlockSpec(memory_space=pl.ANY)
    vmem = pl.BlockSpec(memory_space=pltpu.VMEM)
    dma = pltpu.SemaphoreType.DMA
    out = pl.pallas_call(
        _kernel,
        out_shape=jax.ShapeDtypeStruct((S, 2 * D), BF),
        in_specs=[hbm, hbm, hbm, vmem, hbm, vmem, hbm, hbm, hbm, hbm, hbm, vmem, vmem],
        out_specs=hbm,
        scratch_shapes=[
            pltpu.VMEM((S, D), BF),
            pltpu.VMEM((S + 16, D), BF),
            pltpu.VMEM((S, D), BF),
            pltpu.VMEM((NU, D, 2 * T), BF),
            pltpu.VMEM((NC, S, T), BF),
            pltpu.VMEM((3, NC, D, T), BF),
            pltpu.VMEM((NC, D, T), BF),
            pltpu.VMEM((NC, 3, D, T), BF),
            pltpu.VMEM((6, CB, T), BF),
            pltpu.VMEM((NC, 2, 8, T), F32),
            pltpu.VMEM((2, NC, CB, T), BF),
            pltpu.VMEM((2 * NC + 1, NB, 2 * CB, T), F32),
            pltpu.VMEM((NC - 1, NB, 2 * CB, T), BF),
            pltpu.VMEM((NB, 2 * CB, T), BF),
            pltpu.VMEM((S, D), BF),
            pltpu.VMEM((S, D), BF),
            pltpu.VMEM((NQ, D, T), BF),
            pltpu.VMEM((NQ, D, T), BF),
            pltpu.VMEM((NU, UD + 16, T), F32),
            pltpu.VMEM((NU, UD + 16, T), BF),
            pltpu.VMEM((D, T), F32),
            pltpu.VMEM((3, T // 2, T), F32),
            pltpu.VMEM((L, T), BF),
            pltpu.VMEM((NQ, UH + 2, T, T), BF),
            pltpu.VMEM((3, NQ, UD, T), BF),
            pltpu.VMEM((3, NQ, UD, T), BF),
            pltpu.VMEM((3, NQ, UD, T), BF),
            pltpu.VMEM((3, UH, NQ, 32, T), BF),
            pltpu.VMEM((UH, NQ, 32, T), BF),
            pltpu.VMEM((40 * T, T), F32),
            pltpu.VMEM((40 * T, T), BF),
            pltpu.VMEM((NQ, UH + 2, 8, T), F32),
            pltpu.VMEM((UD, L), F32),
            pltpu.VMEM((NQ, 3 * UD, T), F32),
            pltpu.SMEM((NB,), jnp.int32),
            dma((4 * NC,)), dma((NSEG * NC,)), dma((3 * NU,)), dma(()),
            dma(()), dma(()),
        ],
        compiler_params=pltpu.CompilerParams(
            vmem_limit_bytes=100 * 1024 * 1024,
            flags=({'XLA_TPU_EVENLY_DISTRIBUTE_CRITICAL_NODES': True} if 'EV' in OPT else None)),
        name="h3_infini",
    )(A_q.reshape(S, D), A_k.reshape(S, D), A_v.reshape(S, D), A_shift_k.T, A_ssm_k, A_ssm_D,
      B_x.reshape(S, D), B_wq, B_wk, B_wv, B_wo, B_beta, _DFT)
    return out.reshape(1, S, 2 * D)
```

```python
import math, os

import numpy as np
import jax
import jax.numpy as jnp
from jax import lax
from jax.experimental import pallas as pl
from jax.experimental.pallas import tpu as pltpu

OPT = os.environ.get('OPT', '')
ONLY = os.environ.get('ONLY', '')
ENV = os.environ.get

S, D = 2048, 640
H, DH, NSEG, L = 32, 20, 4, 512
T = 128
NC = D // T
CB = 2 * T
NB = S // CB
NF = T // 8
NQ = L // T
UH = 4
UD = UH * DH
NU = H // UH
UR = L // NU
BF, F32 = jnp.bfloat16, jnp.float32
LOG2E = math.log2(math.e)


def _dft_matrices():
    m = np.arange(T)[:, None]
    r = np.arange(T)[None, :]

    def rows(power):
        ang = np.pi * np.mod((4 * m + 1) * power, 1024) / 512
        f = np.stack([np.cos(ang).reshape(NF, 8, T), -np.sin(ang).reshape(NF, 8, T)], 1)
        return f.reshape(2 * T, T)

    even, odd = rows(2 * r), rows(2 * r + 1)
    lane = np.arange(T)
    even_h = even[:, lane // 2 + (T // 2) * (lane % 2)]
    odd_h = odd[:, lane // 2 + (T // 2) * (1 - lane % 2)]
    inverse = [np.concatenate([f[:T].T, f[T:].T]) / (2 * T) for f in (even, odd)]
    return np.stack([even, odd, even_h, odd_h] + inverse).astype(np.float32).astype(BF)


_DFT = _dft_matrices()


def _halves(x):
    w = pltpu.bitcast(x, jnp.uint32)
    return (lax.bitcast_convert_type(w << 16, F32),
            lax.bitcast_convert_type(w & np.uint32(0xFFFF0000), F32))


def _interleave(even, odd):
    e, o = (lax.bitcast_convert_type(v.astype(BF).astype(F32), jnp.uint32) for v in (even, odd))
    return pltpu.bitcast((e >> 16) | o, BF)


def _dot(a, b):
    return jnp.dot(a, b, preferred_element_type=F32)


def _dot_nt(a, b):
    return lax.dot_general(a, b, (((1,), (1,)), ((), ())), preferred_element_type=F32)


def _phi(t):
    return jnp.where(t > 0, t + 1.0, jnp.exp(t))


def _iota(shape, dim):
    return lax.broadcasted_iota(jnp.int32, shape, dim)


def _head_of(z):
    return sum((z >= DH * i).astype(jnp.int32) for i in range(1, UH))


def _kernel(q_hbm, k_hbm, v_hbm, shift_ref, h_hbm, d_ref, x_hbm, wq_hbm, wk_hbm, wv_hbm,
            wo_hbm, beta_ref, dft_ref, out_hbm,
            q_v, k_v, v_v, h_v, x_v, w_v, wo_v, wt_s, dft_s, kf_s, kv_s, xg_s, y_s, yl_s,
            outa_s, outb_s, ot0_s, ot1_s, mem_s, meml_s, gate_s, bias_s,
            kn_s, rq_s, pk0_s, pk1_s, pq0_s, pq1_s, vt0_s, vt1_s, va0_s, va1_s, s_s, p0_s, p1_s, m_s, ret_s, e_s, zero_s,
            sem_w, sem_x, sem_a, sem_q, sem_oa, sem_ob):
    ot_s = (ot0_s, ot1_s)
    pk_s, pq_s, vt_s = (pk0_s, pk1_s), (pq0_s, pq1_s), (vt0_s, vt1_s)
    va_s, p_s = (va0_s, va1_s), (p0_s, p1_s)

    def y_of(c):
        return yl_s if c == NC - 1 else y_s.at[c]

    def w_copy(i, t):
        cols = pl.ds(t * T, T)
        return pltpu.make_async_copy((wq_hbm, wk_hbm, wv_hbm)[i].at[:, cols], w_v.at[i, t],
                                     sem_w.at[i * NC + t])

    def wo_copy(n):
        return pltpu.make_async_copy(wo_hbm.at[:, pl.ds(n * T, T)], wo_v.at[n],
                                     sem_w.at[3 * NC + n])

    def x_copy(s, c):
        return pltpu.make_async_copy(x_hbm.at[pl.ds(s * L, L), pl.ds(c * T, T)],
                                     x_v.at[c, pl.ds(s * L, L)], sem_x.at[s * NC + c])

    def kv_copies(u):
        src = pl.ds(pl.multiple_of(jnp.minimum(u, NB - 1) * CB, CB), CB)
        dst = pl.ds(pl.multiple_of(u * CB, CB), CB)
        return (pltpu.make_async_copy(k_hbm.at[src], k_v.at[dst], sem_a.at[3 * u]),
                pltpu.make_async_copy(v_hbm.at[src], v_v.at[dst], sem_a.at[3 * u + 1]))

    def h_copy(u):
        r = pl.ds(pl.multiple_of(u * 2 * T, 2 * T), 2 * T)
        return pltpu.make_async_copy(h_hbm.at[:, r], h_v.at[u], sem_a.at[3 * u + 2])

    def q_copy():
        return pltpu.make_async_copy(q_hbm, q_v, sem_q)

    def oa_copy(rows, lanes):
        return pltpu.make_async_copy(outa_s.at[rows, lanes], out_hbm.at[rows, lanes], sem_oa)

    def ob_copy(rows):
        return pltpu.make_async_copy(outb_s.at[rows], out_hbm.at[rows, pl.ds(D, D)], sem_ob)

    def gate_kv(u, half):
        src = pl.multiple_of(u * CB, CB)
        for c in range(NC):
            lanes = slice(c * T, (c + 1) * T)
            taps = [shift_ref[t:t + 1, lanes].astype(F32) for t in range(4)]
            pe, po = kf_s[c, 0], kf_s[c, 1]
            for r in range(0, T, 16):
                rows = pl.ds(pl.multiple_of(src + 2 * r, 32), 32)
                ke, ko = _halves(k_v[rows, lanes])
                ve, vo = _halves(v_v[rows, lanes])
                e1 = pltpu.roll(jnp.concatenate([pe, ke], axis=0), 1, 0)[8:24]
                odd = jnp.concatenate([po, ko], axis=0)
                o1, o2 = pltpu.roll(odd, 1, 0)[8:24], pltpu.roll(odd, 2, 0)[8:24]
                se = ke * taps[0] + o1 * taps[1] + e1 * taps[2] + o2 * taps[3]
                so = ko * taps[0] + ke * taps[1] + o1 * taps[2] + e1 * taps[3]
                kv_s[half, c, r:r + 16, :] = (se * ve).astype(BF)
                kv_s[half, c, T + r:T + r + 16, :] = (so * vo).astype(BF)
                pe, po = ke[8:16], ko[8:16]
                yield 1
            kf_s[c, 0] = pe
            kf_s[c, 1] = po

    def conv_forward(u, half, c):
        lanes = slice(c * T, (c + 1) * T)
        h0, h1 = (pltpu.bitcast(h_v[u, lanes, j * T:(j + 1) * T], jnp.uint32) for j in range(2))
        even = (_iota(h0.shape, 1) & 1) == 0
        he = pltpu.bitcast(jnp.where(even, h0, pltpu.roll(h1, 1, 1)), BF)
        ho = pltpu.bitcast(jnp.where(even, pltpu.roll(h1, T - 1, 1), h0), BF)
        for base, a, b in (
                (c, _dot(dft_s[0], kv_s[half, c, 0:T, :]), _dot(dft_s[1], kv_s[half, c, T:CB, :])),
                (NC + c, _dot_nt(dft_s[2], he), _dot_nt(dft_s[3], ho))):
            xg_s[base, u, 0:CB, :] = a + b
            xg_s[base, u, CB:2 * CB, :] = a - b

    def conv_mac(items, w=2):
        for c, f in items:
            for k in range(NB // w):
                outs = range(k * w, (k + 1) * w)
                r0 = pl.multiple_of((f + zero_s[k]) * 16, 16)
                plus = {}
                for sign in range(2):
                    re = pl.ds(pl.multiple_of(r0 + sign * CB, 8), 8)
                    im = pl.ds(pl.multiple_of(r0 + sign * CB + 8, 8), 8)
                    acc, g, h = {}, {}, {}

                    def filt(n):
                        if n not in g:
                            for m in (n, n - 1):
                                if m >= 0 and m not in h:
                                    h[m] = (xg_s[NC + c, m, re, :], xg_s[NC + c, m, im, :])
                            if n == 0:
                                g[n] = (h[0][0] + d_row[:, c * T:(c + 1) * T], h[0][1])
                            else:
                                g[n] = (h[n][0] - h[n - 1][1], h[n][1] + h[n - 1][0])
                        return g[n]

                    for b in range(max(outs) + 1):
                        xr, xi = xg_s[c, b, re, :], xg_s[c, b, im, :]
                        cost = 0
                        for a in outs:
                            if b > a:
                                continue
                            gr, gi = filt(a - b)
                            p = (xr * gr - xi * gi, xr * gi + xi * gr)
                            acc[a] = p if a not in acc else (acc[a][0] + p[0], acc[a][1] + p[1])
                            cost += 1
                            if a == b and sign == 0:
                                plus[a] = jnp.concatenate(acc[a], axis=0)
                            elif a == b:
                                minus = jnp.concatenate(acc[a], axis=0)
                                y_of(c)[a, pl.ds(r0, 16), :] = (plus[a] + minus).astype(BF)
                                y_of(c)[a, pl.ds(pl.multiple_of(r0 + CB, 16), 16), :] = (
                                    plus[a] - minus).astype(BF)
                        yield cost

    class Filler:
        def __init__(self):
            self.gen, self.credit, self.in_k = None, 0.0, False

        def pin(self, value, amount):
            if self.gen is None or amount == 0:
                return
            if self.in_k:
                k_v[S + CB:S + CB + 16, 0:T] = jnp.concatenate([value, value], axis=0).astype(BF)
            else:
                xg_s[2 * NC, 0, 0:8, :] = value
            self.credit += amount
            while self.gen is not None and self.credit > 0:
                cost = next(self.gen, None)
                if cost is None:
                    self.gen = None
                else:
                    self.credit -= cost

        def drain(self):
            if self.gen is not None:
                for _ in self.gen:
                    pass
            self.gen = None

    filler = Filler()

    def conv_inverse(u, c):
        r0 = pl.multiple_of(u * CB, CB)
        lanes = slice(c * T, (c + 1) * T)
        qs = _halves(q_v[pl.ds(r0, CB), lanes])
        out = []
        for j in range(2):
            inv = jnp.concatenate([dft_s[4 + j, 0:T, :], dft_s[4 + j, T:CB, :]], axis=1)
            y = _dot(inv, y_of(c)[u, j * CB:(j + 1) * CB, :])
            out.append(qs[j] * y)
        outa_s[pl.ds(r0, CB), lanes] = _interleave(*out)

    def out_proj(o, rows, amount):
        m = o[0].shape[0]
        last = NC - 1
        head = jnp.concatenate(o[0:last], axis=1)

        def pin(part):
            for r in range(0, m, 32):
                filler.pin(part[r:r + 8, 0:T], amount * 32 / (6 * m))

        edge = _dot(o[last], jnp.concatenate(
            [wo_v[n, last * T:D, :] for n in range(last)], axis=1))
        pin(edge)
        yield
        corner = _dot(o[last], wo_v[last, last * T:D, :])
        for n in reversed(range(NC)):
            part = _dot(head, wo_v[n, 0:last * T, :])
            pin(part)
            part = part + (corner if n == last else edge[:, n * T:(n + 1) * T])
            outb_s[rows, n * T:(n + 1) * T] = part.astype(BF)
            yield

    def own_rows(x, i, fill):
        low4 = _iota((8, T), 0) < 4
        full = jnp.full((8, T), fill, F32)
        g0 = 5 * (i // 2)
        if i % 2 == 0:
            body = [x[8 * g0:8 * g0 + 16], jnp.where(low4, x[8 * g0 + 16:8 * g0 + 24], fill)]
        else:
            body = [jnp.where(low4, fill, x[8 * g0 + 16:8 * g0 + 24]), x[8 * g0 + 24:8 * g0 + 40]]
        return jnp.concatenate(body + [full] if i < 2 else [full] + body, axis=0).astype(BF)

    def project(n, par, amount, need_q=True, need_k=True):
        s, u = n // NU, n % NU
        w0 = pl.multiple_of(u * UD, 16)
        x0 = pl.multiple_of(s * L, L)
        slot = (n // 2) % 2
        pad = jnp.zeros((T - UD, T), F32)

        def finish(j, qkv):
            cols = slice(j * T, (j + 1) * T)
            qt, kt, vt = qkv[0:UD], qkv[UD:2 * UD], qkv[2 * UD:3 * UD]
            kn_s[cols, :] = jnp.concatenate([kt, pad], axis=0).T.astype(BF)
            qs = qt * (DH ** -0.5 * LOG2E)
            low4 = _iota((8, T), 0) < 4
            left = _iota((8, T), 1) < T // 2
            zero = jnp.zeros((8, T), F32)
            for pr in range(UH // 2):
                qa = [qs[40 * pr + 8 * r:40 * pr + 8 * r + 8] for r in range(3)]
                qb = [pltpu.roll(qs[40 * pr + 8 * r:40 * pr + 8 * r + 8], T // 2, 1) for r in (2, 3, 4)]
                ra = [qa[0], qa[1], jnp.where(low4, qa[2], 0.0)]
                rb = [jnp.where(low4, 0.0, qb[0]), qb[1], qb[2]]
                rh = [jnp.where(left, 0.0, qa[0]), jnp.where(left, 0.0, qa[1]),
                      jnp.where(left, rb[0], ra[2]),
                      jnp.where(left, qb[1], 0.0), jnp.where(left, qb[2], 0.0)]
                for i, rows in ((2 * pr, ra), (2 * pr + 1, rb)):
                    rows = rows + [zero] if pr == 0 else [zero] + rows
                    rq_s[j, i, 16 * i:16 * i + 32, :] = jnp.concatenate(rows, axis=0).astype(BF)
                rows = rh + [zero] if pr == 0 else [zero] + rh
                rq_s[j, UH + pr, 32 * pr:32 * pr + 48, :] = jnp.concatenate(rows, axis=0).astype(BF)
            for i in range(UH):
                va_s[par][slot, i, j] = own_rows(vt, i, 1.0)
            if need_q:
                pq_s[par][slot, j] = _phi(qt).astype(BF)
            if need_k:
                pk_s[par][slot, j] = _phi(kt).astype(BF)
                vt_s[par][slot, j] = vt.astype(BF)

        w = [jnp.concatenate([wt_s[c, i, pl.ds(w0, UD), :] for i in range(3)], axis=0)
             for c in range(NC)]
        part = _dot_nt(w[NC - 1], x_v[NC - 1, pl.ds(x0, L), :])
        for j in range(NQ):
            e_s[j] = part[:, j * T:(j + 1) * T]
        for r in range(0, 3 * UD, 24):
            filler.pin(part[r:r + 8, 0:T], amount / (10 * NC))
        yield
        w = jnp.concatenate(w[0:NC - 1], axis=1)
        for j in reversed(range(NQ)):
            rows = pl.ds(pl.multiple_of(x0 + j * T, T), T)
            part = _dot_nt(w, jnp.concatenate([x_v[c, rows, :] for c in range(NC - 1)], axis=1))
            for r in range(0, 3 * UD, 24):
                filler.pin(part[r:r + 8], amount / (10 * NC))
            finish(j, part + e_s[j])
            yield

    HALF = T // 2

    def s_off(j, i, t, n=T):
        return pl.ds((2 * j * (j + 1) + i * (j + 1) + t) * T, n)

    def hi_off(j, pr):
        return pl.ds((2 * j * (j + 1) + 2 * pr * (j + 1) + j) * T + HALF, HALF)

    def col_max(x):
        return jnp.max(x.reshape(x.shape[0] // 8, 8, T), axis=0)

    def scores(j, t, top, amount):
        rq = jnp.concatenate([rq_s[j, i] for i in range(UH)], axis=1)
        n = T if t < j else HALF
        sc = _dot(kn_s[t * T:t * T + n, :], rq)
        if t == j:
            rh = jnp.concatenate([rq_s[j, UH + pr] for pr in range(2)], axis=1)
            hi = _dot(kn_s[t * T + HALF:(t + 1) * T, :], rh)
        for i in range(UH):
            si = sc[:, i * T:(i + 1) * T]
            if t == j:
                si = si + bias_s[i % 2]
            s_s[s_off(j, i, t, n), :] = si
            if i == 0:
                for r in range(0, n, 32):
                    filler.pin(si[r:r + 8], amount * 32 / n)
            top[i] = col_max(si) if t == 0 else jnp.maximum(top[i], col_max(si))
        if t < j:
            return
        left = _iota((8, T), 1) < HALF
        for pr in range(2):
            si = hi[:, pr * T:(pr + 1) * T] + bias_s[2]
            s_s[hi_off(j, pr), :] = si
            mh = col_max(si)
            ma = jnp.maximum(top[2 * pr], jnp.where(left, -jnp.inf, mh))
            mb = jnp.maximum(top[2 * pr + 1], jnp.where(left, mh, -jnp.inf))
            ma = jnp.broadcast_to(jnp.max(ma, axis=0, keepdims=True), (8, T))
            mb = jnp.broadcast_to(jnp.max(mb, axis=0, keepdims=True), (8, T))
            m_s[j, 2 * pr] = ma
            m_s[j, 2 * pr + 1] = mb
            m_s[j, UH + pr] = jnp.where(left, mb, ma)

    def weights(rows, j, i):
        sc = s_s[rows, :]
        m = jnp.concatenate([m_s[j, i]] * (sc.shape[0] // 8), axis=0)
        return jnp.exp2(sc - m).astype(BF)

    def softmax(par, j, t):
        n = T if t < j else HALF
        for i in range(UH):
            p_s[par][s_off(j, i, t, n), :] = weights(s_off(j, i, t, n), j, i)
        if t < j:
            return
        left = _iota((HALF // 2, T), 1) < HALF
        none = jnp.zeros((HALF // 2, T), jnp.uint32)
        for pr in range(2):
            p = pltpu.bitcast(weights(hi_off(j, pr), j, UH + pr), jnp.uint32)
            for i, part in ((2 * pr, jnp.where(left, none, p)), (2 * pr + 1, jnp.where(left, p, none))):
                p_s[par][pl.ds(s_off(j, i, t).start + HALF, HALF), :] = pltpu.bitcast(part, BF)

    def spread(a, b):
        low4 = _iota(a.shape, 0) < 4
        ar, br = pltpu.roll(a, 4, 0), pltpu.roll(b, 4, 0)
        r0, r1 = jnp.where(low4, a, ar), jnp.where(low4, ar, a)
        r2, r3 = jnp.where(low4, b, br), jnp.where(low4, br, b)
        return jnp.concatenate([r0, r0, a, r1, r1, r2, r2, b, r3, r3], axis=0)

    def retrieve(n, par):
        u, slot = n % NU, (n // 2) % 2
        zpad = jnp.zeros((T - UD, T), BF)
        pq = jnp.concatenate(
            [jnp.concatenate([pq_s[par][slot, j], zpad], axis=0) for j in range(NQ)], axis=1)
        ret = _dot(meml_s[u], pq)
        rd = 1.0 / (ret[UD:UD + 16] + 1e-6)
        ret_s[...] = ret[0:UD] * spread(rd[0:8], rd[8:16])

    def update(n, par, s):
        u, slot = n % NU, (n // 2) % 2
        zpad = jnp.zeros((T - UD, T), BF)
        va = jnp.concatenate(
            [jnp.concatenate([vt_s[par][slot, j], jnp.ones((16, T), BF)], axis=0) for j in range(NQ)],
            axis=1)
        pk = jnp.concatenate(
            [jnp.concatenate([pk_s[par][slot, j], zpad], axis=0) for j in range(NQ)], axis=1)
        mem = _dot_nt(va, pk)
        if s > 0:
            mem = mem_s[u] + mem
        if s < NSEG - 2:
            mem_s[u] = mem
        row = _iota((UD + 16, T), 0)
        row_head = jnp.where(row < UD, _head_of(row), (row - UD) >> 2)
        meml_s[u] = jnp.where(row_head == _head_of(_iota((UD + 16, T), 1)), mem, 0.0).astype(BF)

    def values(n, par, s, j, t, acc):
        u, slot = n % NU, (n // 2) % 2
        for i in range(UH):
            part = _dot(va_s[par][slot, i, t], p_s[par][s_off(j, i, t), :])
            acc[i] = part if t == 0 else acc[i] + part
        if t < j:
            return
        heads = []
        for i in range(UH):
            den = acc[i][24:32] if i < 2 else acc[i][0:8]
            val = acc[i][0:24] if i < 2 else acc[i][8:32]
            val = val * jnp.concatenate([1.0 / den] * 3, axis=0)
            heads.append(pltpu.roll(val, HALF, 1) if i % 2 else val)
        low4 = _iota((8, T), 0) < 4
        att = jnp.concatenate([
            heads[0][0:16], jnp.where(low4, heads[0][16:24], heads[1][0:8]), heads[1][8:24],
            heads[2][0:16], jnp.where(low4, heads[2][16:24], heads[3][0:8]), heads[3][8:24]], axis=0)
        rows = pl.ds(pl.multiple_of(u * UD, 16), UD)
        gt = gate_s[rows, :]
        o = (1.0 - gt) * att
        if s > 0:
            o = o + gt * ret_s[:, j * T:(j + 1) * T]
        o = o.astype(BF)
        ot_s[s % 2][j, rows, :] = o

    ORDERS = [
        ENV('ORD0', 'Q30 V30 V31 P Q31 X V32 Q32 Q33 V33 X V20 P Q20 Q21 U X V21 Q22 V22 P Q10 V10 X Q11 V11 P Q00 P V00 X / P Q30 X V30 V31 Q31 Q32 V32 Q33 P V33 V20 X Q20 Q21 U V21 X Q22 P V22 Q10 V10 X Q11 P V11 Q00 V00 P X'),
        ENV('ORD1', 'R V30 P Q30 Q31 V31 Q32 V32 Q33 V33 P U Q20 V20 O Q21 V21 Q22 V22 P O Q10 V10 Q11 O V11 Q00 V00 P P / V30 P R Q30 Q31 V31 Q32 V32 Q33 V33 P U Q20 V20 Q21 V21 Q22 V22 P Q10 V10 Q11 P Q00 P V11 V00 O O O'),
        ENV('ORD1', 'R V30 P Q30 Q31 V31 Q32 V32 Q33 V33 P U Q20 V20 O Q21 V21 Q22 V22 P O Q10 V10 Q11 O V11 Q00 V00 P P / V30 P R Q30 Q31 V31 Q32 V32 Q33 V33 P U Q20 V20 Q21 V21 Q22 V22 P Q10 V10 Q11 P Q00 P V11 V00 O O O'),
        ENV('ORD3', 'R P Q30 V30 Q31 V31 X V32 Q32 Q33 V33 P X Q20 V20 Q21 V21 X Q22 V22 P Q10 V10 Q11 X V11 O P Q00 P V00 / P Q30 V30 Q31 R V31 X V32 Q32 Q33 V33 P X Q20 V20 Q21 V21 X V22 Q22 Q10 V10 Q11 V11 X P P Q00 P O O O V00 O O'),
    ]
    ORDERS = [[half.split() for half in order.split('/')] for order in ORDERS]
    SHARE = [[float(v) for v in ENV(k, d).split(',')] for k, d in
             (('SH0', '0.4,0.6,0'), ('SH1', '0.15,0.55,0.3'), ('SH1', '0.15,0.55,0.3'), ('SH3', '0.25,0.15,0.6'))]

    def step(n, par, s, order, total, jobs=(), oproj=None, stages='PQSV', need_q=True):
        jobs = list(jobs)
        share = SHARE[s]
        proj = project(n + 3, 1 - par, total * share[1], need_q=need_q, need_k=s < NSEG - 1)
        top, acc = [None] * UH, {}
        for tok in order:
            if tok[0] == 'Q':
                j, t = int(tok[1]), int(tok[2])
                if 'S' in stages:
                    softmax(1 - par, j, t)
                if 'Q' in stages:
                    scores(j, t, top, total * share[0] / 10)
            elif tok[0] == 'V':
                if 'V' in stages:
                    values(n, par, s, int(tok[1]), int(tok[2]), acc.setdefault(tok[1], [None] * UH))
            elif tok == 'P':
                if 'P' in stages:
                    next(proj)
            elif tok == 'R':
                if 'V' in stages and s > 0:
                    retrieve(n, par)
            elif tok == 'U':
                if 'V' in stages and s < NSEG - 1:
                    update(n, par, s)
            elif tok == 'O':
                if oproj is not None:
                    next(oproj)
            elif tok == 'X':
                if jobs:
                    jobs.pop(0)()
        assert not jobs

    def out_tiles(s, j):
        return [ot_s[s % 2][j, c * T:(c + 1) * T, :].T for c in range(NC)]

    def pair_step(s, j, stages=('PQSV', 'PQSV'), between=lambda half: None):
        us = (2 * j, 2 * j + 1)
        stream, total, oproj = None, 0, None
        if s == 0:
            total = 8 * NC
        elif 'nomac' not in OPT:
            tiles = (2 * (s - 1), 2 * s - 1) if s < NSEG - 1 else (NC - 1,)
            total = 72 * 2 * len(tiles)
            stream = conv_mac([(c, 2 * u + r) for u in us for c in tiles for r in range(2)], int(ENV('W', '2')))
        filler.gen, filler.credit, filler.in_k = stream, 0.0, s == 0
        if s > 0:
            rows = pl.ds(pl.multiple_of((s - 1) * L + j * T, T), T)
            oproj = out_proj(out_tiles(s - 1, j), rows, 2 * total * SHARE[s][2])
        for half, u in enumerate(us):
            jobs = []
            if s == 0:
                between(half)
                filler.drain()
                filler.gen, filler.credit = gate_kv(u + 1, 1 - half), 0.0
                jobs = [lambda c=c, u=u, half=half: conv_forward(u, half, c) for c in range(NC)]
            elif s == NSEG - 1:
                jobs = [lambda c=c, u=u: conv_inverse(u, c) for c in range(NC - 1)]
            step(s * NU + u, half, s, ORDERS[s][half], total, jobs, oproj, stages[half])
        filler.drain()

    def transpose_weights(t):
        for i in range(3):
            for c in range(NC):
                wt_s[c, i, t * T:(t + 1) * T, :] = w_v[i, t, c * T:(c + 1) * T, :].T

    d_row = d_ref[...].astype(F32).reshape(1, D)

    if ONLY:
        for k in range(NB):
            zero_s[k] = 0
        with jax.named_scope('loop'):
            lax.fori_loop(0, NQ, lambda j, _: pair_step(int(ONLY), j), None)

        def fin(i, _):
            z = (y_s[i, i, 0:16, :].astype(F32) + yl_s[i, 0:16, :] + ot0_s[i, 0:16, :] + ot1_s[i, 0:16, :] + mem_s[i, 0:16, :]
                 + xg_s[i, i, 0:16, :] + meml_s[i, 0:16, :] + kv_s[0, i, 0:16, :] + p0_s[pl.ds(i * 16, 16), :] + p1_s[pl.ds(i * 16, 16), :] + s_s[pl.ds(i * 16, 16), :])
            for tag, fn in dict(aq=lambda: q_v[0:16, 0:T], ak=lambda: k_v[0:16, 0:T], av=lambda: v_v[0:16, 0:T], ah=lambda: h_v[i, 0:16, 0:T],
                                aw=lambda: w_v[0, i, 0:16, :], ad=lambda: dft_s[i, 0:16, :], af=lambda: kf_s[0, 0, 0:1, :], ag=lambda: gate_s[0:16, :],
                                a1=lambda: shift_ref[0:1, 0:T].astype(F32), a2=lambda: dft_ref[i, 0:16, :],
                                a3=lambda: beta_ref[0:1].astype(F32).reshape(1, 1)).items():
                if tag in OPT.split(',') or 'alive' in OPT:
                    z = z + fn()
            outa_s[0:16, 0:T] = z.astype(BF)
            cp = pltpu.make_async_copy(outa_s, out_hbm.at[:, pl.ds(0, D)], sem_q); cp.start(); cp.wait()
            cp = pltpu.make_async_copy(outb_s, out_hbm.at[:, pl.ds(D, D)], sem_q); cp.start(); cp.wait()
        lax.fori_loop(0, 4, fin, None)
        return

    for i in range(3):
        w_copy(i, 0).start()
    for c in range(NC):
        x_copy(0, c).start()

    sc_setup = jax.named_scope('setup')
    sc_setup.__enter__()
    g = jax.nn.sigmoid(beta_ref[...].astype(F32).reshape(1, H))
    rr = _iota((D, H), 0)
    hh = _iota((D, H), 1) * DH
    gate = jnp.sum(jnp.where((rr >= hh) & (rr < hh + DH), g, 0.0), axis=1, keepdims=True)
    gate_s[...] = jnp.broadcast_to(gate, (D, T))
    key, lane = _iota((T // 2, T), 0), _iota((T // 2, T), 1)
    for b, query in enumerate((lane, lane ^ (T // 2), lane & (T // 2 - 1))):
        bias_s[b] = jnp.where(key > query, -1e9 * LOG2E, 0.0).astype(F32)
    rq_s[...] = jnp.zeros(rq_s.shape, BF)
    dft_s[...] = dft_ref[...]
    kf_s[...] = jnp.zeros(kf_s.shape, F32)
    for k in range(NB):
        zero_s[k] = 0

    sc_setup.__exit__(None, None, None)
    with jax.named_scope("w0"):
        for i in range(3):
            w_copy(i, 0).wait()
        for i in range(3):
            w_copy(i, 1).start()
    with jax.named_scope("t0"):
        transpose_weights(0)
    with jax.named_scope("x0"):
        for c in range(NC):
            x_copy(0, c).wait()
        for i in range(3):
            w_copy(i, 2).start()
    with jax.named_scope("p0"):
        for _ in project(0, 0, 0, need_q=False):
            pass
    with jax.named_scope("w1"):
        for i in range(3):
            w_copy(i, 1).wait()
        for t in range(3, NC):
            for i in range(3):
                w_copy(i, t).start()
        for cp in kv_copies(0):
            cp.start()
    with jax.named_scope("p1"):
        transpose_weights(1)
        step(-2, 0, 0, ORDERS[0][0], 0, stages='PQ', need_q=False)
    with jax.named_scope("w2"):
        for t in range(2, NC):
            for i in range(3):
                w_copy(i, t).wait()
        for cp in kv_copies(0):
            cp.wait()
        h_copy(0).start()
        for cp in kv_copies(1):
            cp.start()
    with jax.named_scope("p2"):
        for t in range(2, NC):
            transpose_weights(t)
        step(-1, 1, 0, ORDERS[0][0], 0, stages='PQS', need_q=False)
        for _ in gate_kv(0, 0):
            pass
    h_copy(1).start()
    for cp in kv_copies(2):
        cp.start()

    def seg0(j, _):
        @pl.when(j < NQ - 1)
        def _():
            for u in (2 * j + 2, 2 * j + 3):
                h_copy(u).start()
                for cp in kv_copies(u + 1):
                    cp.start()

        @pl.when(j == NQ - 3)
        def _():
            for c in range(NC):
                x_copy(1, c).start()

        @pl.when(j == NQ - 2)
        def _():
            for c in range(NC):
                x_copy(1, c).wait()
            for c in range(NC):
                wo_copy(c).start()

        @pl.when(j == NQ - 1)
        def _():
            for s in range(2, NSEG):
                for c in range(NC):
                    x_copy(s, c).start()
            q_copy().start()

        def arrive(u):
            h_copy(u).wait()
            for cp in kv_copies(u + 1):
                cp.wait()

        if 'topwait' in OPT:
            arrive(2 * j)
            arrive(2 * j + 1)
            pair_step(0, j)
        else:
            pair_step(0, j, between=lambda half: arrive(2 * j + half))
    with jax.named_scope("seg0"):
        lax.fori_loop(0, NQ, seg0, None)

    for n in range(NC):
        wo_copy(n).wait()

    for s in (1, 2):
        for c in range(NC):
            x_copy(s + 1, c).wait()
        with jax.named_scope(f"seg{s}"):
            lax.fori_loop(0, NQ, lambda j, _, s=s: pair_step(s, j), None)
        ob_copy(pl.ds((s - 1) * L, L)).start()

    q_copy().wait()

    first = pl.ds(0, (NC - 1) * T)
    with jax.named_scope("seg3"):
        lax.fori_loop(0, NQ - 2, lambda j, _: pair_step(3, j), None)
        pair_step(3, NQ - 2, stages=('PQSV', 'QSV'))
    oa_copy(pl.ds(0, S - L), first).start()
    ob_copy(pl.ds(2 * L, L - T)).start()
    with jax.named_scope("seg3e"):
        pair_step(3, NQ - 1, stages=('SV', 'V'))
    oa_copy(pl.ds(S - L, L), first).start()
    ob_copy(pl.ds(3 * L - T, T)).start()

    with jax.named_scope("tail"):
        for u in range(NB):
            conv_inverse(u, NC - 1)
        oa_copy(pl.ds(0, S), pl.ds((NC - 1) * T, T)).start()
        for j in range(NQ):
            rows = pl.ds((NSEG - 1) * L + j * T, T)
            for _ in out_proj(out_tiles(NSEG - 1, j), rows, 0):
                pass
            ob_copy(rows).start()

    oa_copy(pl.ds(0, S), pl.ds(0, D)).wait()
    ob_copy(pl.ds(0, S)).wait()


@jax.jit
def pallas_concat_heads__ssm_conv_h3__memory_aug_infini_attn__prompt_kernel(
    A_q, A_k, A_v, A_shift_k, A_ssm_k, A_ssm_D, B_x, B_wq, B_wk, B_wv, B_wo, B_beta,
):
    hbm = pl.BlockSpec(memory_space=pl.ANY)
    vmem = pl.BlockSpec(memory_space=pltpu.VMEM)
    dma = pltpu.SemaphoreType.DMA
    out = pl.pallas_call(
        _kernel,
        out_shape=jax.ShapeDtypeStruct((S, 2 * D), BF),
        in_specs=[hbm, hbm, hbm, vmem, hbm, vmem, hbm, hbm, hbm, hbm, hbm, vmem, vmem],
        out_specs=hbm,
        scratch_shapes=[
            pltpu.VMEM((S, D), BF),
            pltpu.VMEM((S + CB + 64, D), BF),
            pltpu.VMEM((S + CB, D), BF),
            pltpu.VMEM((NU, D, 2 * T), BF),
            pltpu.VMEM((NC, S, T), BF),
            pltpu.VMEM((3, NC, D, T), BF),
            pltpu.VMEM((NC, D, T), BF),
            pltpu.VMEM((NC, 3, D, T), BF),
            pltpu.VMEM((6, CB, T), BF),
            pltpu.VMEM((NC + 1, 2, 8, T), F32),
            pltpu.VMEM((2, NC, CB, T), BF),
            pltpu.VMEM((2 * NC + 1, NB, 2 * CB, T), F32),
            pltpu.VMEM((NC - 1, NB, 2 * CB, T), BF),
            pltpu.VMEM((NB, 2 * CB, T), BF),
            pltpu.VMEM((S, D), BF),
            pltpu.VMEM((S, D), BF),
            pltpu.VMEM((NQ, D, T), BF),
            pltpu.VMEM((NQ, D, T), BF),
            pltpu.VMEM((NU, UD + 16, T), F32),
            pltpu.VMEM((NU, UD + 16, T), BF),
            pltpu.VMEM((D, T), F32),
            pltpu.VMEM((3, T // 2, T), F32),
            pltpu.VMEM((L, T), BF),
            pltpu.VMEM((NQ, UH + 2, T, T), BF),
            *[pltpu.VMEM((2, NQ, UD, T), BF)] * 6,
            *[pltpu.VMEM((2, UH, NQ, 32, T), BF)] * 2,
            pltpu.VMEM((40 * T, T), F32),
            *[pltpu.VMEM((40 * T, T), BF)] * 2,
            pltpu.VMEM((NQ, UH + 2, 8, T), F32),
            pltpu.VMEM((UD, L), F32),
            pltpu.VMEM((NQ, 3 * UD, T), F32),
            pltpu.SMEM((NB,), jnp.int32),
            dma((4 * NC,)), dma((NSEG * NC,)), dma((3 * (NB + 1),)), dma(()),
            dma(()), dma(()),
        ],
        compiler_params=pltpu.CompilerParams(
            vmem_limit_bytes=100 * 1024 * 1024,
            flags=({'XLA_TPU_EVENLY_DISTRIBUTE_CRITICAL_NODES': True} if 'EV' in OPT else None)),
        name="h3_infini",
    )(A_q.reshape(S, D), A_k.reshape(S, D), A_v.reshape(S, D), A_shift_k.T, A_ssm_k, A_ssm_D,
      B_x.reshape(S, D), B_wq, B_wk, B_wv, B_wo, B_beta, _DFT)
    return out.reshape(1, S, 2 * D)
```

```python
import math, os

import numpy as np
import jax
import jax.numpy as jnp
from jax import lax
from jax.experimental import pallas as pl
from jax.experimental.pallas import tpu as pltpu

OPT = os.environ.get('OPT', '')
ONLY = os.environ.get('ONLY', '')
ENV = os.environ.get

S, D = 2048, 640
H, DH, NSEG, L = 32, 20, 4, 512
T = 128
NC = D // T
CB = 2 * T
NB = S // CB
NF = T // 8
NQ = L // T
UH = 4
UD = UH * DH
NU = H // UH
UR = L // NU
WPAIR = 192
BF, F32 = jnp.bfloat16, jnp.float32
LOG2E = math.log2(math.e)


def _dft_matrices():
    m = np.arange(T)[:, None]
    r = np.arange(T)[None, :]

    def rows(power):
        ang = np.pi * np.mod((4 * m + 1) * power, 1024) / 512
        f = np.stack([np.cos(ang).reshape(NF, 8, T), -np.sin(ang).reshape(NF, 8, T)], 1)
        return f.reshape(2 * T, T)

    even, odd = rows(2 * r), rows(2 * r + 1)
    lane = np.arange(T)
    even_h = even[:, lane // 2 + (T // 2) * (lane % 2)]
    odd_h = odd[:, lane // 2 + (T // 2) * (1 - lane % 2)]
    inverse = [np.concatenate([f[:T].T, f[T:].T]) / (2 * T) for f in (even, odd)]
    return np.stack([even, odd, even_h, odd_h] + inverse).astype(np.float32).astype(BF)


_DFT = _dft_matrices()


def _halves(x):
    w = pltpu.bitcast(x, jnp.uint32)
    return (lax.bitcast_convert_type(w << 16, F32),
            lax.bitcast_convert_type(w & np.uint32(0xFFFF0000), F32))


def _interleave(even, odd):
    e, o = (lax.bitcast_convert_type(v.astype(BF).astype(F32), jnp.uint32) for v in (even, odd))
    return pltpu.bitcast((e >> 16) | o, BF)


def _dot(a, b):
    return jnp.dot(a, b, preferred_element_type=F32)


def _dot_nt(a, b):
    return lax.dot_general(a, b, (((1,), (1,)), ((), ())), preferred_element_type=F32)


def _phi(t):
    return jnp.where(t > 0, t + 1.0, jnp.exp(t))


def _iota(shape, dim):
    return lax.broadcasted_iota(jnp.int32, shape, dim)


def _head_of(z):
    return sum((z >= DH * i).astype(jnp.int32) for i in range(1, UH))


def _kernel(q_hbm, k_hbm, v_hbm, shift_hbm, h_hbm, d_hbm, x_hbm, wq_hbm, wk_hbm, wv_hbm,
            wo_hbm, beta_hbm, dft_hbm, out_hbm,
            q_v, k_v, v_v, h_v, x_v, w_v, wo_v, wt_s, dft_s, kf_s, kv_s, xg_s, y_s, yl_s,
            outa_s, outb_s, ot0_s, ot1_s, mem_s, meml_s, gate_s, bias_s,
            kn_s, rq_s, pk0_s, pk1_s, pq0_s, pq1_s, vt0_s, vt1_s, va0_s, va1_s, s_s, p0_s, p1_s, m_s, ret_s, e_s, shift_ref, d_ref, beta_ref, zero_s,
            sem_w, sem_x, sem_a, sem_q, sem_c, sem_oa, sem_ob):
    ot_s = (ot0_s, ot1_s)
    pk_s, pq_s, vt_s = (pk0_s, pk1_s), (pq0_s, pq1_s), (vt0_s, vt1_s)
    va_s, p_s = (va0_s, va1_s), (p0_s, p1_s)

    def y_of(c):
        return yl_s if c == NC - 1 else y_s.at[c]

    def w_copy(i, t):
        cols = pl.ds(t * T, T)
        return pltpu.make_async_copy((wq_hbm, wk_hbm, wv_hbm)[i].at[:, cols], w_v.at[i, t],
                                     sem_w.at[i * NC + t])

    def wo_copy(n):
        return pltpu.make_async_copy(wo_hbm.at[:, pl.ds(n * T, T)], wo_v.at[n],
                                     sem_w.at[3 * NC + n])

    def x_copy(c, first, count):
        rows = pl.ds(first * L, count * L)
        return pltpu.make_async_copy(x_hbm.at[rows, pl.ds(c * T, T)], x_v.at[c, rows],
                                     sem_x.at[first * NC + c])

    def conv_copies(j):
        src = pl.ds(pl.multiple_of(jnp.minimum(j, NQ - 1) * L, L), L)
        dst = pl.ds(pl.multiple_of(j * L, L), L)
        return (pltpu.make_async_copy(k_hbm.at[src], k_v.at[dst], sem_a.at[3 * j]),
                pltpu.make_async_copy(v_hbm.at[src], v_v.at[dst], sem_a.at[3 * j + 1]),
                pltpu.make_async_copy(h_hbm.at[:, src], h_v.at[j], sem_a.at[3 * j + 2]))

    def q_copy():
        return pltpu.make_async_copy(q_hbm, q_v, sem_q)

    def const_copy(i):
        src, dst = ((beta_hbm, beta_ref), (shift_hbm, shift_ref), (d_hbm, d_ref),
                    (dft_hbm.at[0:4], dft_s.at[0:4]), (dft_hbm.at[4:6], dft_s.at[4:6]))[i]
        return pltpu.make_async_copy(src, dst, sem_c.at[i])

    def oa_copy(rows, lanes):
        return pltpu.make_async_copy(outa_s.at[rows, lanes], out_hbm.at[rows, lanes], sem_oa)

    def ob_copy(rows):
        return pltpu.make_async_copy(outb_s.at[rows], out_hbm.at[rows, pl.ds(D, D)], sem_ob)

    self_done = []

    def gate_kv(u, half):
        src = pl.multiple_of(u * CB, CB)
        for c in range(NC):
            lanes = slice(c * T, (c + 1) * T)
            taps = [shift_ref[t:t + 1, lanes].astype(F32) for t in range(4)]
            pe, po = kf_s[c, 0], kf_s[c, 1]
            for r in range(0, T, 16):
                rows = pl.ds(pl.multiple_of(src + 2 * r, 32), 32)
                ke, ko = _halves(k_v[rows, lanes])
                ve, vo = _halves(v_v[rows, lanes])
                e1 = pltpu.roll(jnp.concatenate([pe, ke], axis=0), 1, 0)[8:24]
                odd = jnp.concatenate([po, ko], axis=0)
                o1, o2 = pltpu.roll(odd, 1, 0)[8:24], pltpu.roll(odd, 2, 0)[8:24]
                se = ke * taps[0] + o1 * taps[1] + e1 * taps[2] + o2 * taps[3]
                so = ko * taps[0] + ke * taps[1] + o1 * taps[2] + e1 * taps[3]
                kv_s[half, c, r:r + 16, :] = (se * ve).astype(BF)
                kv_s[half, c, T + r:T + r + 16, :] = (so * vo).astype(BF)
                pe, po = ke[8:16], ko[8:16]
                yield 1
            kf_s[c, 0] = pe
            kf_s[c, 1] = po
            self_done.append((half, c))

    def conv_forward(u, half, c):
        lanes = slice(c * T, (c + 1) * T)
        h0, h1 = (pltpu.bitcast(h_v[u // 2, lanes, (2 * half + j) * T:(2 * half + j + 1) * T], jnp.uint32)
                  for j in range(2))
        even = (_iota(h0.shape, 1) & 1) == 0
        he = pltpu.bitcast(jnp.where(even, h0, pltpu.roll(h1, 1, 1)), BF)
        ho = pltpu.bitcast(jnp.where(even, pltpu.roll(h1, T - 1, 1), h0), BF)
        for base, a, b in (
                (c, _dot(dft_s[0], kv_s[half, c, 0:T, :]), _dot(dft_s[1], kv_s[half, c, T:CB, :])),
                (NC + c, _dot_nt(dft_s[2], he), _dot_nt(dft_s[3], ho))):
            xg_s[base, u, 0:CB, :] = a + b
            xg_s[base, u, CB:2 * CB, :] = a - b

    def conv_mac(items, w=2):
        skip = {c: jnp.broadcast_to(d_row(c), (8, T)) for c, _ in items}
        for c, f in items:
            for k in range(NB // w):
                outs = range(k * w, (k + 1) * w)
                r0 = pl.multiple_of((f + zero_s[k]) * 16, 16)
                plus = {}
                for sign in range(2):
                    re = pl.ds(pl.multiple_of(r0 + sign * CB, 8), 8)
                    im = pl.ds(pl.multiple_of(r0 + sign * CB + 8, 8), 8)
                    acc, g, h = {}, {}, {}

                    def filt(n):
                        if n not in g:
                            for m in (n, n - 1):
                                if m >= 0 and m not in h:
                                    h[m] = (xg_s[NC + c, m, re, :], xg_s[NC + c, m, im, :])
                            if n == 0:
                                g[n] = (h[0][0] + skip[c], h[0][1])
                            else:
                                g[n] = (h[n][0] - h[n - 1][1], h[n][1] + h[n - 1][0])
                        return g[n]

                    for b in range(max(outs) + 1):
                        xr, xi = xg_s[c, b, re, :], xg_s[c, b, im, :]
                        cost = 0
                        for a in outs:
                            if b > a:
                                continue
                            gr, gi = filt(a - b)
                            p = (xr * gr - xi * gi, xr * gi + xi * gr)
                            acc[a] = p if a not in acc else (acc[a][0] + p[0], acc[a][1] + p[1])
                            cost += 1
                            if a == b and sign == 0:
                                plus[a] = jnp.concatenate(acc[a], axis=0)
                            elif a == b:
                                minus = jnp.concatenate(acc[a], axis=0)
                                y_of(c)[a, pl.ds(r0, 16), :] = (plus[a] + minus).astype(BF)
                                y_of(c)[a, pl.ds(pl.multiple_of(r0 + CB, 16), 16), :] = (
                                    plus[a] - minus).astype(BF)
                        yield cost

    class Filler:
        def __init__(self):
            self.gen, self.credit, self.in_k = None, 0.0, False

        def pin(self, value, amount):
            if self.gen is None or amount == 0:
                return
            if self.in_k:
                k_v[S + L:S + L + 16, 0:T] = jnp.concatenate([value, value], axis=0).astype(BF)
            else:
                xg_s[2 * NC, 0, 0:8, :] = value
            self.credit += amount
            while self.gen is not None and self.credit > 0:
                cost = next(self.gen, None)
                if cost is None:
                    self.gen = None
                else:
                    self.credit -= cost

        def drain(self):
            if self.gen is not None:
                for _ in self.gen:
                    pass
            self.gen = None

    filler = Filler()

    def conv_inverse(u, c):
        r0 = pl.multiple_of(u * CB, CB)
        lanes = slice(c * T, (c + 1) * T)
        qs = _halves(q_v[pl.ds(r0, CB), lanes])
        out = []
        for j in range(2):
            inv = jnp.concatenate([dft_s[4 + j, 0:T, :], dft_s[4 + j, T:CB, :]], axis=1)
            y = _dot(inv, y_of(c)[u, j * CB:(j + 1) * CB, :])
            out.append(qs[j] * y)
        outa_s[pl.ds(r0, CB), lanes] = _interleave(*out)

    def out_proj(o, rows, amount):
        m = o[0].shape[0]
        last = NC - 1
        head = jnp.concatenate(o[0:last], axis=1)

        def pin(part):
            for r in range(0, m, 32):
                filler.pin(part[r:r + 8, 0:T], amount * 32 / (6 * m))

        edge = _dot(o[last], jnp.concatenate(
            [wo_v[n, last * T:D, :] for n in range(last)], axis=1))
        pin(edge)
        yield
        corner = _dot(o[last], wo_v[last, last * T:D, :])
        for n in reversed(range(NC)):
            part = _dot(head, wo_v[n, 0:last * T, :])
            pin(part)
            part = part + (corner if n == last else edge[:, n * T:(n + 1) * T])
            outb_s[rows, n * T:(n + 1) * T] = part.astype(BF)
            yield

    def own_rows(x, i, fill):
        low4 = _iota((8, T), 0) < 4
        full = jnp.full((8, T), fill, F32)
        g0 = 5 * (i // 2)
        if i % 2 == 0:
            body = [x[8 * g0:8 * g0 + 16], jnp.where(low4, x[8 * g0 + 16:8 * g0 + 24], fill)]
        else:
            body = [jnp.where(low4, fill, x[8 * g0 + 16:8 * g0 + 24]), x[8 * g0 + 24:8 * g0 + 40]]
        return jnp.concatenate(body + [full] if i < 2 else [full] + body, axis=0).astype(BF)

    def project(n, par, amount, need_q=True, need_k=True):
        s, u = n // NU, n % NU
        w0 = pl.multiple_of((u // 2) * WPAIR, 64) + par * UD
        x0 = pl.multiple_of(s * L, L)
        slot = (n // 2) % 2
        pad = jnp.zeros((T - UD, T), F32)

        def finish(j, qkv):
            cols = slice(j * T, (j + 1) * T)
            qt, kt, vt = qkv[0:UD], qkv[UD:2 * UD], qkv[2 * UD:3 * UD]
            kn_s[cols, :] = jnp.concatenate([kt, pad], axis=0).T.astype(BF)
            qs = qt * (DH ** -0.5 * LOG2E)
            low4 = _iota((8, T), 0) < 4
            left = _iota((8, T), 1) < T // 2
            zero = jnp.zeros((8, T), F32)
            for pr in range(UH // 2):
                qa = [qs[40 * pr + 8 * r:40 * pr + 8 * r + 8] for r in range(3)]
                qb = [pltpu.roll(qs[40 * pr + 8 * r:40 * pr + 8 * r + 8], T // 2, 1) for r in (2, 3, 4)]
                ra = [qa[0], qa[1], jnp.where(low4, qa[2], 0.0)]
                rb = [jnp.where(low4, 0.0, qb[0]), qb[1], qb[2]]
                rh = [jnp.where(left, 0.0, qa[0]), jnp.where(left, 0.0, qa[1]),
                      jnp.where(left, rb[0], ra[2]),
                      jnp.where(left, qb[1], 0.0), jnp.where(left, qb[2], 0.0)]
                for i, rows in ((2 * pr, ra), (2 * pr + 1, rb)):
                    rows = rows + [zero] if pr == 0 else [zero] + rows
                    rq_s[j, i, 16 * i:16 * i + 32, :] = jnp.concatenate(rows, axis=0).astype(BF)
                rows = rh + [zero] if pr == 0 else [zero] + rh
                rq_s[j, UH + pr, 32 * pr:32 * pr + 48, :] = jnp.concatenate(rows, axis=0).astype(BF)
            for i in range(UH):
                va_s[par][slot, i, j] = own_rows(vt, i, 1.0)
            if need_q:
                pq_s[par][slot, j] = _phi(qt).astype(BF)
            if need_k:
                pk_s[par][slot, j] = _phi(kt).astype(BF)
                vt_s[par][slot, j] = vt.astype(BF)

        w = [jnp.concatenate([wt_s[c, i, pl.ds(pl.multiple_of(w0, 16), UD), :] for i in range(3)], axis=0)
             for c in range(NC)]
        part = _dot_nt(w[NC - 1], x_v[NC - 1, pl.ds(x0, L), :])
        for j in range(NQ):
            e_s[j] = part[:, j * T:(j + 1) * T]
        for r in range(0, 3 * UD, 24):
            filler.pin(part[r:r + 8, 0:T], amount / (10 * NC))
        yield
        w = jnp.concatenate(w[0:NC - 1], axis=1)
        for j in reversed(range(NQ)):
            rows = pl.ds(pl.multiple_of(x0 + j * T, T), T)
            part = _dot_nt(w, jnp.concatenate([x_v[c, rows, :] for c in range(NC - 1)], axis=1))
            for r in range(0, 3 * UD, 24):
                filler.pin(part[r:r + 8], amount / (10 * NC))
            finish(j, part + e_s[j])
            yield

    HALF = T // 2

    def s_off(j, i, t, n=T):
        return pl.ds((2 * j * (j + 1) + i * (j + 1) + t) * T, n)

    def hi_off(j, pr):
        return pl.ds((2 * j * (j + 1) + 2 * pr * (j + 1) + j) * T + HALF, HALF)

    def col_max(x):
        return jnp.max(x.reshape(x.shape[0] // 8, 8, T), axis=0)

    def scores(j, t, top, amount):
        rq = jnp.concatenate([rq_s[j, i] for i in range(UH)], axis=1)
        n = T if t < j else HALF
        sc = _dot(kn_s[t * T:t * T + n, :], rq)
        if t == j:
            rh = jnp.concatenate([rq_s[j, UH + pr] for pr in range(2)], axis=1)
            hi = _dot(kn_s[t * T + HALF:(t + 1) * T, :], rh)
        for i in range(UH):
            si = sc[:, i * T:(i + 1) * T]
            if t == j:
                si = si + bias_s[i % 2]
            s_s[s_off(j, i, t, n), :] = si
            if i == 0:
                for r in range(0, n, 32):
                    filler.pin(si[r:r + 8], amount * 32 / n)
            top[i] = col_max(si) if t == 0 else jnp.maximum(top[i], col_max(si))
        if t < j:
            return
        left = _iota((8, T), 1) < HALF
        for pr in range(2):
            si = hi[:, pr * T:(pr + 1) * T] + bias_s[2]
            s_s[hi_off(j, pr), :] = si
            mh = col_max(si)
            ma = jnp.maximum(top[2 * pr], jnp.where(left, -jnp.inf, mh))
            mb = jnp.maximum(top[2 * pr + 1], jnp.where(left, mh, -jnp.inf))
            ma = jnp.broadcast_to(jnp.max(ma, axis=0, keepdims=True), (8, T))
            mb = jnp.broadcast_to(jnp.max(mb, axis=0, keepdims=True), (8, T))
            m_s[j, 2 * pr] = ma
            m_s[j, 2 * pr + 1] = mb
            m_s[j, UH + pr] = jnp.where(left, mb, ma)

    def weights(rows, j, i):
        sc = s_s[rows, :]
        m = jnp.concatenate([m_s[j, i]] * (sc.shape[0] // 8), axis=0)
        return jnp.exp2(sc - m).astype(BF)

    def softmax(par, j, t):
        n = T if t < j else HALF
        for i in range(UH):
            p_s[par][s_off(j, i, t, n), :] = weights(s_off(j, i, t, n), j, i)
        if t < j:
            return
        left = _iota((HALF // 2, T), 1) < HALF
        none = jnp.zeros((HALF // 2, T), jnp.uint32)
        for pr in range(2):
            p = pltpu.bitcast(weights(hi_off(j, pr), j, UH + pr), jnp.uint32)
            for i, part in ((2 * pr, jnp.where(left, none, p)), (2 * pr + 1, jnp.where(left, p, none))):
                p_s[par][pl.ds(s_off(j, i, t).start + HALF, HALF), :] = pltpu.bitcast(part, BF)

    def spread(a, b):
        low4 = _iota(a.shape, 0) < 4
        ar, br = pltpu.roll(a, 4, 0), pltpu.roll(b, 4, 0)
        r0, r1 = jnp.where(low4, a, ar), jnp.where(low4, ar, a)
        r2, r3 = jnp.where(low4, b, br), jnp.where(low4, br, b)
        return jnp.concatenate([r0, r0, a, r1, r1, r2, r2, b, r3, r3], axis=0)

    def retrieve(n, par):
        u, slot = n % NU, (n // 2) % 2
        zpad = jnp.zeros((T - UD, T), BF)
        pq = jnp.concatenate(
            [jnp.concatenate([pq_s[par][slot, j], zpad], axis=0) for j in range(NQ)], axis=1)
        ret = _dot(meml_s[u], pq)
        rd = 1.0 / (ret[UD:UD + 16] + 1e-6)
        ret_s[...] = ret[0:UD] * spread(rd[0:8], rd[8:16])

    def update(n, par, s):
        u, slot = n % NU, (n // 2) % 2
        zpad = jnp.zeros((T - UD, T), BF)
        va = jnp.concatenate(
            [jnp.concatenate([vt_s[par][slot, j], jnp.ones((16, T), BF)], axis=0) for j in range(NQ)],
            axis=1)
        pk = jnp.concatenate(
            [jnp.concatenate([pk_s[par][slot, j], zpad], axis=0) for j in range(NQ)], axis=1)
        mem = _dot_nt(va, pk)
        if s > 0:
            mem = mem_s[u] + mem
        if s < NSEG - 2:
            mem_s[u] = mem
        row = _iota((UD + 16, T), 0)
        row_head = jnp.where(row < UD, _head_of(row), (row - UD) >> 2)
        meml_s[u] = jnp.where(row_head == _head_of(_iota((UD + 16, T), 1)), mem, 0.0).astype(BF)

    def values(n, par, s, j, t, acc):
        u, slot = n % NU, (n // 2) % 2
        for i in range(UH):
            part = _dot(va_s[par][slot, i, t], p_s[par][s_off(j, i, t), :])
            acc[i] = part if t == 0 else acc[i] + part
        if t < j:
            return
        heads = []
        for i in range(UH):
            den = acc[i][24:32] if i < 2 else acc[i][0:8]
            val = acc[i][0:24] if i < 2 else acc[i][8:32]
            val = val * jnp.concatenate([1.0 / den] * 3, axis=0)
            heads.append(pltpu.roll(val, HALF, 1) if i % 2 else val)
        low4 = _iota((8, T), 0) < 4
        att = jnp.concatenate([
            heads[0][0:16], jnp.where(low4, heads[0][16:24], heads[1][0:8]), heads[1][8:24],
            heads[2][0:16], jnp.where(low4, heads[2][16:24], heads[3][0:8]), heads[3][8:24]], axis=0)
        rows = pl.ds(pl.multiple_of(u * UD, 16), UD)
        gt = gate_s[rows, :]
        o = (1.0 - gt) * att
        if s > 0:
            o = o + gt * ret_s[:, j * T:(j + 1) * T]
        o = o.astype(BF)
        ot_s[s % 2][j, rows, :] = o

    ORDERS = [
        ENV('ORD0', 'P Q30 V30 Q31 V31 Q32 V32 Q33 V33 P X U Q20 V20 Q21 V21 Q22 X V22 P Q10 V10 Q11 X V11 P X V00 Q00 P X / P Q30 V30 V31 Q31 X Q32 Q33 V32 V33 X U P Q20 X V20 Q21 V21 Q22 V22 P Q10 V10 X Q11 X V11 P V00 Q00 P'),
        ENV('ORD1', 'R V30 P Q30 Q31 V31 Q32 V32 Q33 V33 P U Q20 V20 O Q21 V21 Q22 V22 P O Q10 V10 Q11 O V11 Q00 V00 P P / V30 P R Q30 Q31 V31 Q32 V32 Q33 V33 P U Q20 V20 Q21 V21 Q22 V22 P Q10 V10 Q11 P Q00 P V11 V00 O O O'),
        ENV('ORD1', 'R V30 P Q30 Q31 V31 Q32 V32 Q33 V33 P U Q20 V20 O Q21 V21 Q22 V22 P O Q10 V10 Q11 O V11 Q00 V00 P P / V30 P R Q30 Q31 V31 Q32 V32 Q33 V33 P U Q20 V20 Q21 V21 Q22 V22 P Q10 V10 Q11 P Q00 P V11 V00 O O O'),
        ENV('ORD3', 'R P Q30 V30 Q31 V31 X V32 Q32 Q33 V33 P X Q20 V20 Q21 V21 X Q22 V22 P Q10 V10 Q11 X V11 O P Q00 P V00 / P Q30 V30 Q31 R V31 X V32 Q32 Q33 V33 P X Q20 V20 Q21 V21 X V22 Q22 Q10 V10 Q11 V11 X P P Q00 P O O O V00 O O'),
    ]
    ORDA = ENV('ORDA', 'R P Q30 V30 V31 Q31 X V32 Q32 Q33 V33 P X Q20 V20 Q21 V21 X Q22 V22 P Q10 V10 Q11 X V11 O P Q00 P V00 / P Q30 V30 Q31 V31 R X V32 Q32 Q33 V33 P X Q20 V20 Q21 O V21 X V22 Q22 Q10 V10 O Q11 V11 X P P Q00 P O V00 O O')
    ORDB = ENV('ORDB', 'X R X Q30 V30 X Q31 V31 X Q32 V32 X Q33 V33 X Q20 V20 X Q21 V21 X Q22 V22 X Q10 V10 X Q11 V11 X Q00 V00 X / X R V30 V31 X V32 V33 X V20 V21 X V22 V10 O V11 V00 O O O O O')
    ORDA, ORDB = ([half.split() for half in order.split('/')] for order in (ORDA, ORDB))
    SHA = [float(v) for v in ENV('SHA', '0.6,0.35,0.05').split(',')]
    PRO1 = ENV('PRO1', 'P Q30 Q31 Q32 Q33 P W Q20 Q21 Q22 P Q10 Q11 P Q00 P')
    PRO = ENV('PRO', 'P Q30 Q31 Q32 Q33 P Q20 Q21 Q22 P Q10 Q11 P Q00 P')
    ORDERS = [[half.split() for half in order.split('/')] for order in ORDERS]
    SHARE = [[float(v) for v in ENV(k, d).split(',')] for k, d in
             (('SH0', '0.65,0.65,0'), ('SH1', '0.15,0.55,0.3'), ('SH1', '0.15,0.55,0.3'), ('SH3', '0.25,0.15,0.6'))]

    def step(n, par, s, order, share, jobs=(), oproj=None, stages='PQSV', need_q=True, arrive=None):
        jobs = list(jobs)
        proj = project(n + 3, 1 - par, share[1], need_q=need_q, need_k=s < NSEG - 1)
        top, acc = [None] * UH, {}
        for tok in order:
            if tok[0] == 'Q':
                j, t = int(tok[1]), int(tok[2])
                if 'S' in stages:
                    softmax(1 - par, j, t)
                if 'Q' in stages:
                    scores(j, t, top, share[0] / 10)
            elif tok[0] == 'V':
                if 'V' in stages:
                    values(n, par, s, int(tok[1]), int(tok[2]), acc.setdefault(tok[1], [None] * UH))
            elif tok == 'P':
                if 'P' in stages:
                    next(proj)
            elif tok == 'R':
                if 'V' in stages and s > 0:
                    retrieve(n, par)
            elif tok == 'U':
                if 'V' in stages and s < NSEG - 1:
                    update(n, par, s)
            elif tok == 'O':
                if oproj is not None:
                    next(oproj)
            elif tok == 'W':
                if arrive is not None:
                    arrive()
            elif tok == 'X':
                if jobs:
                    jobs.pop(0)()
        assert not jobs

    def out_tiles(s, j):
        return [ot_s[s % 2][j, c * T:(c + 1) * T, :].T for c in range(NC)]

    def pair_step(s, j, stages=('PQSV', 'PQSV'), arrive=None, mac=None, inverse=None, middle=None,
                  orders=None, mix=None):
        orders, mix = orders or ORDERS[s], mix or SHARE[s]
        us = (2 * j, 2 * j + 1)
        share, oproj = [8 * NC * v for v in mix], None
        filler.gen, filler.credit, filler.in_k = None, 0.0, s == 0
        if s == 0:
            del self_done[:]
            filler.gen = (cost for half, u in enumerate(us) for cost in gate_kv(u, half))
            share = [16 * NC * v for v in mix]
        else:
            if mac is None:
                mac = [(c, 4 * j + r) for c in (2 * s - 2, 2 * s - 1) for r in range(4)]
            weight = (mix[0] * sum('Q' in st for st in stages)
                      + mix[1] * sum('P' in st for st in stages) + 2 * mix[2])
            share = [72 * len(mac) * v / weight for v in mix]
            if mac and 'nomac' not in OPT:
                filler.gen = conv_mac(mac, int(ENV('W', '2')))
            rows = pl.ds(pl.multiple_of((s - 1) * L + j * T, T), T)
            oproj = out_proj(out_tiles(s - 1, j), rows, 2 * share[2])
        for half, u in enumerate(us):
            jobs, wait = [], None
            if half == 1 and middle is not None:
                middle()
            if s == 0:
                def forward(u, half, c):
                    while (half, c) not in self_done and filler.gen is not None:
                        if next(filler.gen, None) is None:
                            filler.gen = None
                        filler.credit -= 1
                    conv_forward(u, half, c)
                jobs = [lambda c=c, u=u, half=half: forward(u, half, c) for c in range(NC)]
            elif s == NSEG - 1:
                todo = (inverse[half] if inverse else []) + [(u, c) for c in range(NC - 1)]
                jobs = [lambda b=b, c=c: conv_inverse(b, c) for b, c in todo]
            step(s * NU + u, half, s, orders[half],
                 share, jobs, oproj, stages[half], arrive=wait)
        filler.drain()

    def last_mac(j, extra=None):
        return [(NC - 1, f) for f in [4 * j + r for r in range(4)] + (extra or [12 + 2 * j])]

    def scoped(f, s, j):
        with jax.named_scope("it"):
            f(s, j)

    def transpose_weights(t):
        for i in range(3):
            for c in range(NC):
                wt = w_v[i, t, c * T:(c + 1) * T, :].T
                for r in range(T // 16):
                    pair, off = divmod(t * T + 16 * r, 2 * UD)
                    wt_s[c, i, pair * WPAIR + off:pair * WPAIR + off + 16, :] = wt[16 * r:16 * r + 16]

    def d_row(c):
        return d_ref[...].astype(F32).reshape(1, D)[:, c * T:(c + 1) * T]

    def epilogue():
        first = pl.ds(0, (NC - 1) * T)
        with jax.named_scope("seg3a"):
            pair_step(3, NQ - 2, stages=('PQSV', 'QSV'), mac=last_mac(NQ - 2, [13, 15]), orders=ORDA, mix=SHA)
        oa_copy(pl.ds(0, S - L), first).start()
        ob_copy(pl.ds(2 * L, L - T)).start()

        def send_conv():
            oa_copy(pl.ds(0, S), pl.ds((NC - 1) * T, T)).start()
            oa_copy(pl.ds(S - 2 * CB, CB), first).start()
        with jax.named_scope("seg3e"):
            pair_step(3, NQ - 1, stages=('SV', 'V'), mac=[], middle=send_conv, orders=ORDB,
                      inverse=[[(b, NC - 1) for b in range(NB)], []])
        oa_copy(pl.ds(S - CB, CB), first).start()
        ob_copy(pl.ds(3 * L - T, T)).start()

        with jax.named_scope("tail"):
            for j in range(NQ):
                rows = pl.ds((NSEG - 1) * L + j * T, T)
                for _ in out_proj(out_tiles(NSEG - 1, j), rows, 0):
                    pass
                ob_copy(rows).start()

    if ONLY == 'E':
        epilogue()
        return
    if ONLY:
        for k in range(NB):
            zero_s[k] = 0
        with jax.named_scope('loop'):
            lax.fori_loop(0, NQ, lambda j, _: pair_step(int(ONLY), j, mac=last_mac(j) if ONLY == '3' else None), None)

        def fin(i, _):
            z = (y_s[i, i, 0:16, :].astype(F32) + yl_s[i, 0:16, :] + ot0_s[i, 0:16, :] + ot1_s[i, 0:16, :] + mem_s[i, 0:16, :]
                 + xg_s[i, i, 0:16, :] + meml_s[i, 0:16, :] + kv_s[0, i, 0:16, :] + p0_s[pl.ds(i * 16, 16), :] + p1_s[pl.ds(i * 16, 16), :] + s_s[pl.ds(i * 16, 16), :])
            for tag, fn in dict(aq=lambda: q_v[0:16, 0:T], ak=lambda: k_v[0:16, 0:T], av=lambda: v_v[0:16, 0:T], ah=lambda: h_v[i, 0:16, 0:T],
                                aw=lambda: w_v[0, i, 0:16, :], ad=lambda: dft_s[i, 0:16, :], af=lambda: kf_s[0, 0, 0:1, :], ag=lambda: gate_s[0:16, :],
                                a1=lambda: shift_ref[0:1, 0:T].astype(F32), a2=lambda: dft_s[i, 0:16, :],
                                a3=lambda: beta_ref[0:1].astype(F32).reshape(1, 1)).items():
                if tag in OPT.split(',') or 'alive' in OPT:
                    z = z + fn()
            outa_s[0:16, 0:T] = z.astype(BF)
            cp = pltpu.make_async_copy(outa_s, out_hbm.at[:, pl.ds(0, D)], sem_q); cp.start(); cp.wait()
            cp = pltpu.make_async_copy(outb_s, out_hbm.at[:, pl.ds(D, D)], sem_q); cp.start(); cp.wait()
        lax.fori_loop(0, 4, fin, None)
        return

    for i in range(3):
        w_copy(i, 0).start()
    const_copy(0).start()
    with jax.named_scope("setup"):
        for c in range(NC):
            x_copy(c, 0, 1).start()
        rq_s[...] = jnp.zeros(rq_s.shape, BF)
        key, lane = _iota((T // 2, T), 0), _iota((T // 2, T), 1)
        for b, query in enumerate((lane, lane ^ (T // 2), lane & (T // 2 - 1))):
            bias_s[b] = jnp.where(key > query, -1e9 * LOG2E, 0.0).astype(F32)
        kf_s[...] = jnp.zeros(kf_s.shape, F32)
        for k in range(NB):
            zero_s[k] = 0
        const_copy(0).wait()
        g = jax.nn.sigmoid(beta_ref[...].astype(F32).reshape(1, H))
        rr = _iota((D, H), 0)
        hh = _iota((D, H), 1) * DH
        gate = jnp.sum(jnp.where((rr >= hh) & (rr < hh + DH), g, 0.0), axis=1, keepdims=True)
        gate_s[...] = jnp.broadcast_to(gate, (D, T))
    with jax.named_scope("w0"):
        for i in range(3):
            w_copy(i, 0).wait()
        for i in range(3):
            w_copy(i, 1).start()
    with jax.named_scope("t0"):
        transpose_weights(0)
    with jax.named_scope("x0"):
        for c in range(NC):
            x_copy(c, 0, 1).wait()
        for i in range(3):
            w_copy(i, 2).start()
    with jax.named_scope("p0"):
        for _ in project(0, 0, 0, need_q=False):
            pass
    with jax.named_scope("w1"):
        for i in range(3):
            w_copy(i, 1).wait()
        for i in range(3):
            w_copy(i, 3).start()
        const_copy(1).start()
        const_copy(3).start()
    with jax.named_scope("p1"):
        transpose_weights(1)

        def fetch_conv():
            for cp in conv_copies(0):
                cp.start()
        step(-2, 0, 0, PRO1.split(), (0, 0), stages='PQ', need_q=False, arrive=fetch_conv)
    with jax.named_scope("w2"):
        for t in (2, 3):
            for i in range(3):
                w_copy(i, t).wait()
    with jax.named_scope("p2"):
        for t in (2, 3):
            transpose_weights(t)
        step(-1, 1, 0, PRO.split(), (0, 0), stages='PQS', need_q=False)
    with jax.named_scope('aw'):
        const_copy(1).wait()
        const_copy(3).wait()
        for cp in conv_copies(0):
            cp.wait()
    for i in range(3):
        w_copy(i, 4).start()
    for c in range(NC):
        x_copy(c, 1, 1).start()

    def seg0(j, _):
        @pl.when(j == 1)
        def _():
            for i in range(3):
                w_copy(i, 4).wait()
            for c in range(NC):
                x_copy(c, 1, 1).wait()
            for c in range(NC):
                wo_copy(c).start()
            const_copy(2).start()
            transpose_weights(4)

        for cp in conv_copies(j + 1):
            cp.start()
        pair_step(0, j)
        for cp in conv_copies(j + 1):
            cp.wait()
    with jax.named_scope("seg0"):
        lax.fori_loop(0, NQ, seg0, None)

    const_copy(2).wait()
    const_copy(4).start()
    for c in range(NC):
        wo_copy(c).wait()
        x_copy(c, 2, 2).start()

    with jax.named_scope("seg1"):
        lax.fori_loop(0, NQ, lambda j, _: pair_step(1, j), None)
    ob_copy(pl.ds(0, L)).start()
    q_copy().start()
    for c in range(NC):
        x_copy(c, 2, 2).wait()
    with jax.named_scope("seg2"):
        lax.fori_loop(0, NQ, lambda j, _: pair_step(2, j), None)
    ob_copy(pl.ds(L, L)).start()
    q_copy().wait()
    const_copy(4).wait()

    with jax.named_scope("seg3"):
        lax.fori_loop(0, NQ - 2, lambda j, _: pair_step(3, j, mac=last_mac(j)), None)
    epilogue()

    with jax.named_scope('wa'):
        oa_copy(pl.ds(0, S), pl.ds(0, D)).wait()
    with jax.named_scope('wb'):
        ob_copy(pl.ds(0, S)).wait()


@jax.jit
def pallas_concat_heads__ssm_conv_h3__memory_aug_infini_attn__prompt_kernel(
    A_q, A_k, A_v, A_shift_k, A_ssm_k, A_ssm_D, B_x, B_wq, B_wk, B_wv, B_wo, B_beta,
):
    hbm = pl.BlockSpec(memory_space=pl.ANY)
    dma = pltpu.SemaphoreType.DMA
    out = pl.pallas_call(
        _kernel,
        out_shape=jax.ShapeDtypeStruct((S, 2 * D), BF),
        in_specs=[hbm] * 13,
        out_specs=hbm,
        scratch_shapes=[
            pltpu.VMEM((S, D), BF),
            pltpu.VMEM((S + L + 64, D), BF),
            pltpu.VMEM((S + L, D), BF),
            pltpu.VMEM((NQ + 1, D, L), BF),
            pltpu.VMEM((NC, S, T), BF),
            pltpu.VMEM((3, NC, D, T), BF),
            pltpu.VMEM((NC, D, T), BF),
            pltpu.VMEM((NC, 3, NQ * WPAIR, T), BF),
            pltpu.VMEM((6, CB, T), BF),
            pltpu.VMEM((NC + 1, 2, 8, T), F32),
            pltpu.VMEM((2, NC, CB, T), BF),
            pltpu.VMEM((2 * NC + 1, NB, 2 * CB, T), F32),
            pltpu.VMEM((NC - 1, NB, 2 * CB, T), BF),
            pltpu.VMEM((NB, 2 * CB, T), BF),
            pltpu.VMEM((S, D), BF),
            pltpu.VMEM((S, D), BF),
            pltpu.VMEM((NQ, D, T), BF),
            pltpu.VMEM((NQ, D, T), BF),
            pltpu.VMEM((NU, UD + 16, T), F32),
            pltpu.VMEM((NU, UD + 16, T), BF),
            pltpu.VMEM((D, T), F32),
            pltpu.VMEM((3, T // 2, T), F32),
            pltpu.VMEM((L, T), BF),
            pltpu.VMEM((NQ, UH + 2, T, T), BF),
            *[pltpu.VMEM((2, NQ, UD, T), BF)] * 6,
            *[pltpu.VMEM((2, UH, NQ, 32, T), BF)] * 2,
            pltpu.VMEM((40 * T, T), F32),
            *[pltpu.VMEM((40 * T, T), BF)] * 2,
            pltpu.VMEM((NQ, UH + 2, 8, T), F32),
            pltpu.VMEM((UD, L), F32),
            pltpu.VMEM((NQ, 3 * UD, T), F32),
            pltpu.VMEM((4, D), BF),
            pltpu.VMEM((D,), BF),
            pltpu.VMEM((H,), BF),
            pltpu.SMEM((NB,), jnp.int32),
            dma((4 * NC,)), dma((NSEG * NC,)), dma((3 * (NQ + 1),)), dma(()),
            dma((5,)), dma(()), dma(()),
        ],
        compiler_params=pltpu.CompilerParams(
            vmem_limit_bytes=100 * 1024 * 1024,
            flags=({'XLA_TPU_EVENLY_DISTRIBUTE_CRITICAL_NODES': True} if 'EV' in OPT else None)),
        name="h3_infini",
    )(A_q.reshape(S, D), A_k.reshape(S, D), A_v.reshape(S, D), A_shift_k.T, A_ssm_k, A_ssm_D,
      B_x.reshape(S, D), B_wq, B_wk, B_wv, B_wo, B_beta, _DFT)
    return out.reshape(1, S, 2 * D)
```

```python
import math, os

import numpy as np
import jax
import jax.numpy as jnp
from jax import lax
from jax.experimental import pallas as pl
from jax.experimental.pallas import tpu as pltpu

OPT = os.environ.get('OPT', '')
ONLY = os.environ.get('ONLY', '')
ENV = os.environ.get

S, D = 2048, 640
H, DH, NSEG, L = 32, 20, 4, 512
T = 128
NC = D // T
CB = 2 * T
NB = S // CB
NF = T // 8
NQ = L // T
UH = 4
UD = UH * DH
NU = H // UH
UR = L // NU
WPAIR = 192
BF, F32 = jnp.bfloat16, jnp.float32
LOG2E = math.log2(math.e)


def _dft_matrices():
    m = np.arange(T)[:, None]
    r = np.arange(T)[None, :]

    def rows(power):
        ang = np.pi * np.mod((4 * m + 1) * power, 1024) / 512
        f = np.stack([np.cos(ang).reshape(NF, 8, T), -np.sin(ang).reshape(NF, 8, T)], 1)
        return f.reshape(2 * T, T)

    even, odd = rows(2 * r), rows(2 * r + 1)
    lane = np.arange(T)
    even_h = even[:, lane // 2 + (T // 2) * (lane % 2)]
    odd_h = odd[:, lane // 2 + (T // 2) * (1 - lane % 2)]
    inverse = [np.concatenate([f[:T].T, f[T:].T]) / (2 * T) for f in (even, odd)]
    bits = np.stack([even, odd, even_h, odd_h] + inverse).astype(np.float32).astype(BF)
    bits = bits.view(np.uint16).astype(np.uint32)
    return bits[:, 0::2] | (bits[:, 1::2] << 16)


_DFT = _dft_matrices()


def _pack(x):
    return pltpu.bitcast(x, jnp.uint32)


def _unpack(w):
    return pltpu.bitcast(w, BF)


def _halves(x):
    w = pltpu.bitcast(x, jnp.uint32)
    return (lax.bitcast_convert_type(w << 16, F32),
            lax.bitcast_convert_type(w & np.uint32(0xFFFF0000), F32))


def _interleave(even, odd):
    e, o = (lax.bitcast_convert_type(v.astype(BF).astype(F32), jnp.uint32) for v in (even, odd))
    return pltpu.bitcast((e >> 16) | o, BF)


import contextlib


def _scope(name):
    return jax.named_scope(name) if 'scope' in OPT else contextlib.nullcontext()


def _dot(a, b):
    return jnp.dot(a, b, preferred_element_type=F32)


def _dot_nt(a, b):
    return lax.dot_general(a, b, (((1,), (1,)), ((), ())), preferred_element_type=F32)


def _phi(t):
    return jnp.where(t > 0, t + 1.0, jnp.exp(t))


def _iota(shape, dim):
    return lax.broadcasted_iota(jnp.int32, shape, dim)


def _head_of(z):
    return sum((z >= DH * i).astype(jnp.int32) for i in range(1, UH))


def _kernel(q_hbm, k_hbm, v_hbm, shift_hbm, h_hbm, d_hbm, x_hbm, wq_hbm, wk_hbm, wv_hbm,
            wo_hbm, beta_hbm, dft_hbm, out_hbm,
            q_v, k_v, v_v, h_v, x_v, w_v, wo_v, wt_s, dft_s, kf_s, kv_s, xg_s, y_s, yl_s,
            outa_s, outb_s, ot0_s, ot1_s, mem_s, meml_s, gate_s, bias_s,
            kn_s, rq_s, pk0_s, pk1_s, pq0_s, pq1_s, vt0_s, vt1_s, va0_s, va1_s, s_s, p0_s, p1_s, m_s, ret_s, e_s, shift_ref, d_ref, beta_ref, zero_s,
            sem_w, sem_x, sem_a, sem_q, sem_c, sem_oa, sem_ob):
    ot_s = (ot0_s, ot1_s)
    pk_s, pq_s, vt_s = (pk0_s, pk1_s), (pq0_s, pq1_s), (vt0_s, vt1_s)
    va_s, p_s = (va0_s, va1_s), (p0_s, p1_s)

    def y_of(c):
        return yl_s if c == NC - 1 else y_s.at[c]

    def w_copy(i, t):
        cols = pl.ds(t * T, T)
        return pltpu.make_async_copy((wq_hbm, wk_hbm, wv_hbm)[i].at[:, cols], w_v.at[i, t],
                                     sem_w.at[i * NC + t])

    def wo_copy(n):
        return pltpu.make_async_copy(wo_hbm.at[:, pl.ds(n * T, T)], wo_v.at[n],
                                     sem_w.at[3 * NC + n])

    def x_copy(c, first, count):
        rows = pl.ds(first * L, count * L)
        return pltpu.make_async_copy(x_hbm.at[rows, pl.ds(c * T, T)], x_v.at[c, rows],
                                     sem_x.at[first * NC + c])

    def conv_copies(j):
        src = pl.ds(pl.multiple_of(jnp.minimum(j, NQ - 1) * L, L), L)
        dst = pl.ds(pl.multiple_of(j * L, L), L)
        return (pltpu.make_async_copy(k_hbm.at[src], k_v.at[dst], sem_a.at[3 * j]),
                pltpu.make_async_copy(v_hbm.at[src], v_v.at[dst], sem_a.at[3 * j + 1]),
                pltpu.make_async_copy(h_hbm.at[:, src], h_v.at[j], sem_a.at[3 * j + 2]))

    def q_copy():
        return pltpu.make_async_copy(q_hbm, q_v, sem_q)

    def const_copy(i):
        src, dst = ((beta_hbm, beta_ref), (shift_hbm, shift_ref), (d_hbm, d_ref),
                    (dft_hbm.at[0:4], dft_s.at[0:4]), (dft_hbm.at[4:6], dft_s.at[4:6]))[i]
        return pltpu.make_async_copy(src, dst, sem_c.at[i])

    def oa_copy(rows, lanes):
        return pltpu.make_async_copy(outa_s.at[rows, lanes], out_hbm.at[rows, lanes], sem_oa)

    def ob_copy(rows):
        return pltpu.make_async_copy(outb_s.at[rows], out_hbm.at[rows, pl.ds(D, D)], sem_ob)

    self_done = []

    def gate_kv(u, half):
        src = pl.multiple_of(u * CB, CB)
        for c in range(NC):
            lanes = slice(c * T, (c + 1) * T)
            taps = [shift_ref[t:t + 1, lanes].astype(F32) for t in range(4)]
            pe, po = kf_s[c, 0], kf_s[c, 1]
            for r in range(0, T, 16):
                rows = pl.ds(pl.multiple_of(src + 2 * r, 32), 32)
                ke, ko = _halves(k_v[rows, lanes])
                ve, vo = _halves(v_v[rows, lanes])
                e1 = pltpu.roll(jnp.concatenate([pe, ke], axis=0), 1, 0)[8:24]
                odd = jnp.concatenate([po, ko], axis=0)
                o1, o2 = pltpu.roll(odd, 1, 0)[8:24], pltpu.roll(odd, 2, 0)[8:24]
                se = ke * taps[0] + o1 * taps[1] + e1 * taps[2] + o2 * taps[3]
                so = ko * taps[0] + ke * taps[1] + o1 * taps[2] + e1 * taps[3]
                kv_s[half, c, r:r + 16, :] = (se * ve).astype(BF)
                kv_s[half, c, T + r:T + r + 16, :] = (so * vo).astype(BF)
                pe, po = ke[8:16], ko[8:16]
                yield 1
            kf_s[c, 0] = pe
            kf_s[c, 1] = po
            self_done.append((half, c))

    def conv_forward(u, half, c):
        lanes = slice(c * T, (c + 1) * T)
        h0, h1 = (pltpu.bitcast(h_v[u // 2, lanes, (2 * half + j) * T:(2 * half + j + 1) * T], jnp.uint32)
                  for j in range(2))
        even = (_iota(h0.shape, 1) & 1) == 0
        he = pltpu.bitcast(jnp.where(even, h0, pltpu.roll(h1, 1, 1)), BF)
        ho = pltpu.bitcast(jnp.where(even, pltpu.roll(h1, T - 1, 1), h0), BF)
        for base, a, b in (
                (c, _dot(_unpack(dft_s[0]), kv_s[half, c, 0:T, :]),
                 _dot(_unpack(dft_s[1]), kv_s[half, c, T:CB, :])),
                (NC + c, _dot_nt(_unpack(dft_s[2]), he), _dot_nt(_unpack(dft_s[3]), ho))):
            xg_s[base, u, 0:CB, :] = a + b
            xg_s[base, u, CB:2 * CB, :] = a - b

    def conv_mac(items, w=2):
        skip = {c: jnp.broadcast_to(d_row(c), (8, T)) for c, _ in items}
        for c, f in items:
            for k in range(NB // w):
                outs = range(k * w, (k + 1) * w)
                r0 = pl.multiple_of((f + zero_s[k]) * 16, 16)
                plus = {}
                for sign in range(2):
                    re = pl.ds(pl.multiple_of(r0 + sign * CB, 8), 8)
                    im = pl.ds(pl.multiple_of(r0 + sign * CB + 8, 8), 8)
                    acc, g, h = {}, {}, {}

                    def filt(n):
                        if n not in g:
                            for m in (n, n - 1):
                                if m >= 0 and m not in h:
                                    h[m] = (xg_s[NC + c, m, re, :], xg_s[NC + c, m, im, :])
                            if n == 0:
                                g[n] = (h[0][0] + skip[c], h[0][1])
                            else:
                                g[n] = (h[n][0] - h[n - 1][1], h[n][1] + h[n - 1][0])
                        return g[n]

                    for b in range(max(outs) + 1):
                        xr, xi = xg_s[c, b, re, :], xg_s[c, b, im, :]
                        cost = 0
                        for a in outs:
                            if b > a:
                                continue
                            gr, gi = filt(a - b)
                            p = (xr * gr - xi * gi, xr * gi + xi * gr)
                            acc[a] = p if a not in acc else (acc[a][0] + p[0], acc[a][1] + p[1])
                            cost += 1
                            if a == b and sign == 0:
                                plus[a] = jnp.concatenate(acc[a], axis=0)
                            elif a == b:
                                minus = jnp.concatenate(acc[a], axis=0)
                                y_of(c)[a, pl.ds(r0, 16), :] = (plus[a] + minus).astype(BF)
                                y_of(c)[a, pl.ds(pl.multiple_of(r0 + CB, 16), 16), :] = (
                                    plus[a] - minus).astype(BF)
                        yield cost

    class Filler:
        def __init__(self):
            self.gen, self.credit, self.in_k = None, 0.0, False

        def pin(self, value, amount):
            if self.gen is None or amount == 0:
                return
            if self.in_k:
                k_v[S + L:S + L + 16, 0:T] = jnp.concatenate([value, value], axis=0).astype(BF)
            else:
                xg_s[2 * NC, 0, 0:8, :] = value
            self.credit += amount
            while self.gen is not None and self.credit > 0:
                cost = next(self.gen, None)
                if cost is None:
                    self.gen = None
                else:
                    self.credit -= cost

        def drain(self):
            if self.gen is not None:
                for _ in self.gen:
                    pass
            self.gen = None

    filler = Filler()

    def conv_inverse(u, c):
        r0 = pl.multiple_of(u * CB, CB)
        lanes = slice(c * T, (c + 1) * T)
        qs = _halves(q_v[pl.ds(r0, CB), lanes])
        out = []
        for j in range(2):
            inv = jnp.concatenate([_unpack(dft_s[4 + j, 0:T // 2, :]),
                                   _unpack(dft_s[4 + j, T // 2:T, :])], axis=1)
            y = _dot(inv, y_of(c)[u, j * CB:(j + 1) * CB, :])
            out.append(qs[j] * y)
        outa_s[pl.ds(r0, CB), lanes] = _interleave(*out)

    def out_proj(o, rows, amount):
        m = o[0].shape[0]
        last = NC - 1
        head = jnp.concatenate(o[0:last], axis=1)

        def pin(part):
            for r in range(0, m, 32):
                filler.pin(part[r:r + 8, 0:T], amount * 32 / (6 * m))

        edge = _dot(o[last], jnp.concatenate(
            [wo_v[n, last * T:D, :] for n in range(last)], axis=1))
        pin(edge)
        yield
        corner = _dot(o[last], wo_v[last, last * T:D, :])
        for n in reversed(range(NC)):
            part = _dot(head, wo_v[n, 0:last * T, :])
            pin(part)
            part = part + (corner if n == last else edge[:, n * T:(n + 1) * T])
            outb_s[rows, n * T:(n + 1) * T] = part.astype(BF)
            yield

    def own_rows(x, i, fill):
        low4 = _iota((8, T), 0) < 4
        full = jnp.full((8, T), fill, F32)
        g0 = 5 * (i // 2)
        if i % 2 == 0:
            body = [x[8 * g0:8 * g0 + 16], jnp.where(low4, x[8 * g0 + 16:8 * g0 + 24], fill)]
        else:
            body = [jnp.where(low4, fill, x[8 * g0 + 16:8 * g0 + 24]), x[8 * g0 + 24:8 * g0 + 40]]
        return jnp.concatenate(body + [full] if i < 2 else [full] + body, axis=0).astype(BF)

    def project(n, par, amount, need_q=True, need_k=True):
        s, u = n // NU, n % NU
        w0 = pl.multiple_of((u // 2) * (WPAIR // 2), 32) + par * (UD // 2)
        x0 = pl.multiple_of(s * L, L)
        slot = (n // 2) % 2
        pad = jnp.zeros((T - UD, T), F32)

        def finish(j, qkv):
            cols = slice(j * T, (j + 1) * T)
            qt, kt, vt = qkv[0:UD], qkv[UD:2 * UD], qkv[2 * UD:3 * UD]
            kn_s[cols, :] = jnp.concatenate([kt, pad], axis=0).T.astype(BF)
            qs = qt * (DH ** -0.5 * LOG2E)
            low4 = _iota((8, T), 0) < 4
            left = _iota((8, T), 1) < T // 2
            zero = jnp.zeros((8, T), F32)
            for pr in range(UH // 2):
                qa = [qs[40 * pr + 8 * r:40 * pr + 8 * r + 8] for r in range(3)]
                qb = [pltpu.roll(qs[40 * pr + 8 * r:40 * pr + 8 * r + 8], T // 2, 1) for r in (2, 3, 4)]
                ra = [qa[0], qa[1], jnp.where(low4, qa[2], 0.0)]
                rb = [jnp.where(low4, 0.0, qb[0]), qb[1], qb[2]]
                rh = [jnp.where(left, 0.0, qa[0]), jnp.where(left, 0.0, qa[1]),
                      jnp.where(left, rb[0], ra[2]),
                      jnp.where(left, qb[1], 0.0), jnp.where(left, qb[2], 0.0)]
                for i, rows in ((2 * pr, ra), (2 * pr + 1, rb)):
                    rows = rows + [zero] if pr == 0 else [zero] + rows
                    rq_s[j, i, 8 * i:8 * i + 16, :] = _pack(jnp.concatenate(rows, axis=0).astype(BF))
                rows = rh + [zero] if pr == 0 else [zero] + rh
                rq_s[j, UH + pr, 16 * pr:16 * pr + 24, :] = _pack(
                    jnp.concatenate(rows, axis=0).astype(BF))
            for i in range(UH):
                va_s[par][slot, i, j] = own_rows(vt, i, 1.0)
            if need_q:
                pq_s[par][slot, j] = _phi(qt).astype(BF)
            if need_k:
                pk_s[par][slot, j] = _phi(kt).astype(BF)
                vt_s[par][slot, j] = vt.astype(BF)

        w = [_unpack(jnp.concatenate(
            [wt_s[c, i, pl.ds(pl.multiple_of(w0, 8), UD // 2), :] for i in range(3)], axis=0))
             for c in range(NC)]
        part = _dot_nt(w[NC - 1], x_v[NC - 1, pl.ds(x0, L), :])
        for j in range(NQ):
            e_s[j] = part[:, j * T:(j + 1) * T]
        for r in range(0, 3 * UD, 24):
            filler.pin(part[r:r + 8, 0:T], amount / (10 * NC))
        yield
        w = jnp.concatenate(w[0:NC - 1], axis=1)
        for j in reversed(range(NQ)):
            rows = pl.ds(pl.multiple_of(x0 + j * T, T), T)
            part = _dot_nt(w, jnp.concatenate([x_v[c, rows, :] for c in range(NC - 1)], axis=1))
            for r in range(0, 3 * UD, 24):
                filler.pin(part[r:r + 8], amount / (10 * NC))
            finish(j, part + e_s[j])
            yield

    HALF = T // 2

    def s_off(j, i, t, n=T):
        return pl.ds((2 * j * (j + 1) + i * (j + 1) + t) * T, n)

    def hi_off(j, pr):
        return pl.ds((2 * j * (j + 1) + 2 * pr * (j + 1) + j) * T + HALF, HALF)

    def sparse(j, i, first, count):
        parts = [_unpack(rq_s[j, i, first // 2:(first + count) // 2, :]),
                 jnp.zeros((T - first - count, T), BF)]
        if first:
            parts.insert(0, jnp.zeros((first, T), BF))
        return jnp.concatenate(parts, axis=0)

    def col_max(x):
        return jnp.max(x.reshape(x.shape[0] // 8, 8, T), axis=0)

    def scores(j, t, top, amount):
        rq = jnp.concatenate([sparse(j, i, i // 1 * 16, 32) for i in range(UH)], axis=1)
        n = T if t < j else HALF
        sc = _dot(kn_s[t * T:t * T + n, :], rq)
        if t == j:
            rh = jnp.concatenate([sparse(j, UH + pr, 32 * pr, 48) for pr in range(2)], axis=1)
            hi = _dot(kn_s[t * T + HALF:(t + 1) * T, :], rh)
        for i in range(UH):
            si = sc[:, i * T:(i + 1) * T]
            if t == j:
                si = si + bias_s[i % 2]
            s_s[s_off(j, i, t, n), :] = si
            if i == 0:
                for r in range(0, n, 32):
                    filler.pin(si[r:r + 8], amount * 32 / n)
            top[i] = col_max(si) if t == 0 else jnp.maximum(top[i], col_max(si))
        if t < j:
            return
        left = _iota((8, T), 1) < HALF
        for pr in range(2):
            si = hi[:, pr * T:(pr + 1) * T] + bias_s[2]
            s_s[hi_off(j, pr), :] = si
            mh = col_max(si)
            ma = jnp.maximum(top[2 * pr], jnp.where(left, -jnp.inf, mh))
            mb = jnp.maximum(top[2 * pr + 1], jnp.where(left, mh, -jnp.inf))
            ma = jnp.broadcast_to(jnp.max(ma, axis=0, keepdims=True), (8, T))
            mb = jnp.broadcast_to(jnp.max(mb, axis=0, keepdims=True), (8, T))
            m_s[j, 2 * pr] = ma
            m_s[j, 2 * pr + 1] = mb
            m_s[j, UH + pr] = jnp.where(left, mb, ma)

    def weights(rows, j, i):
        sc = s_s[rows, :]
        m = jnp.concatenate([m_s[j, i]] * (sc.shape[0] // 8), axis=0)
        return jnp.exp2(sc - m).astype(BF)

    def softmax(par, j, t):
        n = T if t < j else HALF
        for i in range(UH):
            p_s[par][s_off(j, i, t, n), :] = weights(s_off(j, i, t, n), j, i)
        if t < j:
            return
        left = _iota((HALF // 2, T), 1) < HALF
        none = jnp.zeros((HALF // 2, T), jnp.uint32)
        for pr in range(2):
            p = pltpu.bitcast(weights(hi_off(j, pr), j, UH + pr), jnp.uint32)
            for i, part in ((2 * pr, jnp.where(left, none, p)), (2 * pr + 1, jnp.where(left, p, none))):
                p_s[par][pl.ds(s_off(j, i, t).start + HALF, HALF), :] = pltpu.bitcast(part, BF)

    def spread(a, b):
        low4 = _iota(a.shape, 0) < 4
        ar, br = pltpu.roll(a, 4, 0), pltpu.roll(b, 4, 0)
        r0, r1 = jnp.where(low4, a, ar), jnp.where(low4, ar, a)
        r2, r3 = jnp.where(low4, b, br), jnp.where(low4, br, b)
        return jnp.concatenate([r0, r0, a, r1, r1, r2, r2, b, r3, r3], axis=0)

    def retrieve(n, par):
        u, slot = n % NU, (n // 2) % 2
        zpad = jnp.zeros((T - UD, T), BF)
        pq = jnp.concatenate(
            [jnp.concatenate([pq_s[par][slot, j], zpad], axis=0) for j in range(NQ)], axis=1)
        ret = _dot(meml_s[u], pq)
        rd = 1.0 / (ret[UD:UD + 16] + 1e-6)
        ret_s[...] = ret[0:UD] * spread(rd[0:8], rd[8:16])

    def update(n, par, s):
        u, slot = n % NU, (n // 2) % 2
        zpad = jnp.zeros((T - UD, T), BF)
        va = jnp.concatenate(
            [jnp.concatenate([vt_s[par][slot, j], jnp.ones((16, T), BF)], axis=0) for j in range(NQ)],
            axis=1)
        pk = jnp.concatenate(
            [jnp.concatenate([pk_s[par][slot, j], zpad], axis=0) for j in range(NQ)], axis=1)
        mem = _dot_nt(va, pk)
        if s > 0:
            mem = mem_s[u] + mem
        if s < NSEG - 2:
            mem_s[u] = mem
        row = _iota((UD + 16, T), 0)
        row_head = jnp.where(row < UD, _head_of(row), (row - UD) >> 2)
        meml_s[u] = jnp.where(row_head == _head_of(_iota((UD + 16, T), 1)), mem, 0.0).astype(BF)

    def values(n, par, s, j, t, acc):
        u, slot = n % NU, (n // 2) % 2
        for i in range(UH):
            part = _dot(va_s[par][slot, i, t], p_s[par][s_off(j, i, t), :])
            acc[i] = part if t == 0 else acc[i] + part
        if t < j:
            return
        heads = []
        for i in range(UH):
            den = acc[i][24:32] if i < 2 else acc[i][0:8]
            val = acc[i][0:24] if i < 2 else acc[i][8:32]
            val = val * jnp.concatenate([1.0 / den] * 3, axis=0)
            heads.append(pltpu.roll(val, HALF, 1) if i % 2 else val)
        low4 = _iota((8, T), 0) < 4
        att = jnp.concatenate([
            heads[0][0:16], jnp.where(low4, heads[0][16:24], heads[1][0:8]), heads[1][8:24],
            heads[2][0:16], jnp.where(low4, heads[2][16:24], heads[3][0:8]), heads[3][8:24]], axis=0)
        rows = pl.ds(pl.multiple_of(u * UD, 16), UD)
        gt = gate_s[rows, :]
        o = (1.0 - gt) * att
        if s > 0:
            o = o + gt * ret_s[:, j * T:(j + 1) * T]
        o = o.astype(BF)
        ot_s[s % 2][j, rows, :] = o

    ORDERS = [
        ENV('ORD0', 'P Q30 V30 Q31 V31 Q32 V32 Q33 V33 P X U Q20 V20 Q21 V21 Q22 X V22 P Q10 V10 Q11 X V11 P X V00 Q00 P X / P Q30 V30 V31 Q31 X Q32 Q33 V32 V33 X U P Q20 X V20 Q21 V21 Q22 V22 P Q10 V10 X Q11 X V11 P V00 Q00 P'),
        ENV('ORD1', 'R P Q30 Q31 V30 V31 Q32 V32 U Q33 V33 P Q20 V20 O Q21 V21 Q22 V22 P O Q10 Q11 V10 O V11 V00 Q00 P P / V30 P R Q30 Q31 V31 Q32 V32 Q33 V33 U Q20 V20 P Q21 V21 Q22 Q10 V10 Q11 V22 Q00 O P P P V11 V00 O O'),
        ENV('ORD1', 'R P Q30 Q31 V30 V31 Q32 V32 U Q33 V33 P Q20 V20 O Q21 V21 Q22 V22 P O Q10 Q11 V10 O V11 V00 Q00 P P / V30 P R Q30 Q31 V31 Q32 V32 Q33 V33 U Q20 V20 P Q21 V21 Q22 Q10 V10 Q11 V22 Q00 O P P P V11 V00 O O'),
        ENV('ORD3', 'R P Q30 V30 Q31 V31 X V32 Q32 Q33 V33 P X X Q20 V20 Q21 V21 Q22 V22 P Q10 V10 Q11 X V11 O P Q00 P V00 / P Q30 V30 X Q31 R V31 V32 Q32 Q33 V33 P X Q20 V20 Q21 V21 X V22 Q22 Q10 V10 Q11 V11 X P Q00 P O P V00 O O O O'),
    ]
    ORDA = ENV('ORDA', 'R P Q30 V30 V31 Q31 X V32 Q32 Q33 V33 P X Q20 V20 Q21 V21 X Q22 V22 P Q10 V10 Q11 X V11 O P Q00 P V00 / P Q30 V30 Q31 V31 R X V32 Q32 Q33 V33 P X Q20 V20 Q21 O V21 X V22 Q22 Q10 V10 O Q11 V11 X P P Q00 P O V00 O O')
    ORDB = ENV('ORDB', 'R X X X Q30 V30 X Q31 V31 X V32 Q32 X Q33 X Q20 X V20 V33 Q21 V21 X V22 Q22 X Q10 X V10 X Q11 V11 Q00 V00 / R D X V30 V31 X V32 V33 X V20 V21 X V22 O O D O V10 V11 V00 O O O D T3 T3 T3 T3 T3 T3 T2 T2 T2 T2 T1 T2 T1 T1 T1 T2 T1 T1 T0 T0 T0 T0 T0 T0')
    ORDA, ORDB = ([half.split() for half in order.split('/')] for order in (ORDA, ORDB))
    SHA = [float(v) for v in ENV('SHA', '0.6,0.35,0.05').split(',')]
    PRO1 = ENV('PRO1', 'Q30 Q31 Q32 Q33 P P Q20 Q21 W Q22 P Q10 Q11 P Q00 P')
    PRO = ENV('PRO', 'P Q30 Q31 Q32 Q33 P Q20 Q21 Q22 P Q10 Q11 P Q00 P')
    ORDERS = [[half.split() for half in order.split('/')] for order in ORDERS]
    SHARE = [[float(v) for v in ENV(k, d).split(',')] for k, d in
             (('SH0', '0.65,0.65,0'), ('SH1', '0.0,0.7,0.3'), ('SH1', '0.0,0.7,0.3'), ('SH3', '0.15,0.4,0.45'))]

    deliver = []

    def step(n, par, s, order, share, jobs=(), oproj=None, stages='PQSV', need_q=True, arrive=None):
        jobs = list(jobs)
        proj = project(n + 3, 1 - par, share[1], need_q=need_q, need_k=s < NSEG - 1)
        top, acc, final = [None] * UH, {}, {}
        for tok in order:
            if tok[0] == 'Q':
                j, t = int(tok[1]), int(tok[2])
                if 'S' in stages:
                    softmax(1 - par, j, t)
                if 'Q' in stages:
                    scores(j, t, top, share[0] / 10)
            elif tok[0] == 'V':
                if 'V' in stages:
                    values(n, par, s, int(tok[1]), int(tok[2]), acc.setdefault(tok[1], [None] * UH))
            elif tok == 'P':
                if 'P' in stages:
                    next(proj)
            elif tok == 'R':
                if 'V' in stages and s > 0:
                    retrieve(n, par)
            elif tok == 'U':
                if 'V' in stages and s < NSEG - 1:
                    update(n, par, s)
            elif tok[0] == 'T':
                j = int(tok[1])
                rows = pl.ds((NSEG - 1) * L + j * T, T)
                if j not in final:
                    final[j] = [out_proj(out_tiles(NSEG - 1, j), rows, 0), 0]
                next(final[j][0])
                final[j][1] += 1
                if final[j][1] == NC + 1:
                    ob_copy(rows).start()
            elif tok == 'D':
                deliver.pop(0)()
            elif tok == 'O':
                if oproj is not None:
                    next(oproj)
            elif tok == 'W':
                if arrive is not None:
                    arrive()
            elif tok == 'X':
                if jobs:
                    jobs.pop(0)()
        assert not jobs

    def out_tiles(s, j):
        return [ot_s[s % 2][j, c * T:(c + 1) * T, :].T for c in range(NC)]

    def pair_step(s, j, stages=('PQSV', 'PQSV'), arrive=None, mac=None, inverse=None, middle=None,
                  orders=None, mix=None):
        orders, mix = orders or ORDERS[s], mix or SHARE[s]
        us = (2 * j, 2 * j + 1)
        share, oproj = [8 * NC * v for v in mix], None
        filler.gen, filler.credit, filler.in_k = None, 0.0, s == 0
        if s == 0:
            del self_done[:]
            filler.gen = (cost for half, u in enumerate(us) for cost in gate_kv(u, half))
            share = [16 * NC * v for v in mix]
        else:
            if mac is None:
                mac = [(c, 4 * j + r) for c in (2 * s - 2, 2 * s - 1) for r in range(4)]
            weight = (mix[0] * sum('Q' in st for st in stages)
                      + mix[1] * sum('P' in st for st in stages) + 2 * mix[2])
            share = [72 * len(mac) * v / weight for v in mix]
            if mac and 'nomac' not in OPT:
                filler.gen = conv_mac(mac, int(ENV('W', '2')))
            rows = pl.ds(pl.multiple_of((s - 1) * L + j * T, T), T)
            oproj = out_proj(out_tiles(s - 1, j), rows, 2 * share[2])
        for half, u in enumerate(us):
            jobs, wait = [], None
            if half == 1 and middle is not None:
                middle()
            if s == 0:
                def forward(u, half, c):
                    while (half, c) not in self_done and filler.gen is not None:
                        if next(filler.gen, None) is None:
                            filler.gen = None
                        filler.credit -= 1
                    conv_forward(u, half, c)
                jobs = [lambda c=c, u=u, half=half: forward(u, half, c) for c in range(NC)]
            elif s == NSEG - 1:
                todo = (inverse[half] if inverse else []) + [(u, c) for c in range(NC - 1)]
                jobs = [lambda b=b, c=c: conv_inverse(b, c) for b, c in todo]
            step(s * NU + u, half, s, orders[half],
                 share, jobs, oproj, stages[half], arrive=wait)
        filler.drain()

    def last_mac(j, extra=None):
        return [(NC - 1, f) for f in [4 * j + r for r in range(4)] + (extra or [12 + 2 * j])]

    def scoped(f, s, j):
        with _scope("it"):
            f(s, j)

    def transpose_weights(t):
        for i in range(3):
            for c in range(NC):
                wt = _pack(w_v[i, t, c * T:(c + 1) * T, :].T)
                for r in range(T // 16):
                    pair, off = divmod(t * T + 16 * r, 2 * UD)
                    row = (pair * WPAIR + off) // 2
                    wt_s[c, i, row:row + 8, :] = wt[8 * r:8 * r + 8]

    def d_row(c):
        return d_ref[...].astype(F32).reshape(1, D)[:, c * T:(c + 1) * T]

    def send_pair(j):
        oa_copy(pl.ds(pl.multiple_of(j * L, L), L), pl.ds(0, (NC - 1) * T)).start()
        ob_copy(pl.ds(pl.multiple_of(2 * L + j * T, T), T)).start()

    def epilogue():
        first = pl.ds(0, (NC - 1) * T)
        with _scope("seg3a"):
            pair_step(3, NQ - 2, stages=('PQSV', 'QSV'), mac=last_mac(NQ - 2, [13, 15]), orders=ORDA, mix=SHA)
        send_pair(NQ - 2)

        deliver.extend([
            lambda: (oa_copy(pl.ds(0, S), pl.ds((NC - 1) * T, T)).start(),
                     oa_copy(pl.ds(S - 2 * CB, CB), first).start()),
            lambda: oa_copy(pl.ds(S - CB, CB), first).start(),
            lambda: ob_copy(pl.ds(3 * L - T, T)).start()])
        with _scope("seg3e"):
            pair_step(3, NQ - 1, stages=('SV', 'V'), mac=[], orders=ORDB,
                      inverse=[[(b, NC - 1) for b in range(NB)], []])

    if ONLY == 'E':
        epilogue()
        return
    if ONLY:
        for k in range(NB):
            zero_s[k] = 0
        with _scope('loop'):
            if 'quad' in OPT:
                lax.fori_loop(0, 2, lambda j, _: [pair_step(int(ONLY), 2 * j + r, mac=last_mac(2 * j + r) if ONLY == '3' else None) for r in range(2)] and None, None)
            else:
              lax.fori_loop(0, NQ, lambda j, _: pair_step(int(ONLY), j, mac=last_mac(j) if ONLY == '3' else None), None)

        def fin(i, _):
            z = (y_s[i, i, 0:16, :].astype(F32) + yl_s[i, 0:16, :] + ot0_s[i, 0:16, :] + ot1_s[i, 0:16, :] + mem_s[i, 0:16, :]
                 + xg_s[i, i, 0:16, :] + meml_s[i, 0:16, :] + kv_s[0, i, 0:16, :] + p0_s[pl.ds(i * 16, 16), :] + p1_s[pl.ds(i * 16, 16), :] + s_s[pl.ds(i * 16, 16), :])
            for tag, fn in dict(aq=lambda: q_v[0:16, 0:T], ak=lambda: k_v[0:16, 0:T], av=lambda: v_v[0:16, 0:T], ah=lambda: h_v[i, 0:16, 0:T],
                                aw=lambda: w_v[0, i, 0:16, :], ad=lambda: dft_s[i, 0:16, :], af=lambda: kf_s[0, 0, 0:1, :], ag=lambda: gate_s[0:16, :],
                                a1=lambda: shift_ref[0:1, 0:T].astype(F32), a2=lambda: dft_s[i, 0:16, :],
                                a3=lambda: beta_ref[0:1].astype(F32).reshape(1, 1)).items():
                if tag in OPT.split(',') or 'alive' in OPT:
                    z = z + fn()
            outa_s[0:16, 0:T] = z.astype(BF)
            cp = pltpu.make_async_copy(outa_s, out_hbm.at[:, pl.ds(0, D)], sem_q); cp.start(); cp.wait()
            cp = pltpu.make_async_copy(outb_s, out_hbm.at[:, pl.ds(D, D)], sem_q); cp.start(); cp.wait()
        lax.fori_loop(0, 4, fin, None)
        return

    for i in range(3):
        w_copy(i, 0).start()
    const_copy(0).start()
    with _scope("setup"):
        for c in range(NC):
            x_copy(c, 0, 1).start()
        key, lane = _iota((T // 2, T), 0), _iota((T // 2, T), 1)
        for b, query in enumerate((lane, lane ^ (T // 2), lane & (T // 2 - 1))):
            bias_s[b] = jnp.where(key > query, -1e9 * LOG2E, 0.0).astype(F32)
        kf_s[...] = jnp.zeros(kf_s.shape, F32)
        for k in range(NB):
            zero_s[k] = 0
        const_copy(0).wait()
        g = jax.nn.sigmoid(beta_ref[...].astype(F32).reshape(1, H))
        rr = _iota((D, H), 0)
        hh = _iota((D, H), 1) * DH
        gate = jnp.sum(jnp.where((rr >= hh) & (rr < hh + DH), g, 0.0), axis=1, keepdims=True)
        gate_s[...] = jnp.broadcast_to(gate, (D, T))
    with _scope("w0"):
        for i in range(3):
            w_copy(i, 0).wait()
        for i in range(3):
            w_copy(i, 1).start()
    with _scope("t0"):
        transpose_weights(0)
    with _scope("x0"):
        for c in range(NC):
            x_copy(c, 0, 1).wait()
        for i in range(3):
            w_copy(i, 2).start()
    with _scope("p0"):
        for _ in project(0, 0, 0, need_q=False):
            pass
    with _scope("w1"):
        for i in range(3):
            w_copy(i, 1).wait()
        for i in range(3):
            w_copy(i, 3).start()
        const_copy(1).start()
        const_copy(3).start()
    with _scope("p1"):
        transpose_weights(1)

        def fetch_conv():
            for cp in conv_copies(0):
                cp.start()
            if True:
                return
            for t in (2, 3):
                for i in range(3):
                    w_copy(i, t).wait()
            for t in (2, 3):
                transpose_weights(t)
        step(-2, 0, 0, PRO1.split(), (0, 0), stages='PQ', need_q=False, arrive=fetch_conv)
        if True:
            for t in (2, 3):
                for i in range(3):
                    w_copy(i, t).wait()
            for t in (2, 3):
                transpose_weights(t)
        step(-1, 1, 0, PRO.split(), (0, 0), stages='PQS', need_q=False)
    with _scope('aw'):
        const_copy(1).wait()
        const_copy(3).wait()
        for cp in conv_copies(0):
            cp.wait()
    for i in range(3):
        w_copy(i, 4).start()
    for c in range(NC):
        x_copy(c, 1, 1).start()

    def seg0(j, _):
        @pl.when(j == 1)
        def _():
            for i in range(3):
                w_copy(i, 4).wait()
            for c in range(NC):
                x_copy(c, 1, 1).wait()
            for c in range(NC):
                wo_copy(c).start()
                x_copy(c, 2, 2).start()
            const_copy(2).start()
            transpose_weights(4)

        for cp in conv_copies(j + 1):
            cp.start()
        pair_step(0, j)
        for cp in conv_copies(j + 1):
            cp.wait()
    with _scope("seg0"):
        lax.fori_loop(0, NQ, seg0, None)

    const_copy(2).wait()
    const_copy(4).start()
    for c in range(NC):
        wo_copy(c).wait()
        x_copy(c, 2, 2).wait()

    with _scope("seg1"):
        lax.fori_loop(0, NQ, lambda j, _: pair_step(1, j), None)
    ob_copy(pl.ds(0, L)).start()
    q_copy().start()
    with _scope("seg2"):
        lax.fori_loop(0, NQ, lambda j, _: pair_step(2, j), None)
    ob_copy(pl.ds(L, L)).start()
    q_copy().wait()
    const_copy(4).wait()

    with _scope("seg3"):
        def seg3(j, _):
            pair_step(3, j, mac=last_mac(j))
            send_pair(j)
        lax.fori_loop(0, NQ - 2, seg3, None)
    epilogue()

    with _scope('wa'):
        oa_copy(pl.ds(0, S), pl.ds(0, D)).wait()
    with _scope('wb'):
        ob_copy(pl.ds(0, S)).wait()


@jax.jit
def pallas_concat_heads__ssm_conv_h3__memory_aug_infini_attn__prompt_kernel(
    A_q, A_k, A_v, A_shift_k, A_ssm_k, A_ssm_D, B_x, B_wq, B_wk, B_wv, B_wo, B_beta,
):
    hbm = pl.BlockSpec(memory_space=pl.ANY)
    dma = pltpu.SemaphoreType.DMA
    out = pl.pallas_call(
        _kernel,
        out_shape=jax.ShapeDtypeStruct((S, 2 * D), BF),
        in_specs=[hbm] * 13,
        out_specs=hbm,
        scratch_shapes=[
            pltpu.VMEM((S, D), BF),
            pltpu.VMEM((S + L + 64, D), BF),
            pltpu.VMEM((S + L, D), BF),
            pltpu.VMEM((NQ + 1, D, L), BF),
            pltpu.VMEM((NC, S, T), BF),
            pltpu.VMEM((3, NC, D, T), BF),
            pltpu.VMEM((NC, D, T), BF),
            pltpu.VMEM((NC, 3, NQ * WPAIR // 2, T), jnp.uint32),
            pltpu.VMEM((6, T, T), jnp.uint32),
            pltpu.VMEM((NC + 1, 2, 8, T), F32),
            pltpu.VMEM((2, NC, CB, T), BF),
            pltpu.VMEM((2 * NC + 1, NB, 2 * CB, T), F32),
            pltpu.VMEM((NC - 1, NB, 2 * CB, T), BF),
            pltpu.VMEM((NB, 2 * CB, T), BF),
            pltpu.VMEM((S, D), BF),
            pltpu.VMEM((S, D), BF),
            pltpu.VMEM((NQ, D, T), BF),
            pltpu.VMEM((NQ, D, T), BF),
            pltpu.VMEM((NU, UD + 16, T), F32),
            pltpu.VMEM((NU, UD + 16, T), BF),
            pltpu.VMEM((D, T), F32),
            pltpu.VMEM((3, T // 2, T), F32),
            pltpu.VMEM((L, T), BF),
            pltpu.VMEM((NQ, UH + 2, T // 2, T), jnp.uint32),
            *[pltpu.VMEM((2, NQ, UD, T), BF)] * 6,
            *[pltpu.VMEM((2, UH, NQ, 32, T), BF)] * 2,
            pltpu.VMEM((40 * T, T), F32),
            *[pltpu.VMEM((40 * T, T), BF)] * 2,
            pltpu.VMEM((NQ, UH + 2, 8, T), F32),
            pltpu.VMEM((UD, L), F32),
            pltpu.VMEM((NQ, 3 * UD, T), F32),
            pltpu.VMEM((4, D), BF),
            pltpu.VMEM((D,), BF),
            pltpu.VMEM((H,), BF),
            pltpu.SMEM((NB,), jnp.int32),
            dma((4 * NC,)), dma((NSEG * NC,)), dma((3 * (NQ + 1),)), dma(()),
            dma((5,)), dma(()), dma(()),
        ],
        compiler_params=pltpu.CompilerParams(
            vmem_limit_bytes=100 * 1024 * 1024,
            flags=({'XLA_TPU_EVENLY_DISTRIBUTE_CRITICAL_NODES': True} if 'EV' in OPT else None)),
        name="h3_infini",
    )(A_q.reshape(S, D), A_k.reshape(S, D), A_v.reshape(S, D), A_shift_k.T, A_ssm_k, A_ssm_D,
      B_x.reshape(S, D), B_wq, B_wk, B_wv, B_wo, B_beta, _DFT)
    return out.reshape(1, S, 2 * D)
```

```python
import math, os

import numpy as np
import jax
import jax.numpy as jnp
from jax import lax
from jax.experimental import pallas as pl
from jax.experimental.pallas import tpu as pltpu

OPT = os.environ.get('OPT', '')
ONLY = os.environ.get('ONLY', '')
ENV = os.environ.get

S, D = 2048, 640
H, DH, NSEG, L = 32, 20, 4, 512
T = 128
NC = D // T
CB = 2 * T
NB = S // CB
NF = T // 8
NQ = L // T
UH = 4
UD = UH * DH
NU = H // UH
UR = L // NU
WPAIR = 192
BF, F32 = jnp.bfloat16, jnp.float32
LOG2E = math.log2(math.e)


def _dft_matrices():
    m = np.arange(T)[:, None]
    r = np.arange(T)[None, :]

    def rows(power):
        ang = np.pi * np.mod((4 * m + 1) * power, 1024) / 512
        f = np.stack([np.cos(ang).reshape(NF, 8, T), -np.sin(ang).reshape(NF, 8, T)], 1)
        return f.reshape(2 * T, T)

    even, odd = rows(2 * r), rows(2 * r + 1)
    lane = np.arange(T)
    even_h = even[:, lane // 2 + (T // 2) * (lane % 2)]
    odd_h = odd[:, lane // 2 + (T // 2) * (1 - lane % 2)]
    inverse = [np.concatenate([f[:T].T, f[T:].T]) / (2 * T) for f in (even, odd)]
    bits = np.stack([even, odd, even_h, odd_h] + inverse).astype(np.float32).astype(BF)
    bits = bits.view(np.uint16).astype(np.uint32)
    return bits[:, 0::2] | (bits[:, 1::2] << 16)


_DFT = _dft_matrices()


def _pack(x):
    return pltpu.bitcast(x, jnp.uint32)


def _unpack(w):
    return pltpu.bitcast(w, BF)


def _halves(x):
    w = pltpu.bitcast(x, jnp.uint32)
    return (lax.bitcast_convert_type(w << 16, F32),
            lax.bitcast_convert_type(w & np.uint32(0xFFFF0000), F32))


def _interleave(even, odd):
    e, o = (lax.bitcast_convert_type(v.astype(BF).astype(F32), jnp.uint32) for v in (even, odd))
    return pltpu.bitcast((e >> 16) | o, BF)


import contextlib


def _scope(name):
    return jax.named_scope(name) if 'scope' in OPT else contextlib.nullcontext()


def _dot(a, b):
    return jnp.dot(a, b, preferred_element_type=F32)


def _dot_nt(a, b):
    return lax.dot_general(a, b, (((1,), (1,)), ((), ())), preferred_element_type=F32)


def _phi(t):
    return jnp.where(t > 0, t + 1.0, jnp.exp(t))


def _iota(shape, dim):
    return lax.broadcasted_iota(jnp.int32, shape, dim)


def _head_of(z):
    return sum((z >= DH * i).astype(jnp.int32) for i in range(1, UH))


def _kernel(q_hbm, k_hbm, v_hbm, shift_hbm, h_hbm, d_hbm, x_hbm, wq_hbm, wk_hbm, wv_hbm,
            wo_hbm, beta_hbm, dft_hbm, out_hbm,
            q_v, k_v, v_v, h_v, x_v, w_v, wo_v, wt_s, dft_s, kf_s, kv_s, xg_s, y_s, yl_s,
            outa_s, outb_s, ot0_s, ot1_s, mem_s, meml_s, gate_s, bias_s,
            kn_s, rq_s, pk0_s, pk1_s, pq0_s, pq1_s, vt0_s, vt1_s, va0_s, va1_s, s_s, p0_s, p1_s, m_s, ret_s, e_s, shift_ref, d_ref, beta_ref, zero_s,
            sem_w, sem_x, sem_a, sem_q, sem_c, sem_oa, sem_ob):
    ot_s = (ot0_s, ot1_s)
    pk_s, pq_s, vt_s = (pk0_s, pk1_s), (pq0_s, pq1_s), (vt0_s, vt1_s)
    va_s, p_s = (va0_s, va1_s), (p0_s, p1_s)

    def y_of(c):
        return yl_s if c == NC - 1 else y_s.at[c]

    def w_copy(i, t):
        cols = pl.ds(t * T, T)
        return pltpu.make_async_copy((wq_hbm, wk_hbm, wv_hbm)[i].at[:, cols], w_v.at[i, t],
                                     sem_w.at[i * NC + t])

    def wo_copy(n):
        return pltpu.make_async_copy(wo_hbm.at[:, pl.ds(n * T, T)], wo_v.at[n],
                                     sem_w.at[3 * NC + n])

    def x_copy(c, first, count):
        rows = pl.ds(first * L, count * L)
        return pltpu.make_async_copy(x_hbm.at[rows, pl.ds(c * T, T)], x_v.at[c, rows],
                                     sem_x.at[first * NC + c])

    def conv_copies(j):
        src = pl.ds(pl.multiple_of(jnp.minimum(j, NQ - 1) * L, L), L)
        dst = pl.ds(pl.multiple_of(j * L, L), L)
        return (pltpu.make_async_copy(k_hbm.at[src], k_v.at[dst], sem_a.at[3 * j]),
                pltpu.make_async_copy(v_hbm.at[src], v_v.at[dst], sem_a.at[3 * j + 1]),
                pltpu.make_async_copy(h_hbm.at[:, src], h_v.at[j], sem_a.at[3 * j + 2]))

    def q_copy():
        return pltpu.make_async_copy(q_hbm, q_v, sem_q)

    def const_copy(i):
        src, dst = ((beta_hbm, beta_ref), (shift_hbm, shift_ref), (d_hbm, d_ref),
                    (dft_hbm.at[0:4], dft_s.at[0:4]), (dft_hbm.at[4:6], dft_s.at[4:6]))[i]
        return pltpu.make_async_copy(src, dst, sem_c.at[i])

    def oa_copy(rows, lanes):
        return pltpu.make_async_copy(outa_s.at[rows, lanes], out_hbm.at[rows, lanes], sem_oa)

    def ob_copy(rows):
        return pltpu.make_async_copy(outb_s.at[rows], out_hbm.at[rows, pl.ds(D, D)], sem_ob)

    self_done = []

    def gate_kv(u, half):
        src = pl.multiple_of(u * CB, CB)
        for c in range(NC):
            lanes = slice(c * T, (c + 1) * T)
            taps = [shift_ref[t:t + 1, lanes].astype(F32) for t in range(4)]
            pe, po = kf_s[c, 0], kf_s[c, 1]
            for r in range(0, T, 16):
                rows = pl.ds(pl.multiple_of(src + 2 * r, 32), 32)
                ke, ko = _halves(k_v[rows, lanes])
                ve, vo = _halves(v_v[rows, lanes])
                e1 = pltpu.roll(jnp.concatenate([pe, ke], axis=0), 1, 0)[8:24]
                odd = jnp.concatenate([po, ko], axis=0)
                o1, o2 = pltpu.roll(odd, 1, 0)[8:24], pltpu.roll(odd, 2, 0)[8:24]
                se = ke * taps[0] + o1 * taps[1] + e1 * taps[2] + o2 * taps[3]
                so = ko * taps[0] + ke * taps[1] + o1 * taps[2] + e1 * taps[3]
                kv_s[half, c, r:r + 16, :] = (se * ve).astype(BF)
                kv_s[half, c, T + r:T + r + 16, :] = (so * vo).astype(BF)
                pe, po = ke[8:16], ko[8:16]
                yield 1
            kf_s[c, 0] = pe
            kf_s[c, 1] = po
            self_done.append((half, c))

    def conv_forward(u, half, c):
        lanes = slice(c * T, (c + 1) * T)
        h0, h1 = (pltpu.bitcast(h_v[u // 2, lanes, (2 * half + j) * T:(2 * half + j + 1) * T], jnp.uint32)
                  for j in range(2))
        even = (_iota(h0.shape, 1) & 1) == 0
        he = pltpu.bitcast(jnp.where(even, h0, pltpu.roll(h1, 1, 1)), BF)
        ho = pltpu.bitcast(jnp.where(even, pltpu.roll(h1, T - 1, 1), h0), BF)
        for base, a, b in (
                (c, _dot(_unpack(dft_s[0]), kv_s[half, c, 0:T, :]),
                 _dot(_unpack(dft_s[1]), kv_s[half, c, T:CB, :])),
                (NC + c, _dot_nt(_unpack(dft_s[2]), he), _dot_nt(_unpack(dft_s[3]), ho))):
            xg_s[base, u, 0:CB, :] = a + b
            xg_s[base, u, CB:2 * CB, :] = a - b

    def conv_mac(items, w=2):
        skip = {c: jnp.broadcast_to(d_row(c), (8, T)) for c, _ in items}
        for c, f in items:
            for k in range(NB // w):
                outs = range(k * w, (k + 1) * w)
                r0 = pl.multiple_of((f + zero_s[k]) * 16, 16)
                plus = {}
                for sign in range(2):
                    re = pl.ds(pl.multiple_of(r0 + sign * CB, 8), 8)
                    im = pl.ds(pl.multiple_of(r0 + sign * CB + 8, 8), 8)
                    acc, g, h = {}, {}, {}

                    def filt(n):
                        if n not in g:
                            for m in (n, n - 1):
                                if m >= 0 and m not in h:
                                    h[m] = (xg_s[NC + c, m, re, :], xg_s[NC + c, m, im, :])
                            if n == 0:
                                g[n] = (h[0][0] + skip[c], h[0][1])
                            else:
                                g[n] = (h[n][0] - h[n - 1][1], h[n][1] + h[n - 1][0])
                        return g[n]

                    for b in range(max(outs) + 1):
                        xr, xi = xg_s[c, b, re, :], xg_s[c, b, im, :]
                        cost = 0
                        for a in outs:
                            if b > a:
                                continue
                            gr, gi = filt(a - b)
                            p = (xr * gr - xi * gi, xr * gi + xi * gr)
                            acc[a] = p if a not in acc else (acc[a][0] + p[0], acc[a][1] + p[1])
                            cost += 1
                            if a == b and sign == 0:
                                plus[a] = jnp.concatenate(acc[a], axis=0)
                            elif a == b:
                                minus = jnp.concatenate(acc[a], axis=0)
                                y_of(c)[a, pl.ds(r0, 16), :] = (plus[a] + minus).astype(BF)
                                y_of(c)[a, pl.ds(pl.multiple_of(r0 + CB, 16), 16), :] = (
                                    plus[a] - minus).astype(BF)
                        yield cost

    class Filler:
        def __init__(self):
            self.gen, self.credit, self.in_k = None, 0.0, False

        def pin(self, value, amount):
            if self.gen is None or amount == 0:
                return
            if self.in_k:
                k_v[S + L:S + L + 16, 0:T] = jnp.concatenate([value, value], axis=0).astype(BF)
            else:
                xg_s[2 * NC, 0, 0:8, :] = value
            self.credit += amount
            while self.gen is not None and self.credit > 0:
                cost = next(self.gen, None)
                if cost is None:
                    self.gen = None
                else:
                    self.credit -= cost

        def drain(self):
            if self.gen is not None:
                for _ in self.gen:
                    pass
            self.gen = None

    filler = Filler()

    def conv_inverse(u, c):
        r0 = pl.multiple_of(u * CB, CB)
        lanes = slice(c * T, (c + 1) * T)
        qs = _halves(q_v[pl.ds(r0, CB), lanes])
        out = []
        for j in range(2):
            inv = jnp.concatenate([_unpack(dft_s[4 + j, 0:T // 2, :]),
                                   _unpack(dft_s[4 + j, T // 2:T, :])], axis=1)
            y = _dot(inv, y_of(c)[u, j * CB:(j + 1) * CB, :])
            out.append(qs[j] * y)
        outa_s[pl.ds(r0, CB), lanes] = _interleave(*out)

    def out_proj(o, rows, amount):
        m = o[0].shape[0]
        last = NC - 1
        head = jnp.concatenate(o[0:last], axis=1)

        def pin(part):
            for r in range(0, m, 32):
                filler.pin(part[r:r + 8, 0:T], amount * 32 / (6 * m))

        edge = _dot(o[last], jnp.concatenate(
            [wo_v[n, last * T:D, :] for n in range(last)], axis=1))
        pin(edge)
        yield
        corner = _dot(o[last], wo_v[last, last * T:D, :])
        for n in reversed(range(NC)):
            part = _dot(head, wo_v[n, 0:last * T, :])
            pin(part)
            part = part + (corner if n == last else edge[:, n * T:(n + 1) * T])
            outb_s[rows, n * T:(n + 1) * T] = part.astype(BF)
            yield

    def own_rows(x, i, fill):
        low4 = _iota((8, T), 0) < 4
        full = jnp.full((8, T), fill, F32)
        g0 = 5 * (i // 2)
        if i % 2 == 0:
            body = [x[8 * g0:8 * g0 + 16], jnp.where(low4, x[8 * g0 + 16:8 * g0 + 24], fill)]
        else:
            body = [jnp.where(low4, fill, x[8 * g0 + 16:8 * g0 + 24]), x[8 * g0 + 24:8 * g0 + 40]]
        return jnp.concatenate(body + [full] if i < 2 else [full] + body, axis=0).astype(BF)

    def project(n, par, amount, need_q=True, need_k=True):
        s, u = n // NU, n % NU
        w0 = pl.multiple_of((u // 2) * (WPAIR // 2), 32) + par * (UD // 2)
        x0 = pl.multiple_of(s * L, L)
        slot = (n // 2) % 2
        pad = jnp.zeros((T - UD, T), F32)

        def finish(j, qkv):
            cols = slice(j * T, (j + 1) * T)
            qt, kt, vt = qkv[0:UD], qkv[UD:2 * UD], qkv[2 * UD:3 * UD]
            kn_s[cols, :] = jnp.concatenate([kt, pad], axis=0).T.astype(BF)
            qs = qt * (DH ** -0.5 * LOG2E)
            low4 = _iota((8, T), 0) < 4
            left = _iota((8, T), 1) < T // 2
            zero = jnp.zeros((8, T), F32)
            for pr in range(UH // 2):
                qa = [qs[40 * pr + 8 * r:40 * pr + 8 * r + 8] for r in range(3)]
                qb = [pltpu.roll(qs[40 * pr + 8 * r:40 * pr + 8 * r + 8], T // 2, 1) for r in (2, 3, 4)]
                ra = [qa[0], qa[1], jnp.where(low4, qa[2], 0.0)]
                rb = [jnp.where(low4, 0.0, qb[0]), qb[1], qb[2]]
                rh = [jnp.where(left, 0.0, qa[0]), jnp.where(left, 0.0, qa[1]),
                      jnp.where(left, rb[0], ra[2]),
                      jnp.where(left, qb[1], 0.0), jnp.where(left, qb[2], 0.0)]
                for i, rows in ((2 * pr, ra), (2 * pr + 1, rb)):
                    rows = rows + [zero] if pr == 0 else [zero] + rows
                    rq_s[j, i, 8 * i:8 * i + 16, :] = _pack(jnp.concatenate(rows, axis=0).astype(BF))
                rows = rh + [zero] if pr == 0 else [zero] + rh
                rq_s[j, UH + pr, 16 * pr:16 * pr + 24, :] = _pack(
                    jnp.concatenate(rows, axis=0).astype(BF))
            for i in range(UH):
                va_s[par][slot, i, j] = own_rows(vt, i, 1.0)
            if need_q:
                pq_s[par][slot, j] = _phi(qt).astype(BF)
            if need_k:
                pk_s[par][slot, j] = _phi(kt).astype(BF)
                vt_s[par][slot, j] = vt.astype(BF)

        w = [_unpack(jnp.concatenate(
            [wt_s[c, i, pl.ds(pl.multiple_of(w0, 8), UD // 2), :] for i in range(3)], axis=0))
             for c in range(NC)]
        part = _dot_nt(w[NC - 1], x_v[NC - 1, pl.ds(x0, L), :])
        for j in range(NQ):
            e_s[j] = part[:, j * T:(j + 1) * T]
        for r in range(0, 3 * UD, 24):
            filler.pin(part[r:r + 8, 0:T], amount / (10 * NC))
        yield
        w = jnp.concatenate(w[0:NC - 1], axis=1)
        for j in reversed(range(NQ)):
            rows = pl.ds(pl.multiple_of(x0 + j * T, T), T)
            part = _dot_nt(w, jnp.concatenate([x_v[c, rows, :] for c in range(NC - 1)], axis=1))
            for r in range(0, 3 * UD, 24):
                filler.pin(part[r:r + 8], amount / (10 * NC))
            finish(j, part + e_s[j])
            yield

    HALF = T // 2

    def s_off(j, i, t, n=T):
        return pl.ds((2 * j * (j + 1) + i * (j + 1) + t) * T, n)

    def hi_off(j, pr):
        return pl.ds((2 * j * (j + 1) + 2 * pr * (j + 1) + j) * T + HALF, HALF)

    def sparse(j, i, first, count):
        parts = [_unpack(rq_s[j, i, first // 2:(first + count) // 2, :]),
                 jnp.zeros((T - first - count, T), BF)]
        if first:
            parts.insert(0, jnp.zeros((first, T), BF))
        return jnp.concatenate(parts, axis=0)

    def col_max(x):
        return jnp.max(x.reshape(x.shape[0] // 8, 8, T), axis=0)

    def scores(j, t, top, amount):
        rq = jnp.concatenate([sparse(j, i, i // 1 * 16, 32) for i in range(UH)], axis=1)
        n = T if t < j else HALF
        sc = _dot(kn_s[t * T:t * T + n, :], rq)
        if t == j:
            rh = jnp.concatenate([sparse(j, UH + pr, 32 * pr, 48) for pr in range(2)], axis=1)
            hi = _dot(kn_s[t * T + HALF:(t + 1) * T, :], rh)
        for i in range(UH):
            si = sc[:, i * T:(i + 1) * T]
            if t == j:
                si = si + bias_s[i % 2]
            s_s[s_off(j, i, t, n), :] = si
            if i == 0:
                for r in range(0, n, 32):
                    filler.pin(si[r:r + 8], amount * 32 / n)
            top[i] = col_max(si) if t == 0 else jnp.maximum(top[i], col_max(si))
        if t < j:
            return
        left = _iota((8, T), 1) < HALF
        for pr in range(2):
            si = hi[:, pr * T:(pr + 1) * T] + bias_s[2]
            s_s[hi_off(j, pr), :] = si
            mh = col_max(si)
            ma = jnp.maximum(top[2 * pr], jnp.where(left, -jnp.inf, mh))
            mb = jnp.maximum(top[2 * pr + 1], jnp.where(left, mh, -jnp.inf))
            ma = jnp.broadcast_to(jnp.max(ma, axis=0, keepdims=True), (8, T))
            mb = jnp.broadcast_to(jnp.max(mb, axis=0, keepdims=True), (8, T))
            m_s[j, 2 * pr] = ma
            m_s[j, 2 * pr + 1] = mb
            m_s[j, UH + pr] = jnp.where(left, mb, ma)

    def weights(rows, j, i):
        sc = s_s[rows, :]
        m = jnp.concatenate([m_s[j, i]] * (sc.shape[0] // 8), axis=0)
        return jnp.exp2(sc - m).astype(BF)

    def softmax(par, j, t):
        n = T if t < j else HALF
        for i in range(UH):
            p_s[par][s_off(j, i, t, n), :] = weights(s_off(j, i, t, n), j, i)
        if t < j:
            return
        left = _iota((HALF // 2, T), 1) < HALF
        none = jnp.zeros((HALF // 2, T), jnp.uint32)
        for pr in range(2):
            p = pltpu.bitcast(weights(hi_off(j, pr), j, UH + pr), jnp.uint32)
            for i, part in ((2 * pr, jnp.where(left, none, p)), (2 * pr + 1, jnp.where(left, p, none))):
                p_s[par][pl.ds(s_off(j, i, t).start + HALF, HALF), :] = pltpu.bitcast(part, BF)

    def spread(a, b):
        low4 = _iota(a.shape, 0) < 4
        ar, br = pltpu.roll(a, 4, 0), pltpu.roll(b, 4, 0)
        r0, r1 = jnp.where(low4, a, ar), jnp.where(low4, ar, a)
        r2, r3 = jnp.where(low4, b, br), jnp.where(low4, br, b)
        return jnp.concatenate([r0, r0, a, r1, r1, r2, r2, b, r3, r3], axis=0)

    def retrieve(n, par):
        u, slot = n % NU, (n // 2) % 2
        zpad = jnp.zeros((T - UD, T), BF)
        pq = jnp.concatenate(
            [jnp.concatenate([pq_s[par][slot, j], zpad], axis=0) for j in range(NQ)], axis=1)
        ret = _dot(meml_s[u], pq)
        rd = 1.0 / (ret[UD:UD + 16] + 1e-6)
        ret_s[...] = ret[0:UD] * spread(rd[0:8], rd[8:16])

    def update(n, par, s):
        u, slot = n % NU, (n // 2) % 2
        zpad = jnp.zeros((T - UD, T), BF)
        va = jnp.concatenate(
            [jnp.concatenate([vt_s[par][slot, j], jnp.ones((16, T), BF)], axis=0) for j in range(NQ)],
            axis=1)
        pk = jnp.concatenate(
            [jnp.concatenate([pk_s[par][slot, j], zpad], axis=0) for j in range(NQ)], axis=1)
        mem = _dot_nt(va, pk)
        if s > 0:
            mem = mem_s[u] + mem
        if s < NSEG - 2:
            mem_s[u] = mem
        row = _iota((UD + 16, T), 0)
        row_head = jnp.where(row < UD, _head_of(row), (row - UD) >> 2)
        meml_s[u] = jnp.where(row_head == _head_of(_iota((UD + 16, T), 1)), mem, 0.0).astype(BF)

    def values(n, par, s, j, t, acc):
        u, slot = n % NU, (n // 2) % 2
        for i in range(UH):
            part = _dot(va_s[par][slot, i, t], p_s[par][s_off(j, i, t), :])
            acc[i] = part if t == 0 else acc[i] + part
        if t < j:
            return
        heads = []
        for i in range(UH):
            den = acc[i][24:32] if i < 2 else acc[i][0:8]
            val = acc[i][0:24] if i < 2 else acc[i][8:32]
            val = val * jnp.concatenate([1.0 / den] * 3, axis=0)
            heads.append(pltpu.roll(val, HALF, 1) if i % 2 else val)
        low4 = _iota((8, T), 0) < 4
        att = jnp.concatenate([
            heads[0][0:16], jnp.where(low4, heads[0][16:24], heads[1][0:8]), heads[1][8:24],
            heads[2][0:16], jnp.where(low4, heads[2][16:24], heads[3][0:8]), heads[3][8:24]], axis=0)
        rows = pl.ds(pl.multiple_of(u * UD, 16), UD)
        gt = gate_s[rows, :]
        o = (1.0 - gt) * att
        if s > 0:
            o = o + gt * ret_s[:, j * T:(j + 1) * T]
        o = o.astype(BF)
        ot_s[s % 2][j, rows, :] = o

    ORDERS = [
        ENV('ORD0', 'Q30 V30 Q31 V31 P Q32 V32 Q33 V33 P X U Q20 Q21 V20 X V21 Q22 V22 P Q10 V10 Q11 X V11 V00 P X Q00 P X / Q30 P V30 V31 Q31 Q32 Q33 X V32 V33 X U P Q20 X Q21 V20 V21 Q22 V22 P Q10 V10 X Q11 X V00 P V11 Q00 P'),
        ENV('ORD1', 'R P Q30 Q31 V30 V31 Q32 V32 Q33 U V33 P Q20 V20 O Q21 V21 Q22 V22 P O Q10 Q11 V10 V11 V00 Q00 P P O / V30 P R Q30 Q31 V31 Q32 V32 V20 Q33 V33 Q20 U P Q21 Q22 Q10 V10 Q11 V21 V22 Q00 P O P P V11 V00 O O'),
        ENV('ORD1', 'R P Q30 Q31 V30 V31 Q32 V32 Q33 U V33 P Q20 V20 O Q21 V21 Q22 V22 P O Q10 Q11 V10 V11 V00 Q00 P P O / V30 P R Q30 Q31 V31 Q32 V32 V20 Q33 V33 Q20 U P Q21 Q22 Q10 V10 Q11 V21 V22 Q00 P O P P V11 V00 O O'),
        ENV('ORD3', 'R P Q30 V30 Q31 V31 X V32 V33 Q32 Q33 P X X Q20 V20 Q21 V21 Q22 V22 P Q10 V10 X Q11 V11 O P Q00 P V00 / P R Q30 V30 X Q31 V31 V32 X Q32 Q33 V33 P Q20 V20 V21 Q21 V22 Q22 Q10 V10 X Q11 V11 X P Q00 P O O P V00 O O O'),
    ]
    ORDA = ENV('ORDA', 'R P Q30 V30 V31 Q31 X V32 Q32 Q33 V33 P X Q20 V20 Q21 V21 X Q22 V22 P Q10 V10 Q11 X V11 O P Q00 P V00 / P Q30 V30 Q31 V31 R X V32 Q32 Q33 V33 P X Q20 V20 Q21 O V21 X V22 Q22 Q10 V10 O Q11 V11 X P P Q00 P O V00 O O')
    ORDB = ENV('ORDB', 'R X X X Q30 V30 X Q31 V31 X V32 Q32 X Q33 X Q20 X V20 V33 Q21 V21 X V22 Q22 X Q10 X V10 X Q11 V11 Q00 V00 / R D X V30 V31 X V32 V33 X V20 V21 X V22 O O D O V10 V11 V00 O O O D T3 T3 T3 T3 T3 T3 T2 T2 T2 T2 T1 T2 T1 T1 T1 T2 T1 T1 T0 T0 T0 T0 T0 T0')
    ORDA, ORDB = ([half.split() for half in order.split('/')] for order in (ORDA, ORDB))
    SHA = [float(v) for v in ENV('SHA', '0.6,0.35,0.05').split(',')]
    PRO1 = ENV('PRO1', 'Q30 Q31 Q32 Q33 P P Q20 Q21 W Q22 P Q10 Q11 P Q00 P')
    PRO = ENV('PRO', 'P Q30 Q31 Q32 Q33 P Q20 Q21 Q22 P Q10 Q11 P Q00 P')
    ORDERS = [[half.split() for half in order.split('/')] for order in ORDERS]
    SHARE = [[float(v) for v in ENV(k, d).split(',')] for k, d in
             (('SH0', '0.5,0.8,0.0'), ('SH1', '0.1,0.6,0.3'), ('SH1', '0.1,0.6,0.3'), ('SH3', '0.15,0.4,0.45'))]

    deliver = []

    def step(n, par, s, order, share, jobs=(), oproj=None, stages='PQSV', need_q=True, arrive=None):
        jobs = list(jobs)
        proj = project(n + 3, 1 - par, share[1], need_q=need_q, need_k=s < NSEG - 1)
        top, acc, final = [None] * UH, {}, {}
        for tok in order:
            if tok[0] == 'Q':
                j, t = int(tok[1]), int(tok[2])
                if 'S' in stages:
                    softmax(1 - par, j, t)
                if 'Q' in stages:
                    scores(j, t, top, share[0] / 10)
            elif tok[0] == 'V':
                if 'V' in stages:
                    values(n, par, s, int(tok[1]), int(tok[2]), acc.setdefault(tok[1], [None] * UH))
            elif tok == 'P':
                if 'P' in stages:
                    next(proj)
            elif tok == 'R':
                if 'V' in stages and s > 0:
                    retrieve(n, par)
            elif tok == 'U':
                if 'V' in stages and s < NSEG - 1:
                    update(n, par, s)
            elif tok[0] == 'T':
                j = int(tok[1])
                rows = pl.ds((NSEG - 1) * L + j * T, T)
                if j not in final:
                    final[j] = [out_proj(out_tiles(NSEG - 1, j), rows, 0), 0]
                next(final[j][0])
                final[j][1] += 1
                if final[j][1] == NC + 1:
                    ob_copy(rows).start()
            elif tok == 'D':
                deliver.pop(0)()
            elif tok == 'O':
                if oproj is not None:
                    next(oproj)
            elif tok == 'W':
                if arrive is not None:
                    arrive()
            elif tok == 'X':
                if jobs:
                    jobs.pop(0)()
        assert not jobs

    def out_tiles(s, j):
        return [ot_s[s % 2][j, c * T:(c + 1) * T, :].T for c in range(NC)]

    def pair_step(s, j, stages=('PQSV', 'PQSV'), arrive=None, mac=None, inverse=None, middle=None,
                  orders=None, mix=None):
        orders, mix = orders or ORDERS[s], mix or SHARE[s]
        us = (2 * j, 2 * j + 1)
        share, oproj = [8 * NC * v for v in mix], None
        filler.gen, filler.credit, filler.in_k = None, 0.0, s == 0
        if s == 0:
            del self_done[:]
            filler.gen = (cost for half, u in enumerate(us) for cost in gate_kv(u, half))
            share = [16 * NC * v for v in mix]
        else:
            if mac is None:
                mac = [(c, 4 * j + r) for c in (2 * s - 2, 2 * s - 1) for r in range(4)]
            weight = (mix[0] * sum('Q' in st for st in stages)
                      + mix[1] * sum('P' in st for st in stages) + 2 * mix[2])
            share = [72 * len(mac) * v / weight for v in mix]
            if mac and 'nomac' not in OPT:
                filler.gen = conv_mac(mac, int(ENV('W', '2')))
            rows = pl.ds(pl.multiple_of((s - 1) * L + j * T, T), T)
            oproj = out_proj(out_tiles(s - 1, j), rows, 2 * share[2])
        for half, u in enumerate(us):
            jobs, wait = [], None
            if half == 1 and middle is not None:
                middle()
            if s == 0:
                def forward(u, half, c):
                    while (half, c) not in self_done and filler.gen is not None:
                        if next(filler.gen, None) is None:
                            filler.gen = None
                        filler.credit -= 1
                    conv_forward(u, half, c)
                jobs = [lambda c=c, u=u, half=half: forward(u, half, c) for c in range(NC)]
            elif s == NSEG - 1:
                todo = (inverse[half] if inverse else []) + [(u, c) for c in range(NC - 1)]
                jobs = [lambda b=b, c=c: conv_inverse(b, c) for b, c in todo]
            step(s * NU + u, half, s, orders[half],
                 share, jobs, oproj, stages[half], arrive=wait)
        filler.drain()

    def last_mac(j, extra=None):
        return [(NC - 1, f) for f in [4 * j + r for r in range(4)] + (extra or [12 + 2 * j])]

    def scoped(f, s, j):
        with _scope("it"):
            f(s, j)

    def transpose_weights(t):
        for i in range(3):
            for c in range(NC):
                wt = _pack(w_v[i, t, c * T:(c + 1) * T, :].T)
                for r in range(T // 16):
                    pair, off = divmod(t * T + 16 * r, 2 * UD)
                    row = (pair * WPAIR + off) // 2
                    wt_s[c, i, row:row + 8, :] = wt[8 * r:8 * r + 8]

    def d_row(c):
        return d_ref[...].astype(F32).reshape(1, D)[:, c * T:(c + 1) * T]

    def send_pair(j):
        oa_copy(pl.ds(pl.multiple_of(j * L, L), L), pl.ds(0, (NC - 1) * T)).start()
        ob_copy(pl.ds(pl.multiple_of(2 * L + j * T, T), T)).start()

    def epilogue():
        first = pl.ds(0, (NC - 1) * T)
        with _scope("seg3a"):
            pair_step(3, NQ - 2, stages=('PQSV', 'QSV'), mac=last_mac(NQ - 2, [13, 15]), orders=ORDA, mix=SHA)
        send_pair(NQ - 2)

        deliver.extend([
            lambda: (oa_copy(pl.ds(0, S), pl.ds((NC - 1) * T, T)).start(),
                     oa_copy(pl.ds(S - 2 * CB, CB), first).start()),
            lambda: oa_copy(pl.ds(S - CB, CB), first).start(),
            lambda: ob_copy(pl.ds(3 * L - T, T)).start()])
        with _scope("seg3e"):
            pair_step(3, NQ - 1, stages=('SV', 'V'), mac=[], orders=ORDB,
                      inverse=[[(b, NC - 1) for b in range(NB)], []])

    if ONLY == 'E':
        epilogue()
        return
    if ONLY:
        for k in range(NB):
            zero_s[k] = 0
        with _scope('loop'):
            if 'quad' in OPT:
                lax.fori_loop(0, 2, lambda j, _: [pair_step(int(ONLY), 2 * j + r, mac=last_mac(2 * j + r) if ONLY == '3' else None) for r in range(2)] and None, None)
            else:
              lax.fori_loop(0, NQ, lambda j, _: pair_step(int(ONLY), j, mac=last_mac(j) if ONLY == '3' else None), None)

        def fin(i, _):
            z = (y_s[i, i, 0:16, :].astype(F32) + yl_s[i, 0:16, :] + ot0_s[i, 0:16, :] + ot1_s[i, 0:16, :] + mem_s[i, 0:16, :]
                 + xg_s[i, i, 0:16, :] + meml_s[i, 0:16, :] + kv_s[0, i, 0:16, :] + p0_s[pl.ds(i * 16, 16), :] + p1_s[pl.ds(i * 16, 16), :] + s_s[pl.ds(i * 16, 16), :])
            for tag, fn in dict(aq=lambda: q_v[0:16, 0:T], ak=lambda: k_v[0:16, 0:T], av=lambda: v_v[0:16, 0:T], ah=lambda: h_v[i, 0:16, 0:T],
                                aw=lambda: w_v[0, i, 0:16, :], ad=lambda: dft_s[i, 0:16, :], af=lambda: kf_s[0, 0, 0:1, :], ag=lambda: gate_s[0:16, :],
                                a1=lambda: shift_ref[0:1, 0:T].astype(F32), a2=lambda: dft_s[i, 0:16, :],
                                a3=lambda: beta_ref[0:1].astype(F32).reshape(1, 1)).items():
                if tag in OPT.split(',') or 'alive' in OPT:
                    z = z + fn()
            outa_s[0:16, 0:T] = z.astype(BF)
            cp = pltpu.make_async_copy(outa_s, out_hbm.at[:, pl.ds(0, D)], sem_q); cp.start(); cp.wait()
            cp = pltpu.make_async_copy(outb_s, out_hbm.at[:, pl.ds(D, D)], sem_q); cp.start(); cp.wait()
        lax.fori_loop(0, 4, fin, None)
        return

    for i in range(3):
        w_copy(i, 0).start()
    const_copy(0).start()
    with _scope("setup"):
        for c in range(NC):
            x_copy(c, 0, 1).start()
        key, lane = _iota((T // 2, T), 0), _iota((T // 2, T), 1)
        for b, query in enumerate((lane, lane ^ (T // 2), lane & (T // 2 - 1))):
            bias_s[b] = jnp.where(key > query, -1e9 * LOG2E, 0.0).astype(F32)
        kf_s[...] = jnp.zeros(kf_s.shape, F32)
        for k in range(NB):
            zero_s[k] = 0
        const_copy(0).wait()
        g = jax.nn.sigmoid(beta_ref[...].astype(F32).reshape(1, H))
        rr = _iota((D, H), 0)
        hh = _iota((D, H), 1) * DH
        gate = jnp.sum(jnp.where((rr >= hh) & (rr < hh + DH), g, 0.0), axis=1, keepdims=True)
        gate_s[...] = jnp.broadcast_to(gate, (D, T))
    with _scope("w0"):
        for i in range(3):
            w_copy(i, 0).wait()
        for i in range(3):
            w_copy(i, 1).start()
    with _scope("t0"):
        transpose_weights(0)
    with _scope("x0"):
        for c in range(NC):
            x_copy(c, 0, 1).wait()
        for i in range(3):
            w_copy(i, 2).start()
    with _scope("p0"):
        for _ in project(0, 0, 0, need_q=False):
            pass
    with _scope("w1"):
        for i in range(3):
            w_copy(i, 1).wait()
        for i in range(3):
            w_copy(i, 3).start()
        const_copy(1).start()
        const_copy(3).start()
    with _scope("p1"):
        transpose_weights(1)

        def fetch_conv():
            for cp in conv_copies(0):
                cp.start()
            if True:
                return
            for t in (2, 3):
                for i in range(3):
                    w_copy(i, t).wait()
            for t in (2, 3):
                transpose_weights(t)
        step(-2, 0, 0, PRO1.split(), (0, 0), stages='PQ', need_q=False, arrive=fetch_conv)
        if True:
            for t in (2, 3):
                for i in range(3):
                    w_copy(i, t).wait()
            for t in (2, 3):
                transpose_weights(t)
        step(-1, 1, 0, PRO.split(), (0, 0), stages='PQS', need_q=False)
    with _scope('aw'):
        const_copy(1).wait()
        const_copy(3).wait()
        for cp in conv_copies(0):
            cp.wait()
    for i in range(3):
        w_copy(i, 4).start()
    for c in range(NC):
        x_copy(c, 1, 1).start()

    def seg0(j, _):
        @pl.when(j == 1)
        def _():
            for i in range(3):
                w_copy(i, 4).wait()
            for c in range(NC):
                x_copy(c, 1, 1).wait()
            for c in range(NC):
                wo_copy(c).start()
                x_copy(c, 2, 2).start()
            const_copy(2).start()
            transpose_weights(4)

        for cp in conv_copies(j + 1):
            cp.start()
        pair_step(0, j)
        for cp in conv_copies(j + 1):
            cp.wait()
    with _scope("seg0"):
        lax.fori_loop(0, NQ, seg0, None)

    const_copy(2).wait()
    const_copy(4).start()
    for c in range(NC):
        wo_copy(c).wait()
        x_copy(c, 2, 2).wait()

    with _scope("seg1"):
        lax.fori_loop(0, NQ, lambda j, _: pair_step(1, j), None)
    ob_copy(pl.ds(0, L)).start()
    q_copy().start()
    with _scope("seg2"):
        lax.fori_loop(0, NQ, lambda j, _: pair_step(2, j), None)
    ob_copy(pl.ds(L, L)).start()
    q_copy().wait()
    const_copy(4).wait()

    with _scope("seg3"):
        def seg3(j, _):
            pair_step(3, j, mac=last_mac(j))
            send_pair(j)
        lax.fori_loop(0, NQ - 2, seg3, None)
    epilogue()

    with _scope('wa'):
        oa_copy(pl.ds(0, S), pl.ds(0, D)).wait()
    with _scope('wb'):
        ob_copy(pl.ds(0, S)).wait()


@jax.jit
def pallas_concat_heads__ssm_conv_h3__memory_aug_infini_attn__prompt_kernel(
    A_q, A_k, A_v, A_shift_k, A_ssm_k, A_ssm_D, B_x, B_wq, B_wk, B_wv, B_wo, B_beta,
):
    hbm = pl.BlockSpec(memory_space=pl.ANY)
    dma = pltpu.SemaphoreType.DMA
    out = pl.pallas_call(
        _kernel,
        out_shape=jax.ShapeDtypeStruct((S, 2 * D), BF),
        in_specs=[hbm] * 13,
        out_specs=hbm,
        scratch_shapes=[
            pltpu.VMEM((S, D), BF),
            pltpu.VMEM((S + L + 64, D), BF),
            pltpu.VMEM((S + L, D), BF),
            pltpu.VMEM((NQ + 1, D, L), BF),
            pltpu.VMEM((NC, S, T), BF),
            pltpu.VMEM((3, NC, D, T), BF),
            pltpu.VMEM((NC, D, T), BF),
            pltpu.VMEM((NC, 3, NQ * WPAIR // 2, T), jnp.uint32),
            pltpu.VMEM((6, T, T), jnp.uint32),
            pltpu.VMEM((NC + 1, 2, 8, T), F32),
            pltpu.VMEM((2, NC, CB, T), BF),
            pltpu.VMEM((2 * NC + 1, NB, 2 * CB, T), F32),
            pltpu.VMEM((NC - 1, NB, 2 * CB, T), BF),
            pltpu.VMEM((NB, 2 * CB, T), BF),
            pltpu.VMEM((S, D), BF),
            pltpu.VMEM((S, D), BF),
            pltpu.VMEM((NQ, D, T), BF),
            pltpu.VMEM((NQ, D, T), BF),
            pltpu.VMEM((NU, UD + 16, T), F32),
            pltpu.VMEM((NU, UD + 16, T), BF),
            pltpu.VMEM((D, T), F32),
            pltpu.VMEM((3, T // 2, T), F32),
            pltpu.VMEM((L, T), BF),
            pltpu.VMEM((NQ, UH + 2, T // 2, T), jnp.uint32),
            *[pltpu.VMEM((2, NQ, UD, T), BF)] * 6,
            *[pltpu.VMEM((2, UH, NQ, 32, T), BF)] * 2,
            pltpu.VMEM((40 * T, T), F32),
            *[pltpu.VMEM((40 * T, T), BF)] * 2,
            pltpu.VMEM((NQ, UH + 2, 8, T), F32),
            pltpu.VMEM((UD, L), F32),
            pltpu.VMEM((NQ, 3 * UD, T), F32),
            pltpu.VMEM((4, D), BF),
            pltpu.VMEM((D,), BF),
            pltpu.VMEM((H,), BF),
            pltpu.SMEM((NB,), jnp.int32),
            dma((4 * NC,)), dma((NSEG * NC,)), dma((3 * (NQ + 1),)), dma(()),
            dma((5,)), dma(()), dma(()),
        ],
        compiler_params=pltpu.CompilerParams(
            vmem_limit_bytes=100 * 1024 * 1024,
            flags=({'XLA_TPU_EVENLY_DISTRIBUTE_CRITICAL_NODES': True} if 'EV' in OPT else None)),
        name="h3_infini",
    )(A_q.reshape(S, D), A_k.reshape(S, D), A_v.reshape(S, D), A_shift_k.T, A_ssm_k, A_ssm_D,
      B_x.reshape(S, D), B_wq, B_wk, B_wv, B_wo, B_beta, _DFT)
    return out.reshape(1, S, 2 * D)
```

```python
import math, os

import numpy as np
import jax
import jax.numpy as jnp
from jax import lax
from jax.experimental import pallas as pl
from jax.experimental.pallas import tpu as pltpu

OPT = os.environ.get('OPT', '')
ONLY = os.environ.get('ONLY', '')
ENV = os.environ.get

S, D = 2048, 640
H, DH, NSEG, L = 32, 20, 4, 512
T = 128
NC = D // T
CB = 2 * T
NB = S // CB
NF = T // 8
NQ = L // T
UH = 4
UD = UH * DH
NU = H // UH
UR = L // NU
WPAIR = 192
BF, F32 = jnp.bfloat16, jnp.float32
LOG2E = math.log2(math.e)


def _dft_matrices():
    m = np.arange(T)[:, None]
    r = np.arange(T)[None, :]

    def rows(power):
        ang = np.pi * np.mod((4 * m + 1) * power, 1024) / 512
        f = np.stack([np.cos(ang).reshape(NF, 8, T), -np.sin(ang).reshape(NF, 8, T)], 1)
        return f.reshape(2 * T, T)

    even, odd = rows(2 * r), rows(2 * r + 1)
    lane = np.arange(T)
    even_h = even[:, lane // 2 + (T // 2) * (lane % 2)]
    odd_h = odd[:, lane // 2 + (T // 2) * (1 - lane % 2)]
    inverse = [np.concatenate([f[:T].T, f[T:].T]) / (2 * T) for f in (even, odd)]
    bits = np.stack([even, odd, even_h, odd_h] + inverse).astype(np.float32).astype(BF)
    bits = bits.view(np.uint16).astype(np.uint32)
    return bits[:, 0::2] | (bits[:, 1::2] << 16)


_DFT = _dft_matrices()


def _pack(x):
    return pltpu.bitcast(x, jnp.uint32)


def _unpack(w):
    return pltpu.bitcast(w, BF)


def _halves(x):
    w = pltpu.bitcast(x, jnp.uint32)
    return (lax.bitcast_convert_type(w << 16, F32),
            lax.bitcast_convert_type(w & np.uint32(0xFFFF0000), F32))


def _interleave(even, odd):
    e, o = (lax.bitcast_convert_type(v.astype(BF).astype(F32), jnp.uint32) for v in (even, odd))
    return pltpu.bitcast((e >> 16) | o, BF)


import contextlib


def _scope(name):
    return jax.named_scope(name) if 'scope' in OPT else contextlib.nullcontext()


def _dot(a, b):
    return jnp.dot(a, b, preferred_element_type=F32)


def _dot_nt(a, b):
    return lax.dot_general(a, b, (((1,), (1,)), ((), ())), preferred_element_type=F32)


def _phi(t):
    return jnp.where(t > 0, t + 1.0, jnp.exp(t))


def _iota(shape, dim):
    return lax.broadcasted_iota(jnp.int32, shape, dim)


def _head_of(z):
    return sum((z >= DH * i).astype(jnp.int32) for i in range(1, UH))


def _kernel(q_hbm, k_hbm, v_hbm, shift_hbm, h_hbm, d_hbm, x_hbm, wq_hbm, wk_hbm, wv_hbm,
            wo_hbm, beta_hbm, dft_hbm, out_hbm,
            q_v, k_v, v_v, h_v, x_v, w_v, wo_v, wt_s, dft_s, kf_s, kv_s, xg_s, y_s, yl_s,
            outa_s, outb_s, ot0_s, ot1_s, mem_s, meml_s, gate_s, bias_s,
            kn_s, rq_s, pk0_s, pk1_s, pq0_s, pq1_s, vt0_s, vt1_s, va0_s, va1_s, s_s, p0_s, p1_s, m_s, ret_s, e_s, shift_ref, d_ref, beta_ref, zero_s,
            sem_w, sem_x, sem_a, sem_q, sem_c, sem_oa, sem_ob):
    ot_s = (ot0_s, ot1_s)
    pk_s, pq_s, vt_s = (pk0_s, pk1_s), (pq0_s, pq1_s), (vt0_s, vt1_s)
    va_s, p_s = (va0_s, va1_s), (p0_s, p1_s)

    def y_of(c):
        return yl_s if c == NC - 1 else y_s.at[c]

    def w_copy(i, t):
        cols = pl.ds(t * T, T)
        return pltpu.make_async_copy((wq_hbm, wk_hbm, wv_hbm)[i].at[:, cols], w_v.at[i, t],
                                     sem_w.at[i * NC + t])

    def wo_copy():
        return pltpu.make_async_copy(wo_hbm, wo_v, sem_w.at[3 * NC])

    def x_copy(first, count):
        rows = pl.ds(first * L, count * L)
        return pltpu.make_async_copy(x_hbm.at[rows], x_v.at[rows], sem_x.at[first])

    def conv_copies(j):
        src = pl.ds(pl.multiple_of(jnp.minimum(j, NQ - 1) * L, L), L)
        dst = pl.ds(pl.multiple_of(j * L, L), L)
        return (pltpu.make_async_copy(k_hbm.at[src], k_v.at[dst], sem_a.at[3 * j]),
                pltpu.make_async_copy(v_hbm.at[src], v_v.at[dst], sem_a.at[3 * j + 1]),
                pltpu.make_async_copy(h_hbm.at[:, src], h_v.at[j], sem_a.at[3 * j + 2]))

    def q_copy():
        return pltpu.make_async_copy(q_hbm, q_v, sem_q)

    def const_copy(i):
        src, dst = ((beta_hbm, beta_ref), (shift_hbm, shift_ref), (d_hbm, d_ref),
                    (dft_hbm.at[0:4], dft_s.at[0:4]), (dft_hbm.at[4:6], dft_s.at[4:6]))[i]
        return pltpu.make_async_copy(src, dst, sem_c.at[i])

    def oa_copy(rows, lanes):
        return pltpu.make_async_copy(outa_s.at[rows, lanes], out_hbm.at[rows, lanes], sem_oa)

    def ob_copy(rows):
        return pltpu.make_async_copy(outb_s.at[rows], out_hbm.at[rows, pl.ds(D, D)], sem_ob)

    self_done = []

    def gate_kv(u, half):
        src = pl.multiple_of(u * CB, CB)
        for c in range(NC):
            lanes = slice(c * T, (c + 1) * T)
            taps = [shift_ref[t:t + 1, lanes].astype(F32) for t in range(4)]
            pe, po = kf_s[c, 0], kf_s[c, 1]
            for r in range(0, T, 16):
                rows = pl.ds(pl.multiple_of(src + 2 * r, 32), 32)
                ke, ko = _halves(k_v[rows, lanes])
                ve, vo = _halves(v_v[rows, lanes])
                e1 = pltpu.roll(jnp.concatenate([pe, ke], axis=0), 1, 0)[8:24]
                odd = jnp.concatenate([po, ko], axis=0)
                o1, o2 = pltpu.roll(odd, 1, 0)[8:24], pltpu.roll(odd, 2, 0)[8:24]
                se = ke * taps[0] + o1 * taps[1] + e1 * taps[2] + o2 * taps[3]
                so = ko * taps[0] + ke * taps[1] + o1 * taps[2] + e1 * taps[3]
                kv_s[half, c, r:r + 16, :] = (se * ve).astype(BF)
                kv_s[half, c, T + r:T + r + 16, :] = (so * vo).astype(BF)
                pe, po = ke[8:16], ko[8:16]
                yield 1
            kf_s[c, 0] = pe
            kf_s[c, 1] = po
            self_done.append((half, c))

    def conv_forward(u, half, c):
        lanes = slice(c * T, (c + 1) * T)
        h0, h1 = (pltpu.bitcast(h_v[u // 2, lanes, (2 * half + j) * T:(2 * half + j + 1) * T], jnp.uint32)
                  for j in range(2))
        even = (_iota(h0.shape, 1) & 1) == 0
        he = pltpu.bitcast(jnp.where(even, h0, pltpu.roll(h1, 1, 1)), BF)
        ho = pltpu.bitcast(jnp.where(even, pltpu.roll(h1, T - 1, 1), h0), BF)
        for base, a, b in (
                (c, _dot(_unpack(dft_s[0]), kv_s[half, c, 0:T, :]),
                 _dot(_unpack(dft_s[1]), kv_s[half, c, T:CB, :])),
                (NC + c, _dot_nt(_unpack(dft_s[2]), he), _dot_nt(_unpack(dft_s[3]), ho))):
            xg_s[base, u, 0:CB, :] = a + b
            xg_s[base, u, CB:2 * CB, :] = a - b

    def conv_mac(items, w=2):
        skip = {c: jnp.broadcast_to(d_row(c), (8, T)) for c, _ in items}
        for c, f in items:
            for k in range(NB // w):
                outs = range(k * w, (k + 1) * w)
                r0 = pl.multiple_of((f + zero_s[k]) * 16, 16)
                plus = {}
                for sign in range(2):
                    re = pl.ds(pl.multiple_of(r0 + sign * CB, 8), 8)
                    im = pl.ds(pl.multiple_of(r0 + sign * CB + 8, 8), 8)
                    acc, g, h = {}, {}, {}

                    def filt(n):
                        if n not in g:
                            for m in (n, n - 1):
                                if m >= 0 and m not in h:
                                    h[m] = (xg_s[NC + c, m, re, :], xg_s[NC + c, m, im, :])
                            if n == 0:
                                g[n] = (h[0][0] + skip[c], h[0][1])
                            else:
                                g[n] = (h[n][0] - h[n - 1][1], h[n][1] + h[n - 1][0])
                        return g[n]

                    for b in range(max(outs) + 1):
                        xr, xi = xg_s[c, b, re, :], xg_s[c, b, im, :]
                        cost = 0
                        for a in outs:
                            if b > a:
                                continue
                            gr, gi = filt(a - b)
                            p = (xr * gr - xi * gi, xr * gi + xi * gr)
                            acc[a] = p if a not in acc else (acc[a][0] + p[0], acc[a][1] + p[1])
                            cost += 1
                            if a == b and sign == 0:
                                plus[a] = jnp.concatenate(acc[a], axis=0)
                            elif a == b:
                                minus = jnp.concatenate(acc[a], axis=0)
                                y_of(c)[a, pl.ds(r0, 16), :] = (plus[a] + minus).astype(BF)
                                y_of(c)[a, pl.ds(pl.multiple_of(r0 + CB, 16), 16), :] = (
                                    plus[a] - minus).astype(BF)
                        yield cost

    class Filler:
        def __init__(self):
            self.gen, self.credit, self.in_k = None, 0.0, False

        def pin(self, value, amount):
            if self.gen is None or amount == 0:
                return
            if self.in_k:
                k_v[S + L:S + L + 16, 0:T] = jnp.concatenate([value, value], axis=0).astype(BF)
            else:
                xg_s[2 * NC, 0, 0:8, :] = value
            self.credit += amount
            while self.gen is not None and self.credit > 0:
                cost = next(self.gen, None)
                if cost is None:
                    self.gen = None
                else:
                    self.credit -= cost

        def drain(self):
            if self.gen is not None:
                for _ in self.gen:
                    pass
            self.gen = None

    filler = Filler()

    def conv_inverse(u, c):
        r0 = pl.multiple_of(u * CB, CB)
        lanes = slice(c * T, (c + 1) * T)
        qs = _halves(q_v[pl.ds(r0, CB), lanes])
        out = []
        for j in range(2):
            inv = jnp.concatenate([_unpack(dft_s[4 + j, 0:T // 2, :]),
                                   _unpack(dft_s[4 + j, T // 2:T, :])], axis=1)
            y = _dot(inv, y_of(c)[u, j * CB:(j + 1) * CB, :])
            out.append(qs[j] * y)
        outa_s[pl.ds(r0, CB), lanes] = _interleave(*out)

    def out_proj(o, rows, amount):
        m = o[0].shape[0]
        last = NC - 1
        head = jnp.concatenate(o[0:last], axis=1)

        def pin(part):
            for r in range(0, m, 32):
                filler.pin(part[r:r + 8, 0:T], amount * 32 / (6 * m))

        edge = _dot(o[last], wo_v[last * T:D, 0:last * T])
        pin(edge)
        yield
        corner = _dot(o[last], wo_v[last * T:D, last * T:D])
        for n in reversed(range(NC)):
            part = _dot(head, wo_v[0:last * T, n * T:(n + 1) * T])
            pin(part)
            part = part + (corner if n == last else edge[:, n * T:(n + 1) * T])
            outb_s[rows, n * T:(n + 1) * T] = part.astype(BF)
            yield

    def own_rows(x, i, fill):
        low4 = _iota((8, T), 0) < 4
        full = jnp.full((8, T), fill, F32)
        g0 = 5 * (i // 2)
        if i % 2 == 0:
            body = [x[8 * g0:8 * g0 + 16], jnp.where(low4, x[8 * g0 + 16:8 * g0 + 24], fill)]
        else:
            body = [jnp.where(low4, fill, x[8 * g0 + 16:8 * g0 + 24]), x[8 * g0 + 24:8 * g0 + 40]]
        return jnp.concatenate(body + [full] if i < 2 else [full] + body, axis=0).astype(BF)

    def project(n, par, amount, need_q=True, need_k=True):
        s, u = n // NU, n % NU
        w0 = pl.multiple_of((u // 2) * (WPAIR // 2), 32) + par * (UD // 2)
        x0 = pl.multiple_of(s * L, L)
        slot = (n // 2) % 2
        pad = jnp.zeros((T - UD, T), F32)

        def finish(j, qkv):
            cols = slice(j * T, (j + 1) * T)
            qt, kt, vt = qkv[0:UD], qkv[UD:2 * UD], qkv[2 * UD:3 * UD]
            kn_s[cols, :] = jnp.concatenate([kt, pad], axis=0).T.astype(BF)
            qs = qt * (DH ** -0.5 * LOG2E)
            low4 = _iota((8, T), 0) < 4
            left = _iota((8, T), 1) < T // 2
            zero = jnp.zeros((8, T), F32)
            for pr in range(UH // 2):
                qa = [qs[40 * pr + 8 * r:40 * pr + 8 * r + 8] for r in range(3)]
                qb = [pltpu.roll(qs[40 * pr + 8 * r:40 * pr + 8 * r + 8], T // 2, 1) for r in (2, 3, 4)]
                ra = [qa[0], qa[1], jnp.where(low4, qa[2], 0.0)]
                rb = [jnp.where(low4, 0.0, qb[0]), qb[1], qb[2]]
                rh = [jnp.where(left, 0.0, qa[0]), jnp.where(left, 0.0, qa[1]),
                      jnp.where(left, rb[0], ra[2]),
                      jnp.where(left, qb[1], 0.0), jnp.where(left, qb[2], 0.0)]
                for i, rows in ((2 * pr, ra), (2 * pr + 1, rb)):
                    rows = rows + [zero] if pr == 0 else [zero] + rows
                    rq_s[j, i, 8 * i:8 * i + 16, :] = _pack(jnp.concatenate(rows, axis=0).astype(BF))
                rows = rh + [zero] if pr == 0 else [zero] + rh
                rq_s[j, UH + pr, 16 * pr:16 * pr + 24, :] = _pack(
                    jnp.concatenate(rows, axis=0).astype(BF))
            for i in range(UH):
                va_s[par][slot, i, j] = own_rows(vt, i, 1.0)
            if need_q:
                pq_s[par][slot, j] = _phi(qt).astype(BF)
            if need_k:
                pk_s[par][slot, j] = _phi(kt).astype(BF)
                vt_s[par][slot, j] = vt.astype(BF)

        w = [_unpack(jnp.concatenate(
            [wt_s[c, i, pl.ds(pl.multiple_of(w0, 8), UD // 2), :] for i in range(3)], axis=0))
             for c in range(NC)]
        part = _dot_nt(w[NC - 1], x_v[pl.ds(x0, L), (NC - 1) * T:D])
        for j in range(NQ):
            e_s[j] = part[:, j * T:(j + 1) * T]
        for r in range(0, 3 * UD, 24):
            filler.pin(part[r:r + 8, 0:T], amount / (10 * NC))
        yield
        w = jnp.concatenate(w[0:NC - 1], axis=1)
        for j in reversed(range(NQ)):
            rows = pl.ds(pl.multiple_of(x0 + j * T, T), T)
            part = _dot_nt(w, x_v[rows, 0:(NC - 1) * T])
            for r in range(0, 3 * UD, 24):
                filler.pin(part[r:r + 8], amount / (10 * NC))
            finish(j, part + e_s[j])
            yield

    HALF = T // 2

    def s_off(j, i, t, n=T):
        return pl.ds((2 * j * (j + 1) + i * (j + 1) + t) * T, n)

    def hi_off(j, pr):
        return pl.ds((2 * j * (j + 1) + 2 * pr * (j + 1) + j) * T + HALF, HALF)

    def sparse(j, i, first, count):
        parts = [_unpack(rq_s[j, i, first // 2:(first + count) // 2, :]),
                 jnp.zeros((T - first - count, T), BF)]
        if first:
            parts.insert(0, jnp.zeros((first, T), BF))
        return jnp.concatenate(parts, axis=0)

    def col_max(x):
        return jnp.max(x.reshape(x.shape[0] // 8, 8, T), axis=0)

    def scores(j, t, top, amount):
        rq = jnp.concatenate([sparse(j, i, i // 1 * 16, 32) for i in range(UH)], axis=1)
        n = T if t < j else HALF
        sc = _dot(kn_s[t * T:t * T + n, :], rq)
        if t == j:
            rh = jnp.concatenate([sparse(j, UH + pr, 32 * pr, 48) for pr in range(2)], axis=1)
            hi = _dot(kn_s[t * T + HALF:(t + 1) * T, :], rh)
        for i in range(UH):
            si = sc[:, i * T:(i + 1) * T]
            if t == j:
                si = si + bias_s[i % 2]
            s_s[s_off(j, i, t, n), :] = si
            if i == 0:
                for r in range(0, n, 32):
                    filler.pin(si[r:r + 8], amount * 32 / n)
            top[i] = col_max(si) if t == 0 else jnp.maximum(top[i], col_max(si))
        if t < j:
            return
        left = _iota((8, T), 1) < HALF
        for pr in range(2):
            si = hi[:, pr * T:(pr + 1) * T] + bias_s[2]
            s_s[hi_off(j, pr), :] = si
            mh = col_max(si)
            ma = jnp.maximum(top[2 * pr], jnp.where(left, -jnp.inf, mh))
            mb = jnp.maximum(top[2 * pr + 1], jnp.where(left, mh, -jnp.inf))
            ma = jnp.broadcast_to(jnp.max(ma, axis=0, keepdims=True), (8, T))
            mb = jnp.broadcast_to(jnp.max(mb, axis=0, keepdims=True), (8, T))
            m_s[j, 2 * pr] = ma
            m_s[j, 2 * pr + 1] = mb
            m_s[j, UH + pr] = jnp.where(left, mb, ma)

    def weights(rows, j, i):
        sc = s_s[rows, :]
        m = jnp.concatenate([m_s[j, i]] * (sc.shape[0] // 8), axis=0)
        return jnp.exp2(sc - m).astype(BF)

    def softmax(par, j, t):
        n = T if t < j else HALF
        for i in range(UH):
            p_s[par][s_off(j, i, t, n), :] = weights(s_off(j, i, t, n), j, i)
        if t < j:
            return
        left = _iota((HALF // 2, T), 1) < HALF
        none = jnp.zeros((HALF // 2, T), jnp.uint32)
        for pr in range(2):
            p = pltpu.bitcast(weights(hi_off(j, pr), j, UH + pr), jnp.uint32)
            for i, part in ((2 * pr, jnp.where(left, none, p)), (2 * pr + 1, jnp.where(left, p, none))):
                p_s[par][pl.ds(s_off(j, i, t).start + HALF, HALF), :] = pltpu.bitcast(part, BF)

    def spread(a, b):
        low4 = _iota(a.shape, 0) < 4
        ar, br = pltpu.roll(a, 4, 0), pltpu.roll(b, 4, 0)
        r0, r1 = jnp.where(low4, a, ar), jnp.where(low4, ar, a)
        r2, r3 = jnp.where(low4, b, br), jnp.where(low4, br, b)
        return jnp.concatenate([r0, r0, a, r1, r1, r2, r2, b, r3, r3], axis=0)

    def retrieve(n, par):
        u, slot = n % NU, (n // 2) % 2
        zpad = jnp.zeros((T - UD, T), BF)
        pq = jnp.concatenate(
            [jnp.concatenate([pq_s[par][slot, j], zpad], axis=0) for j in range(NQ)], axis=1)
        ret = _dot(meml_s[u], pq)
        rd = 1.0 / (ret[UD:UD + 16] + 1e-6)
        ret_s[...] = ret[0:UD] * spread(rd[0:8], rd[8:16])

    def update(n, par, s):
        u, slot = n % NU, (n // 2) % 2
        zpad = jnp.zeros((T - UD, T), BF)
        va = jnp.concatenate(
            [jnp.concatenate([vt_s[par][slot, j], jnp.ones((16, T), BF)], axis=0) for j in range(NQ)],
            axis=1)
        pk = jnp.concatenate(
            [jnp.concatenate([pk_s[par][slot, j], zpad], axis=0) for j in range(NQ)], axis=1)
        mem = _dot_nt(va, pk)
        if s > 0:
            mem = mem_s[u] + mem
        if s < NSEG - 2:
            mem_s[u] = mem
        row = _iota((UD + 16, T), 0)
        row_head = jnp.where(row < UD, _head_of(row), (row - UD) >> 2)
        meml_s[u] = jnp.where(row_head == _head_of(_iota((UD + 16, T), 1)), mem, 0.0).astype(BF)

    def values(n, par, s, j, t, acc):
        u, slot = n % NU, (n // 2) % 2
        for i in range(UH):
            part = _dot(va_s[par][slot, i, t], p_s[par][s_off(j, i, t), :])
            acc[i] = part if t == 0 else acc[i] + part
        if t < j:
            return
        heads = []
        for i in range(UH):
            den = acc[i][24:32] if i < 2 else acc[i][0:8]
            val = acc[i][0:24] if i < 2 else acc[i][8:32]
            val = val * jnp.concatenate([1.0 / den] * 3, axis=0)
            heads.append(pltpu.roll(val, HALF, 1) if i % 2 else val)
        low4 = _iota((8, T), 0) < 4
        att = jnp.concatenate([
            heads[0][0:16], jnp.where(low4, heads[0][16:24], heads[1][0:8]), heads[1][8:24],
            heads[2][0:16], jnp.where(low4, heads[2][16:24], heads[3][0:8]), heads[3][8:24]], axis=0)
        rows = pl.ds(pl.multiple_of(u * UD, 16), UD)
        gt = gate_s[rows, :]
        o = (1.0 - gt) * att
        if s > 0:
            o = o + gt * ret_s[:, j * T:(j + 1) * T]
        o = o.astype(BF)
        ot_s[s % 2][j, rows, :] = o

    ORDERS = [
        ENV('ORD0', 'Q30 V30 Q31 V31 P Q32 V32 Q33 V33 P X U Q20 Q21 V20 X V21 Q22 V22 P Q10 V10 Q11 X V11 V00 P X Q00 P X / Q30 P V30 V31 Q31 Q32 Q33 X V32 V33 X U P Q20 X Q21 V20 V21 Q22 V22 P Q10 V10 X Q11 X V00 P V11 Q00 P'),
        ENV('ORD1', 'R P Q30 Q31 V30 V31 Q32 V32 Q33 U V33 P Q20 V20 O Q21 V21 Q22 V22 P O Q10 Q11 V10 V11 V00 Q00 P P O / V30 P R Q30 Q31 V31 Q32 V32 V20 Q33 V33 Q20 U P Q21 Q22 Q10 V10 Q11 V21 V22 Q00 P O P P V11 V00 O O'),
        ENV('ORD1', 'R P Q30 Q31 V30 V31 Q32 V32 Q33 U V33 P Q20 V20 O Q21 V21 Q22 V22 P O Q10 Q11 V10 V11 V00 Q00 P P O / V30 P R Q30 Q31 V31 Q32 V32 V20 Q33 V33 Q20 U P Q21 Q22 Q10 V10 Q11 V21 V22 Q00 P O P P V11 V00 O O'),
        ENV('ORD3', 'R P Q30 V30 Q31 V31 X V32 V33 Q32 Q33 P X X Q20 V20 Q21 V21 Q22 V22 P Q10 V10 X Q11 V11 O P Q00 P V00 / P R Q30 V30 X Q31 V31 V32 X Q32 Q33 V33 P Q20 V20 V21 Q21 V22 Q22 Q10 V10 X Q11 V11 X P Q00 P O O P V00 O O O'),
    ]
    ORDA = ENV('ORDA', 'R P Q30 V30 V31 Q31 X V32 Q32 Q33 V33 P X Q20 V20 Q21 V21 X Q22 V22 P Q10 V10 Q11 X V11 O P Q00 P V00 / P Q30 V30 Q31 V31 R X V32 Q32 Q33 V33 P X Q20 V20 Q21 O V21 X V22 Q22 Q10 V10 O Q11 V11 X P P Q00 P O V00 O O')
    ORDB = ENV('ORDB', 'R X X X Q30 V30 X Q31 V31 X V32 Q32 X Q33 X Q20 X V20 V33 Q21 V21 X V22 Q22 X Q10 X V10 X Q11 V11 Q00 V00 / R D X V30 V31 X V32 V33 X V20 V21 X V22 O O D O V10 V11 V00 O O O D T3 T3 T3 T3 T3 T3 T2 T2 T2 T2 T1 T2 T1 T1 T1 T2 T1 T1 T0 T0 T0 T0 T0 T0')
    ORDA, ORDB = ([half.split() for half in order.split('/')] for order in (ORDA, ORDB))
    SHA = [float(v) for v in ENV('SHA', '0.6,0.35,0.05').split(',')]
    PRO1 = ENV('PRO1', 'Q30 Q31 Q32 Q33 P P Q20 Q21 W Q22 P Q10 Q11 P Q00 P')
    PRO = ENV('PRO', 'P Q30 Q31 Q32 Q33 P Q20 Q21 Q22 P Q10 Q11 P Q00 P')
    ORDERS = [[half.split() for half in order.split('/')] for order in ORDERS]
    SHARE = [[float(v) for v in ENV(k, d).split(',')] for k, d in
             (('SH0', '0.5,0.8,0.0'), ('SH1', '0.1,0.6,0.3'), ('SH1', '0.1,0.6,0.3'), ('SH3', '0.15,0.4,0.45'))]

    deliver = []

    def step(n, par, s, order, share, jobs=(), oproj=None, stages='PQSV', need_q=True, arrive=None):
        jobs = list(jobs)
        proj = project(n + 3, 1 - par, share[1], need_q=need_q, need_k=s < NSEG - 1)
        top, acc, final = [None] * UH, {}, {}
        for tok in order:
            if tok[0] == 'Q':
                j, t = int(tok[1]), int(tok[2])
                if 'S' in stages:
                    softmax(1 - par, j, t)
                if 'Q' in stages:
                    scores(j, t, top, share[0] / 10)
            elif tok[0] == 'V':
                if 'V' in stages:
                    values(n, par, s, int(tok[1]), int(tok[2]), acc.setdefault(tok[1], [None] * UH))
            elif tok == 'P':
                if 'P' in stages:
                    next(proj)
            elif tok == 'R':
                if 'V' in stages and s > 0:
                    retrieve(n, par)
            elif tok == 'U':
                if 'V' in stages and s < NSEG - 1:
                    update(n, par, s)
            elif tok[0] == 'T':
                j = int(tok[1])
                rows = pl.ds((NSEG - 1) * L + j * T, T)
                if j not in final:
                    final[j] = [out_proj(out_tiles(NSEG - 1, j), rows, 0), 0]
                next(final[j][0])
                final[j][1] += 1
                if final[j][1] == NC + 1:
                    ob_copy(rows).start()
            elif tok == 'D':
                deliver.pop(0)()
            elif tok == 'O':
                if oproj is not None:
                    next(oproj)
            elif tok == 'W':
                if arrive is not None:
                    arrive()
            elif tok == 'X':
                if jobs:
                    jobs.pop(0)()
        assert not jobs

    def out_tiles(s, j):
        return [ot_s[s % 2][j, c * T:(c + 1) * T, :].T for c in range(NC)]

    def pair_step(s, j, stages=('PQSV', 'PQSV'), arrive=None, mac=None, inverse=None, middle=None,
                  orders=None, mix=None):
        orders, mix = orders or ORDERS[s], mix or SHARE[s]
        us = (2 * j, 2 * j + 1)
        share, oproj = [8 * NC * v for v in mix], None
        filler.gen, filler.credit, filler.in_k = None, 0.0, s == 0
        if s == 0:
            del self_done[:]
            filler.gen = (cost for half, u in enumerate(us) for cost in gate_kv(u, half))
            share = [16 * NC * v for v in mix]
        else:
            if mac is None:
                mac = [(c, 4 * j + r) for c in (2 * s - 2, 2 * s - 1) for r in range(4)]
            weight = (mix[0] * sum('Q' in st for st in stages)
                      + mix[1] * sum('P' in st for st in stages) + 2 * mix[2])
            share = [72 * len(mac) * v / weight for v in mix]
            if mac and 'nomac' not in OPT:
                filler.gen = conv_mac(mac, int(ENV('W', '2')))
            rows = pl.ds(pl.multiple_of((s - 1) * L + j * T, T), T)
            oproj = out_proj(out_tiles(s - 1, j), rows, 2 * share[2])
        for half, u in enumerate(us):
            jobs, wait = [], None
            if half == 1 and middle is not None:
                middle()
            if s == 0:
                def forward(u, half, c):
                    while (half, c) not in self_done and filler.gen is not None:
                        if next(filler.gen, None) is None:
                            filler.gen = None
                        filler.credit -= 1
                    conv_forward(u, half, c)
                jobs = [lambda c=c, u=u, half=half: forward(u, half, c) for c in range(NC)]
            elif s == NSEG - 1:
                todo = (inverse[half] if inverse else []) + [(u, c) for c in range(NC - 1)]
                jobs = [lambda b=b, c=c: conv_inverse(b, c) for b, c in todo]
            step(s * NU + u, half, s, orders[half],
                 share, jobs, oproj, stages[half], arrive=wait)
        filler.drain()

    def last_mac(j, extra=None):
        return [(NC - 1, f) for f in [4 * j + r for r in range(4)] + (extra or [12 + 2 * j])]

    def scoped(f, s, j):
        with _scope("it"):
            f(s, j)

    def transpose_weights(t):
        for i in range(3):
            for c in range(NC):
                wt = _pack(w_v[i, t, c * T:(c + 1) * T, :].T)
                for r in range(T // 16):
                    pair, off = divmod(t * T + 16 * r, 2 * UD)
                    row = (pair * WPAIR + off) // 2
                    wt_s[c, i, row:row + 8, :] = wt[8 * r:8 * r + 8]

    def d_row(c):
        return d_ref[...].astype(F32).reshape(1, D)[:, c * T:(c + 1) * T]

    def send_pair(j):
        oa_copy(pl.ds(pl.multiple_of(j * L, L), L), pl.ds(0, (NC - 1) * T)).start()
        ob_copy(pl.ds(pl.multiple_of(2 * L + j * T, T), T)).start()

    def epilogue():
        first = pl.ds(0, (NC - 1) * T)
        with _scope("seg3a"):
            pair_step(3, NQ - 2, stages=('PQSV', 'QSV'), mac=last_mac(NQ - 2, [13, 15]), orders=ORDA, mix=SHA)
        send_pair(NQ - 2)

        deliver.extend([
            lambda: (oa_copy(pl.ds(0, S), pl.ds((NC - 1) * T, T)).start(),
                     oa_copy(pl.ds(S - 2 * CB, CB), first).start()),
            lambda: oa_copy(pl.ds(S - CB, CB), first).start(),
            lambda: ob_copy(pl.ds(3 * L - T, T)).start()])
        with _scope("seg3e"):
            pair_step(3, NQ - 1, stages=('SV', 'V'), mac=[], orders=ORDB,
                      inverse=[[(b, NC - 1) for b in range(NB)], []])

    if ONLY == 'E':
        epilogue()
        return
    if ONLY:
        for k in range(NB):
            zero_s[k] = 0
        with _scope('loop'):
            if 'quad' in OPT:
                lax.fori_loop(0, 2, lambda j, _: [pair_step(int(ONLY), 2 * j + r, mac=last_mac(2 * j + r) if ONLY == '3' else None) for r in range(2)] and None, None)
            else:
              lax.fori_loop(0, NQ, lambda j, _: pair_step(int(ONLY), j, mac=last_mac(j) if ONLY == '3' else None), None)

        def fin(i, _):
            z = (y_s[i, i, 0:16, :].astype(F32) + yl_s[i, 0:16, :] + ot0_s[i, 0:16, :] + ot1_s[i, 0:16, :] + mem_s[i, 0:16, :]
                 + xg_s[i, i, 0:16, :] + meml_s[i, 0:16, :] + kv_s[0, i, 0:16, :] + p0_s[pl.ds(i * 16, 16), :] + p1_s[pl.ds(i * 16, 16), :] + s_s[pl.ds(i * 16, 16), :])
            for tag, fn in dict(aq=lambda: q_v[0:16, 0:T], ak=lambda: k_v[0:16, 0:T], av=lambda: v_v[0:16, 0:T], ah=lambda: h_v[i, 0:16, 0:T],
                                aw=lambda: w_v[0, i, 0:16, :], ad=lambda: dft_s[i, 0:16, :], af=lambda: kf_s[0, 0, 0:1, :], ag=lambda: gate_s[0:16, :],
                                a1=lambda: shift_ref[0:1, 0:T].astype(F32), a2=lambda: dft_s[i, 0:16, :],
                                a3=lambda: beta_ref[0:1].astype(F32).reshape(1, 1)).items():
                if tag in OPT.split(',') or 'alive' in OPT:
                    z = z + fn()
            outa_s[0:16, 0:T] = z.astype(BF)
            cp = pltpu.make_async_copy(outa_s, out_hbm.at[:, pl.ds(0, D)], sem_q); cp.start(); cp.wait()
            cp = pltpu.make_async_copy(outb_s, out_hbm.at[:, pl.ds(D, D)], sem_q); cp.start(); cp.wait()
        lax.fori_loop(0, 4, fin, None)
        return

    for i in range(3):
        w_copy(i, 0).start()
    const_copy(0).start()
    with _scope("setup"):
        x_copy(0, 1).start()
        key, lane = _iota((T // 2, T), 0), _iota((T // 2, T), 1)
        for b, query in enumerate((lane, lane ^ (T // 2), lane & (T // 2 - 1))):
            bias_s[b] = jnp.where(key > query, -1e9 * LOG2E, 0.0).astype(F32)
        kf_s[...] = jnp.zeros(kf_s.shape, F32)
        for k in range(NB):
            zero_s[k] = 0
        const_copy(0).wait()
        g = jax.nn.sigmoid(beta_ref[...].astype(F32).reshape(1, H))
        rr = _iota((D, H), 0)
        hh = _iota((D, H), 1) * DH
        gate = jnp.sum(jnp.where((rr >= hh) & (rr < hh + DH), g, 0.0), axis=1, keepdims=True)
        gate_s[...] = jnp.broadcast_to(gate, (D, T))
    with _scope("w0"):
        for i in range(3):
            w_copy(i, 0).wait()
        for i in range(3):
            w_copy(i, 1).start()
    with _scope("t0"):
        transpose_weights(0)
    with _scope("x0"):
        x_copy(0, 1).wait()
        for i in range(3):
            w_copy(i, 2).start()
    with _scope("p0"):
        for _ in project(0, 0, 0, need_q=False):
            pass
    with _scope("w1"):
        for i in range(3):
            w_copy(i, 1).wait()
        for i in range(3):
            w_copy(i, 3).start()
        const_copy(1).start()
        const_copy(3).start()
    with _scope("p1"):
        transpose_weights(1)

        def fetch_conv():
            for cp in conv_copies(0):
                cp.start()
            if True:
                return
            for t in (2, 3):
                for i in range(3):
                    w_copy(i, t).wait()
            for t in (2, 3):
                transpose_weights(t)
        step(-2, 0, 0, PRO1.split(), (0, 0), stages='PQ', need_q=False, arrive=fetch_conv)
        if True:
            for t in (2, 3):
                for i in range(3):
                    w_copy(i, t).wait()
            for t in (2, 3):
                transpose_weights(t)
        step(-1, 1, 0, PRO.split(), (0, 0), stages='PQS', need_q=False)
    with _scope('aw'):
        const_copy(1).wait()
        const_copy(3).wait()
        for cp in conv_copies(0):
            cp.wait()
    for i in range(3):
        w_copy(i, 4).start()
    x_copy(1, 1).start()

    def seg0(j, _):
        @pl.when(j == 1)
        def _():
            for i in range(3):
                w_copy(i, 4).wait()
            x_copy(1, 1).wait()
            wo_copy().start()
            x_copy(2, 2).start()
            const_copy(2).start()
            transpose_weights(4)

        for cp in conv_copies(j + 1):
            cp.start()
        pair_step(0, j)
        for cp in conv_copies(j + 1):
            cp.wait()
    with _scope("seg0"):
        lax.fori_loop(0, NQ, seg0, None)

    const_copy(2).wait()
    const_copy(4).start()
    wo_copy().wait()
    x_copy(2, 2).wait()

    with _scope("seg1"):
        lax.fori_loop(0, NQ, lambda j, _: pair_step(1, j), None)
    ob_copy(pl.ds(0, L)).start()
    q_copy().start()
    with _scope("seg2"):
        lax.fori_loop(0, NQ, lambda j, _: pair_step(2, j), None)
    ob_copy(pl.ds(L, L)).start()
    q_copy().wait()
    const_copy(4).wait()

    with _scope("seg3"):
        def seg3(j, _):
            pair_step(3, j, mac=last_mac(j))
            send_pair(j)
        lax.fori_loop(0, NQ - 2, seg3, None)
    epilogue()

    with _scope('wa'):
        oa_copy(pl.ds(0, S), pl.ds(0, D)).wait()
    with _scope('wb'):
        ob_copy(pl.ds(0, S)).wait()


@jax.jit
def pallas_concat_heads__ssm_conv_h3__memory_aug_infini_attn__prompt_kernel(
    A_q, A_k, A_v, A_shift_k, A_ssm_k, A_ssm_D, B_x, B_wq, B_wk, B_wv, B_wo, B_beta,
):
    hbm = pl.BlockSpec(memory_space=pl.ANY)
    dma = pltpu.SemaphoreType.DMA
    out = pl.pallas_call(
        _kernel,
        out_shape=jax.ShapeDtypeStruct((S, 2 * D), BF),
        in_specs=[hbm] * 13,
        out_specs=hbm,
        scratch_shapes=[
            pltpu.VMEM((S, D), BF),
            pltpu.VMEM((S + L + 64, D), BF),
            pltpu.VMEM((S + L, D), BF),
            pltpu.VMEM((NQ + 1, D, L), BF),
            pltpu.VMEM((S, D), BF),
            pltpu.VMEM((3, NC, D, T), BF),
            pltpu.VMEM((D, D), BF),
            pltpu.VMEM((NC, 3, NQ * WPAIR // 2, T), jnp.uint32),
            pltpu.VMEM((6, T, T), jnp.uint32),
            pltpu.VMEM((NC + 1, 2, 8, T), F32),
            pltpu.VMEM((2, NC, CB, T), BF),
            pltpu.VMEM((2 * NC + 1, NB, 2 * CB, T), F32),
            pltpu.VMEM((NC - 1, NB, 2 * CB, T), BF),
            pltpu.VMEM((NB, 2 * CB, T), BF),
            pltpu.VMEM((S, D), BF),
            pltpu.VMEM((S, D), BF),
            pltpu.VMEM((NQ, D, T), BF),
            pltpu.VMEM((NQ, D, T), BF),
            pltpu.VMEM((NU, UD + 16, T), F32),
            pltpu.VMEM((NU, UD + 16, T), BF),
            pltpu.VMEM((D, T), F32),
            pltpu.VMEM((3, T // 2, T), F32),
            pltpu.VMEM((L, T), BF),
            pltpu.VMEM((NQ, UH + 2, T // 2, T), jnp.uint32),
            *[pltpu.VMEM((2, NQ, UD, T), BF)] * 6,
            *[pltpu.VMEM((2, UH, NQ, 32, T), BF)] * 2,
            pltpu.VMEM((40 * T, T), F32),
            *[pltpu.VMEM((40 * T, T), BF)] * 2,
            pltpu.VMEM((NQ, UH + 2, 8, T), F32),
            pltpu.VMEM((UD, L), F32),
            pltpu.VMEM((NQ, 3 * UD, T), F32),
            pltpu.VMEM((4, D), BF),
            pltpu.VMEM((D,), BF),
            pltpu.VMEM((H,), BF),
            pltpu.SMEM((NB,), jnp.int32),
            dma((3 * NC + 1,)), dma((3,)), dma((3 * (NQ + 1),)), dma(()),
            dma((5,)), dma(()), dma(()),
        ],
        compiler_params=pltpu.CompilerParams(
            vmem_limit_bytes=100 * 1024 * 1024,
            flags=({'XLA_TPU_EVENLY_DISTRIBUTE_CRITICAL_NODES': True} if 'EV' in OPT else None)),
        name="h3_infini",
    )(A_q.reshape(S, D), A_k.reshape(S, D), A_v.reshape(S, D), A_shift_k.T, A_ssm_k, A_ssm_D,
      B_x.reshape(S, D), B_wq, B_wk, B_wv, B_wo, B_beta, _DFT)
    return out.reshape(1, S, 2 * D)
```

```python
import math

import numpy as np
import jax
import jax.numpy as jnp
from jax import lax
from jax.experimental import pallas as pl
from jax.experimental.pallas import tpu as pltpu

S, D = 2048, 640
H, DH, NSEG, L = 32, 20, 4, 512
T = 128
HALF = T // 2
NC = D // T
CB = 2 * T
NB = S // CB
NF = T // 8
NQ = L // T
UH = 4
UD = UH * DH
NU = H // UH
WPAIR = 192
BF, F32 = jnp.bfloat16, jnp.float32
LOG2E = math.log2(math.e)


def _dft_matrices():
    m = np.arange(T)[:, None]
    r = np.arange(T)[None, :]

    def rows(power):
        ang = np.pi * np.mod((4 * m + 1) * power, 1024) / 512
        f = np.stack([np.cos(ang).reshape(NF, 8, T), -np.sin(ang).reshape(NF, 8, T)], 1)
        return f.reshape(2 * T, T)

    even, odd = rows(2 * r), rows(2 * r + 1)
    lane = np.arange(T)
    even_h = even[:, lane // 2 + (T // 2) * (lane % 2)]
    odd_h = odd[:, lane // 2 + (T // 2) * (1 - lane % 2)]
    inverse = [np.concatenate([f[:T].T, f[T:].T]) / (2 * T) for f in (even, odd)]
    bits = np.stack([even, odd, even_h, odd_h] + inverse).astype(np.float32).astype(BF)
    bits = bits.view(np.uint16).astype(np.uint32)
    return (bits[:, 0::2] | (bits[:, 1::2] << 16))[4:]


_INVERSE_DFT = _dft_matrices()


def _forward_dft(which):
    row, lane = _iota((8, T), 0), _iota((8, T), 1)
    odd = which % 2
    sample = lane if which < 2 else (lane >> 1) + (T // 2) * ((lane & 1) ^ odd)
    power = 2 * sample + odd

    def unit(turn):
        angle = lambda t: (t & 1023).astype(F32) * (math.pi / 512)
        return jnp.cos(angle(turn)), jnp.cos(angle(turn + 256))

    (re, im), (step_re, step_im) = unit((4 * row + 1) * power), unit(32 * power)
    for _ in range(NF):
        yield jnp.concatenate([re, im], axis=0).astype(BF)
        re, im = re * step_re - im * step_im, re * step_im + im * step_re


def _pack(x):
    return pltpu.bitcast(x, jnp.uint32)


def _unpack(w):
    return pltpu.bitcast(w, BF)


def _halves(x):
    w = pltpu.bitcast(x, jnp.uint32)
    return (lax.bitcast_convert_type(w << 16, F32),
            lax.bitcast_convert_type(w & np.uint32(0xFFFF0000), F32))


def _interleave(even, odd):
    e, o = (lax.bitcast_convert_type(v.astype(BF).astype(F32), jnp.uint32) for v in (even, odd))
    return pltpu.bitcast((e >> 16) | o, BF)


def _dot(a, b):
    return jnp.dot(a, b, preferred_element_type=F32)


def _dot_nt(a, b):
    return lax.dot_general(a, b, (((1,), (1,)), ((), ())), preferred_element_type=F32)


def _phi(t):
    return jnp.where(t > 0, t + 1.0, jnp.exp(t))


def _iota(shape, dim):
    return lax.broadcasted_iota(jnp.int32, shape, dim)


def _head_of(z):
    return sum((z >= DH * i).astype(jnp.int32) for i in range(1, UH))


_PLANS = {
    "conv_forward": (
    ("Q30 V30 Q31 V31 P Q32 V32 Q33 V33 P X U Q20 Q21 V20 X V21 Q22 V22 P Q10 V10 Q11 X "
     "V11 V00 P X Q00 P X",
     "Q30 P V30 V31 Q31 Q32 Q33 X V32 V33 X U P Q20 X Q21 V20 V21 Q22 V22 P Q10 V10 X Q11 "
     "X V00 P V11 Q00 P"),
     (0.5, 0.8, 0.0)),
    "conv_mix": (
    ("R P Q30 Q31 V30 V31 Q32 V32 Q33 U V33 P Q20 V20 O Q21 V21 Q22 V22 P O Q10 Q11 V10 "
     "V11 V00 Q00 P P O",
     "V30 P R Q30 Q31 V31 Q32 V32 V20 Q33 V33 Q20 U P Q21 Q22 Q10 V10 Q11 V21 V22 Q00 P O "
     "P P V11 V00 O O"),
     (0.1, 0.6, 0.3)),
    "conv_inverse": (
    ("R P Q30 V30 Q31 V31 X V32 V33 Q32 Q33 P X X Q20 V20 Q21 V21 Q22 V22 P Q10 V10 X Q11 "
     "V11 O P Q00 P V00",
     "P R Q30 V30 X Q31 V31 V32 X Q32 Q33 V33 P Q20 V20 V21 Q21 V22 Q22 Q10 V10 X Q11 V11 "
     "X P Q00 P O O P V00 O O O"),
     (0.15, 0.4, 0.45)),
    "third_last": (
    ("V30 R P Q30 V31 Q31 X V32 Q32 Q33 V33 P V20 X Q20 Q21 V21 X Q22 V22 P Q10 V10 X Q11 "
     "V11 O P Q00 P V00",
     "V30 P Q30 X Q31 V31 R V32 Q32 V33 Q33 P X Q20 V20 Q21 O V21 X V22 Q22 Q10 V10 O Q11 "
     "V11 X P P Q00 O P V00 O O"),
     (0.5, 0.5, 0.0)),
    "last": (
    ("R X X X Q30 V30 X Q31 V31 X V32 Q32 X Q33 X Q20 X V20 V33 Q21 V21 X V22 Q22 X Q10 X "
     "V10 X Q11 V11 Q00 V00",
     "R D X V30 V31 X V32 V33 X V20 V21 X V22 O O D O V10 V11 V00 O O O D T3 T3 T3 T3 T3 "
     "T3 T2 T2 T2 T2 T1 T2 T1 T1 T1 T2 T1 T1 T0 T0 T0 T0 T0 T0"),
     (1.0, 1.0, 1.0)),
}
_PLANS = {name: ([half.split() for half in halves], share) for name, (halves, share) in _PLANS.items()}
_WARM_UP = ("Q30 Q31 Q32 Q33 P P Q20 Q21 W Q22 P Q10 Q11 P Q00 P".split(),
            "P Q30 Q31 Q32 Q33 P Q20 Q21 Q22 P Q10 Q11 P Q00 P".split())


def _kernel(q_hbm, k_hbm, v_hbm, shift_hbm, h_hbm, d_hbm, x_hbm, wq_hbm, wk_hbm, wv_hbm,
            wo_hbm, beta_hbm, dft_hbm, out_hbm,
            q_v, k_v, v_v, h_v, x_v, w_v, wo_v, wt_s, dft_s, kf_s, kv_s, xg_s, y_s, yl_s,
            outa_s, outb_s, ot0_s, ot1_s, mem_s, meml_s, gate_s, bias_s,
            kn_s, rq_s, pk0_s, pk1_s, pq0_s, pq1_s, vt0_s, vt1_s, va0_s, va1_s,
            s_s, p0_s, p1_s, m_s, ret_s, e_s, shift_ref, d_ref, beta_ref, zero_s,
            sem_w, sem_x, sem_a, sem_q, sem_c, sem_oa, sem_ob):
    ot_s = (ot0_s, ot1_s)
    pk_s, pq_s, vt_s = (pk0_s, pk1_s), (pq0_s, pq1_s), (vt0_s, vt1_s)
    va_s, p_s = (va0_s, va1_s), (p0_s, p1_s)

    def y_of(c):
        return yl_s if c == NC - 1 else y_s.at[c]

    def w_copy(i, t):
        cols = pl.ds(t * T, T)
        return pltpu.make_async_copy((wq_hbm, wk_hbm, wv_hbm)[i].at[:, cols], w_v.at[i, t],
                                     sem_w.at[i * NC + t])

    def wo_copy():
        return pltpu.make_async_copy(wo_hbm, wo_v, sem_w.at[3 * NC])

    def x_copy(first, count):
        rows = pl.ds(first * L, count * L)
        return pltpu.make_async_copy(x_hbm.at[rows], x_v.at[rows], sem_x.at[first])

    def conv_copies(j):
        src = pl.ds(pl.multiple_of(jnp.minimum(j, NQ - 1) * L, L), L)
        dst = pl.ds(pl.multiple_of(j * L, L), L)
        return (pltpu.make_async_copy(k_hbm.at[src], k_v.at[dst], sem_a.at[3 * j]),
                pltpu.make_async_copy(v_hbm.at[src], v_v.at[dst], sem_a.at[3 * j + 1]),
                pltpu.make_async_copy(h_hbm.at[:, src], h_v.at[j], sem_a.at[3 * j + 2]))

    def q_copy():
        return pltpu.make_async_copy(q_hbm, q_v, sem_q)

    def const_copy(i):
        src, dst = ((beta_hbm, beta_ref), (shift_hbm, shift_ref), (d_hbm, d_ref),
                    (dft_hbm, dft_s.at[4:6]))[i]
        return pltpu.make_async_copy(src, dst, sem_c.at[i])

    def oa_copy(rows, lanes):
        return pltpu.make_async_copy(outa_s.at[rows, lanes], out_hbm.at[rows, lanes], sem_oa)

    def ob_copy(rows):
        return pltpu.make_async_copy(outb_s.at[rows], out_hbm.at[rows, pl.ds(D, D)], sem_ob)

    kv_ready = []

    def gate_kv(u, half):
        src = pl.multiple_of(u * CB, CB)
        for c in range(NC):
            lanes = slice(c * T, (c + 1) * T)
            taps = [shift_ref[t:t + 1, lanes].astype(F32) for t in range(4)]
            pe, po = kf_s[c, 0], kf_s[c, 1]
            for r in range(0, T, 16):
                rows = pl.ds(pl.multiple_of(src + 2 * r, 32), 32)
                ke, ko = _halves(k_v[rows, lanes])
                ve, vo = _halves(v_v[rows, lanes])
                e1 = pltpu.roll(jnp.concatenate([pe, ke], axis=0), 1, 0)[8:24]
                odd = jnp.concatenate([po, ko], axis=0)
                o1, o2 = pltpu.roll(odd, 1, 0)[8:24], pltpu.roll(odd, 2, 0)[8:24]
                se = ke * taps[0] + o1 * taps[1] + e1 * taps[2] + o2 * taps[3]
                so = ko * taps[0] + ke * taps[1] + o1 * taps[2] + e1 * taps[3]
                kv_s[half, c, r:r + 16, :] = (se * ve).astype(BF)
                kv_s[half, c, T + r:T + r + 16, :] = (so * vo).astype(BF)
                pe, po = ke[8:16], ko[8:16]
                yield 1
            kf_s[c, 0] = pe
            kf_s[c, 1] = po
            kv_ready.append((half, c))

    def conv_forward(u, half, c):
        lanes = slice(c * T, (c + 1) * T)
        h0, h1 = (pltpu.bitcast(h_v[u // 2, lanes, (2 * half + j) * T:(2 * half + j + 1) * T], jnp.uint32)
                  for j in range(2))
        even = (_iota(h0.shape, 1) & 1) == 0
        he = pltpu.bitcast(jnp.where(even, h0, pltpu.roll(h1, 1, 1)), BF)
        ho = pltpu.bitcast(jnp.where(even, pltpu.roll(h1, T - 1, 1), h0), BF)
        for base, a, b in (
                (c, _dot(_unpack(dft_s[0]), kv_s[half, c, 0:T, :]),
                 _dot(_unpack(dft_s[1]), kv_s[half, c, T:CB, :])),
                (NC + c, _dot_nt(_unpack(dft_s[2]), he), _dot_nt(_unpack(dft_s[3]), ho))):
            xg_s[base, u, 0:CB, :] = a + b
            xg_s[base, u, CB:2 * CB, :] = a - b

    def conv_mac(items, w=2):
        skip = {c: jnp.broadcast_to(d_row(c), (8, T)) for c, _ in items}
        for c, f in items:
            for k in range(NB // w):
                outs = range(k * w, (k + 1) * w)
                r0 = pl.multiple_of((f + zero_s[k]) * 16, 16)
                plus = {}
                for sign in range(2):
                    re = pl.ds(pl.multiple_of(r0 + sign * CB, 8), 8)
                    im = pl.ds(pl.multiple_of(r0 + sign * CB + 8, 8), 8)
                    acc, g, h = {}, {}, {}

                    def filt(n):
                        if n not in g:
                            for m in (n, n - 1):
                                if m >= 0 and m not in h:
                                    h[m] = (xg_s[NC + c, m, re, :], xg_s[NC + c, m, im, :])
                            if n == 0:
                                g[n] = (h[0][0] + skip[c], h[0][1])
                            else:
                                g[n] = (h[n][0] - h[n - 1][1], h[n][1] + h[n - 1][0])
                        return g[n]

                    for b in range(max(outs) + 1):
                        xr, xi = xg_s[c, b, re, :], xg_s[c, b, im, :]
                        cost = 0
                        for a in outs:
                            if b > a:
                                continue
                            gr, gi = filt(a - b)
                            p = (xr * gr - xi * gi, xr * gi + xi * gr)
                            acc[a] = p if a not in acc else (acc[a][0] + p[0], acc[a][1] + p[1])
                            cost += 1
                            if a == b and sign == 0:
                                plus[a] = jnp.concatenate(acc[a], axis=0)
                            elif a == b:
                                minus = jnp.concatenate(acc[a], axis=0)
                                y_of(c)[a, pl.ds(r0, 16), :] = (plus[a] + minus).astype(BF)
                                y_of(c)[a, pl.ds(pl.multiple_of(r0 + CB, 16), 16), :] = (
                                    plus[a] - minus).astype(BF)
                        yield cost

    class Filler:
        def __init__(self):
            self.gen, self.credit, self.in_k = None, 0.0, False

        def pin(self, value, amount):
            if self.gen is None or amount == 0:
                return
            if self.in_k:
                k_v[S + L:S + L + 16, 0:T] = jnp.concatenate([value, value], axis=0).astype(BF)
            else:
                xg_s[2 * NC, 0, 0:8, :] = value
            self.credit += amount
            while self.gen is not None and self.credit > 0:
                cost = next(self.gen, None)
                if cost is None:
                    self.gen = None
                else:
                    self.credit -= cost

        def drain(self):
            if self.gen is not None:
                for _ in self.gen:
                    pass
            self.gen = None

    filler = Filler()

    def conv_inverse(u, c):
        r0 = pl.multiple_of(u * CB, CB)
        lanes = slice(c * T, (c + 1) * T)
        qs = _halves(q_v[pl.ds(r0, CB), lanes])
        out = []
        for j in range(2):
            inv = jnp.concatenate([_unpack(dft_s[4 + j, 0:T // 2, :]),
                                   _unpack(dft_s[4 + j, T // 2:T, :])], axis=1)
            y = _dot(inv, y_of(c)[u, j * CB:(j + 1) * CB, :])
            out.append(qs[j] * y)
        outa_s[pl.ds(r0, CB), lanes] = _interleave(*out)

    def out_proj(o, rows, amount):
        m = o[0].shape[0]
        last = NC - 1
        head = jnp.concatenate(o[0:last], axis=1)

        def pin(part):
            for r in range(0, m, 32):
                filler.pin(part[r:r + 8, 0:T], amount * 32 / (6 * m))

        edge = _dot(o[last], wo_v[last * T:D, 0:last * T])
        pin(edge)
        yield
        corner = _dot(o[last], wo_v[last * T:D, last * T:D])
        for n in reversed(range(NC)):
            part = _dot(head, wo_v[0:last * T, n * T:(n + 1) * T])
            pin(part)
            part = part + (corner if n == last else edge[:, n * T:(n + 1) * T])
            outb_s[rows, n * T:(n + 1) * T] = part.astype(BF)
            yield

    def own_rows(x, i, fill):
        low4 = _iota((8, T), 0) < 4
        full = jnp.full((8, T), fill, F32)
        g0 = 5 * (i // 2)
        if i % 2 == 0:
            body = [x[8 * g0:8 * g0 + 16], jnp.where(low4, x[8 * g0 + 16:8 * g0 + 24], fill)]
        else:
            body = [jnp.where(low4, fill, x[8 * g0 + 16:8 * g0 + 24]), x[8 * g0 + 24:8 * g0 + 40]]
        return jnp.concatenate(body + [full] if i < 2 else [full] + body, axis=0).astype(BF)

    def project(n, par, amount, need_q=True, need_k=True):
        s, u = n // NU, n % NU
        w0 = pl.multiple_of((u // 2) * (WPAIR // 2), 32) + par * (UD // 2)
        x0 = pl.multiple_of(s * L, L)
        slot = (n // 2) % 2
        pad = jnp.zeros((T - UD, T), F32)

        def finish(j, qkv):
            cols = slice(j * T, (j + 1) * T)
            qt, kt, vt = qkv[0:UD], qkv[UD:2 * UD], qkv[2 * UD:3 * UD]
            kn_s[cols, :] = jnp.concatenate([kt, pad], axis=0).T.astype(BF)
            qs = qt * (DH ** -0.5 * LOG2E)
            low4 = _iota((8, T), 0) < 4
            left = _iota((8, T), 1) < T // 2
            zero = jnp.zeros((8, T), F32)
            for pr in range(UH // 2):
                qa = [qs[40 * pr + 8 * r:40 * pr + 8 * r + 8] for r in range(3)]
                qb = [pltpu.roll(qs[40 * pr + 8 * r:40 * pr + 8 * r + 8], T // 2, 1) for r in (2, 3, 4)]
                ra = [qa[0], qa[1], jnp.where(low4, qa[2], 0.0)]
                rb = [jnp.where(low4, 0.0, qb[0]), qb[1], qb[2]]
                rh = [jnp.where(left, 0.0, qa[0]), jnp.where(left, 0.0, qa[1]),
                      jnp.where(left, rb[0], ra[2]),
                      jnp.where(left, qb[1], 0.0), jnp.where(left, qb[2], 0.0)]
                for i, rows in ((2 * pr, ra), (2 * pr + 1, rb)):
                    rows = rows + [zero] if pr == 0 else [zero] + rows
                    rq_s[j, i, 8 * i:8 * i + 16, :] = _pack(jnp.concatenate(rows, axis=0).astype(BF))
                rows = rh + [zero] if pr == 0 else [zero] + rh
                rq_s[j, UH + pr, 16 * pr:16 * pr + 24, :] = _pack(
                    jnp.concatenate(rows, axis=0).astype(BF))
            for i in range(UH):
                va_s[par][slot, i, j] = own_rows(vt, i, 1.0)
            if need_q:
                pq_s[par][slot, j] = _phi(qt).astype(BF)
            if need_k:
                pk_s[par][slot, j] = _phi(kt).astype(BF)
                vt_s[par][slot, j] = vt.astype(BF)

        w = [_unpack(jnp.concatenate(
            [wt_s[c, i, pl.ds(pl.multiple_of(w0, 8), UD // 2), :] for i in range(3)], axis=0))
             for c in range(NC)]
        part = _dot_nt(w[NC - 1], x_v[pl.ds(x0, L), (NC - 1) * T:D])
        for j in range(NQ):
            e_s[j] = part[:, j * T:(j + 1) * T]
        for r in range(0, 3 * UD, 24):
            filler.pin(part[r:r + 8, 0:T], amount / (10 * NC))
        yield
        w = jnp.concatenate(w[0:NC - 1], axis=1)
        for j in reversed(range(NQ)):
            rows = pl.ds(pl.multiple_of(x0 + j * T, T), T)
            part = _dot_nt(w, x_v[rows, 0:(NC - 1) * T])
            for r in range(0, 3 * UD, 24):
                filler.pin(part[r:r + 8], amount / (10 * NC))
            finish(j, part + e_s[j])
            yield

    def s_off(j, i, t, n=T):
        return pl.ds((2 * j * (j + 1) + i * (j + 1) + t) * T, n)

    def hi_off(j, pr):
        return pl.ds((2 * j * (j + 1) + 2 * pr * (j + 1) + j) * T + HALF, HALF)

    def sparse(j, i, first, count):
        parts = [_unpack(rq_s[j, i, first // 2:(first + count) // 2, :]),
                 jnp.zeros((T - first - count, T), BF)]
        if first:
            parts.insert(0, jnp.zeros((first, T), BF))
        return jnp.concatenate(parts, axis=0)

    def col_max(x):
        return jnp.max(x.reshape(x.shape[0] // 8, 8, T), axis=0)

    def scores(j, t, top, amount):
        rq = jnp.concatenate([sparse(j, i, 16 * i, 32) for i in range(UH)], axis=1)
        n = T if t < j else HALF
        sc = _dot(kn_s[t * T:t * T + n, :], rq)
        if t == j:
            rh = jnp.concatenate([sparse(j, UH + pr, 32 * pr, 48) for pr in range(2)], axis=1)
            hi = _dot(kn_s[t * T + HALF:(t + 1) * T, :], rh)
        for i in range(UH):
            si = sc[:, i * T:(i + 1) * T]
            if t == j:
                si = si + bias_s[i % 2]
            s_s[s_off(j, i, t, n), :] = si
            if i == 0:
                for r in range(0, n, 32):
                    filler.pin(si[r:r + 8], amount * 32 / n)
            top[i] = col_max(si) if t == 0 else jnp.maximum(top[i], col_max(si))
        if t < j:
            return
        left = _iota((8, T), 1) < HALF
        for pr in range(2):
            si = hi[:, pr * T:(pr + 1) * T] + bias_s[2]
            s_s[hi_off(j, pr), :] = si
            mh = col_max(si)
            ma = jnp.maximum(top[2 * pr], jnp.where(left, -jnp.inf, mh))
            mb = jnp.maximum(top[2 * pr + 1], jnp.where(left, mh, -jnp.inf))
            ma = jnp.broadcast_to(jnp.max(ma, axis=0, keepdims=True), (8, T))
            mb = jnp.broadcast_to(jnp.max(mb, axis=0, keepdims=True), (8, T))
            m_s[j, 2 * pr] = ma
            m_s[j, 2 * pr + 1] = mb
            m_s[j, UH + pr] = jnp.where(left, mb, ma)

    def weights(rows, j, i):
        sc = s_s[rows, :]
        m = jnp.concatenate([m_s[j, i]] * (sc.shape[0] // 8), axis=0)
        return jnp.exp2(sc - m).astype(BF)

    def softmax(par, j, t):
        n = T if t < j else HALF
        for i in range(UH):
            p_s[par][s_off(j, i, t, n), :] = weights(s_off(j, i, t, n), j, i)
        if t < j:
            return
        left = _iota((HALF // 2, T), 1) < HALF
        none = jnp.zeros((HALF // 2, T), jnp.uint32)
        for pr in range(2):
            p = pltpu.bitcast(weights(hi_off(j, pr), j, UH + pr), jnp.uint32)
            for i, part in ((2 * pr, jnp.where(left, none, p)), (2 * pr + 1, jnp.where(left, p, none))):
                p_s[par][pl.ds(s_off(j, i, t).start + HALF, HALF), :] = pltpu.bitcast(part, BF)

    def spread(a, b):
        low4 = _iota(a.shape, 0) < 4
        ar, br = pltpu.roll(a, 4, 0), pltpu.roll(b, 4, 0)
        r0, r1 = jnp.where(low4, a, ar), jnp.where(low4, ar, a)
        r2, r3 = jnp.where(low4, b, br), jnp.where(low4, br, b)
        return jnp.concatenate([r0, r0, a, r1, r1, r2, r2, b, r3, r3], axis=0)

    def retrieve(n, par):
        u, slot = n % NU, (n // 2) % 2
        zpad = jnp.zeros((T - UD, T), BF)
        pq = jnp.concatenate(
            [jnp.concatenate([pq_s[par][slot, j], zpad], axis=0) for j in range(NQ)], axis=1)
        ret = _dot(meml_s[u], pq)
        rd = 1.0 / (ret[UD:UD + 16] + 1e-6)
        ret_s[...] = ret[0:UD] * spread(rd[0:8], rd[8:16])

    def update(n, par, s):
        u, slot = n % NU, (n // 2) % 2
        zpad = jnp.zeros((T - UD, T), BF)
        va = jnp.concatenate(
            [jnp.concatenate([vt_s[par][slot, j], jnp.ones((16, T), BF)], axis=0) for j in range(NQ)],
            axis=1)
        pk = jnp.concatenate(
            [jnp.concatenate([pk_s[par][slot, j], zpad], axis=0) for j in range(NQ)], axis=1)
        mem = _dot_nt(va, pk)
        if s > 0:
            mem = mem_s[u] + mem
        if s < NSEG - 2:
            mem_s[u] = mem
        row = _iota((UD + 16, T), 0)
        row_head = jnp.where(row < UD, _head_of(row), (row - UD) >> 2)
        meml_s[u] = jnp.where(row_head == _head_of(_iota((UD + 16, T), 1)), mem, 0.0).astype(BF)

    def values(n, par, s, j, t, acc):
        u, slot = n % NU, (n // 2) % 2
        for i in range(UH):
            part = _dot(va_s[par][slot, i, t], p_s[par][s_off(j, i, t), :])
            acc[i] = part if t == 0 else acc[i] + part
        if t < j:
            return
        heads = []
        for i in range(UH):
            den = acc[i][24:32] if i < 2 else acc[i][0:8]
            val = acc[i][0:24] if i < 2 else acc[i][8:32]
            val = val * jnp.concatenate([1.0 / den] * 3, axis=0)
            heads.append(pltpu.roll(val, HALF, 1) if i % 2 else val)
        low4 = _iota((8, T), 0) < 4
        att = jnp.concatenate([
            heads[0][0:16], jnp.where(low4, heads[0][16:24], heads[1][0:8]), heads[1][8:24],
            heads[2][0:16], jnp.where(low4, heads[2][16:24], heads[3][0:8]), heads[3][8:24]], axis=0)
        rows = pl.ds(pl.multiple_of(u * UD, 16), UD)
        gt = gate_s[rows, :]
        o = (1.0 - gt) * att
        if s > 0:
            o = o + gt * ret_s[:, j * T:(j + 1) * T]
        o = o.astype(BF)
        ot_s[s % 2][j, rows, :] = o

    deliver = []

    def step(n, par, s, order, share, jobs=(), oproj=None, stages='PQSV', need_q=True, arrive=None):
        jobs = list(jobs)
        proj = project(n + 3, 1 - par, share[1], need_q=need_q, need_k=s < NSEG - 1)
        top, acc, final = [None] * UH, {}, {}
        for tok in order:
            if tok[0] == 'Q':
                j, t = int(tok[1]), int(tok[2])
                if 'S' in stages:
                    softmax(1 - par, j, t)
                if 'Q' in stages:
                    scores(j, t, top, share[0] / 10)
            elif tok[0] == 'V':
                if 'V' in stages:
                    values(n, par, s, int(tok[1]), int(tok[2]), acc.setdefault(tok[1], [None] * UH))
            elif tok == 'P':
                if 'P' in stages:
                    next(proj)
            elif tok == 'R':
                if 'V' in stages and s > 0:
                    retrieve(n, par)
            elif tok == 'U':
                if 'V' in stages and s < NSEG - 1:
                    update(n, par, s)
            elif tok[0] == 'T':
                j = int(tok[1])
                rows = pl.ds((NSEG - 1) * L + j * T, T)
                if j not in final:
                    final[j] = [out_proj(out_tiles(NSEG - 1, j), rows, 0), 0]
                next(final[j][0])
                final[j][1] += 1
                if final[j][1] == NC + 1:
                    ob_copy(rows).start()
            elif tok == 'D':
                deliver.pop(0)()
            elif tok == 'O':
                if oproj is not None:
                    next(oproj)
            elif tok == 'W':
                if arrive is not None:
                    arrive()
            elif tok == 'X':
                if jobs:
                    jobs.pop(0)()
        assert not jobs

    def out_tiles(s, j):
        return [ot_s[s % 2][j, c * T:(c + 1) * T, :].T for c in range(NC)]

    def pair_step(s, j, stages=('PQSV', 'PQSV'), mac=None, inverse=None, plan=None):
        orders, mix = _PLANS[plan or ("conv_forward", "conv_mix", "conv_mix", "conv_inverse")[s]]
        us = (2 * j, 2 * j + 1)
        oproj = None
        filler.gen, filler.credit, filler.in_k = None, 0.0, s == 0
        if s == 0:
            del kv_ready[:]
            filler.gen = (cost for half, u in enumerate(us) for cost in gate_kv(u, half))
            share = [16 * NC * v for v in mix]
        else:
            if mac is None:
                mac = [(c, 4 * j + r) for c in (2 * s - 2, 2 * s - 1) for r in range(4)]
            weight = (mix[0] * sum('Q' in st for st in stages)
                      + mix[1] * sum('P' in st for st in stages) + 2 * mix[2])
            share = [72 * len(mac) * v / weight for v in mix]
            if mac:
                filler.gen = conv_mac(mac)
            rows = pl.ds(pl.multiple_of((s - 1) * L + j * T, T), T)
            oproj = out_proj(out_tiles(s - 1, j), rows, 2 * share[2])
        for half, u in enumerate(us):
            jobs = []
            if s == 0:
                def forward(u, half, c):
                    while (half, c) not in kv_ready and filler.gen is not None:
                        if next(filler.gen, None) is None:
                            filler.gen = None
                        filler.credit -= 1
                    conv_forward(u, half, c)
                jobs = [lambda c=c, u=u, half=half: forward(u, half, c) for c in range(NC)]
            elif s == NSEG - 1:
                todo = (inverse[half] if inverse else []) + [(u, c) for c in range(NC - 1)]
                jobs = [lambda b=b, c=c: conv_inverse(b, c) for b, c in todo]
            step(s * NU + u, half, s, orders[half], share, jobs, oproj, stages[half])
        filler.drain()

    def last_mac(j, extra=None):
        return [(NC - 1, f) for f in [4 * j + r for r in range(4)] + (extra or [12 + 2 * j])]

    def transpose_weights(t):
        for i in range(3):
            for c in range(NC):
                wt = _pack(w_v[i, t, c * T:(c + 1) * T, :].T)
                for r in range(T // 16):
                    pair, off = divmod(t * T + 16 * r, 2 * UD)
                    row = (pair * WPAIR + off) // 2
                    wt_s[c, i, row:row + 8, :] = wt[8 * r:8 * r + 8]

    def d_row(c):
        return d_ref[...].astype(F32).reshape(1, D)[:, c * T:(c + 1) * T]

    def send_pair(j):
        oa_copy(pl.ds(pl.multiple_of(j * L, L), L), pl.ds(0, (NC - 1) * T)).start()
        ob_copy(pl.ds(pl.multiple_of(2 * L + j * T, T), T)).start()

    def epilogue():
        first = pl.ds(0, (NC - 1) * T)
        pair_step(3, NQ - 2, stages=('PQSV', 'QSV'), mac=last_mac(NQ - 2, [13, 15]), plan="third_last")
        send_pair(NQ - 2)

        deliver.extend([
            lambda: (oa_copy(pl.ds(0, S), pl.ds((NC - 1) * T, T)).start(),
                     oa_copy(pl.ds(S - 2 * CB, CB), first).start()),
            lambda: oa_copy(pl.ds(S - CB, CB), first).start(),
            lambda: ob_copy(pl.ds(3 * L - T, T)).start()])
        pair_step(3, NQ - 1, stages=('SV', 'V'), mac=[], plan="last",
                  inverse=[[(b, NC - 1) for b in range(NB)], []])

    for i in range(3):
        w_copy(i, 0).start()
    const_copy(0).start()
    x_copy(0, 1).start()
    key, lane = _iota((T // 2, T), 0), _iota((T // 2, T), 1)
    for b, query in enumerate((lane, lane ^ (T // 2), lane & (T // 2 - 1))):
        bias_s[b] = jnp.where(key > query, -1e9 * LOG2E, 0.0).astype(F32)
    kf_s[...] = jnp.zeros(kf_s.shape, F32)
    for k in range(NB):
        zero_s[k] = 0
    for which in range(4):
        for f, rows in enumerate(_forward_dft(which)):
            dft_s[which, 8 * f:8 * f + 8, :] = _pack(rows)
    const_copy(0).wait()
    g = jax.nn.sigmoid(beta_ref[...].astype(F32).reshape(1, H))
    rr = _iota((D, H), 0)
    hh = _iota((D, H), 1) * DH
    gate = jnp.sum(jnp.where((rr >= hh) & (rr < hh + DH), g, 0.0), axis=1, keepdims=True)
    gate_s[...] = jnp.broadcast_to(gate, (D, T))
    for i in range(3):
        w_copy(i, 0).wait()
    for i in range(3):
        w_copy(i, 1).start()
    transpose_weights(0)
    x_copy(0, 1).wait()
    for i in range(3):
        w_copy(i, 2).start()
    for _ in project(0, 0, 0, need_q=False):
        pass
    for i in range(3):
        w_copy(i, 1).wait()
    for i in range(3):
        w_copy(i, 3).start()
    const_copy(1).start()
    transpose_weights(1)

    def fetch_conv():
        for cp in conv_copies(0):
            cp.start()
    step(-2, 0, 0, _WARM_UP[0], (0, 0), stages='PQ', need_q=False, arrive=fetch_conv)
    for t in (2, 3):
        for i in range(3):
            w_copy(i, t).wait()
    for t in (2, 3):
        transpose_weights(t)
    step(-1, 1, 0, _WARM_UP[1], (0, 0), stages='PQS', need_q=False)
    const_copy(1).wait()
    for cp in conv_copies(0):
        cp.wait()
    for i in range(3):
        w_copy(i, 4).start()
    x_copy(1, 1).start()

    def seg0(j, _):
        @pl.when(j == 1)
        def _():
            for i in range(3):
                w_copy(i, 4).wait()
            x_copy(1, 1).wait()
            wo_copy().start()
            x_copy(2, 2).start()
            const_copy(2).start()
            transpose_weights(4)

        for cp in conv_copies(j + 1):
            cp.start()
        pair_step(0, j)
        for cp in conv_copies(j + 1):
            cp.wait()
    lax.fori_loop(0, NQ, seg0, None)

    const_copy(2).wait()
    const_copy(3).start()
    wo_copy().wait()
    x_copy(2, 2).wait()

    lax.fori_loop(0, NQ, lambda j, _: pair_step(1, j), None)
    ob_copy(pl.ds(0, L)).start()
    q_copy().start()
    lax.fori_loop(0, NQ, lambda j, _: pair_step(2, j), None)
    ob_copy(pl.ds(L, L)).start()
    q_copy().wait()
    const_copy(3).wait()

    def seg3(j, _):
        pair_step(3, j, mac=last_mac(j))
        send_pair(j)
    lax.fori_loop(0, NQ - 2, seg3, None)
    epilogue()

    oa_copy(pl.ds(0, S), pl.ds(0, D)).wait()
    ob_copy(pl.ds(0, S)).wait()


@jax.jit
def pallas_concat_heads__ssm_conv_h3__memory_aug_infini_attn__prompt_kernel(
    A_q, A_k, A_v, A_shift_k, A_ssm_k, A_ssm_D, B_x, B_wq, B_wk, B_wv, B_wo, B_beta,
):
    hbm = pl.BlockSpec(memory_space=pl.ANY)
    dma = pltpu.SemaphoreType.DMA
    out = pl.pallas_call(
        _kernel,
        out_shape=jax.ShapeDtypeStruct((S, 2 * D), BF),
        in_specs=[hbm] * 13,
        out_specs=hbm,
        scratch_shapes=[
            pltpu.VMEM((S, D), BF),
            pltpu.VMEM((S + L + 64, D), BF),
            pltpu.VMEM((S + L, D), BF),
            pltpu.VMEM((NQ + 1, D, L), BF),
            pltpu.VMEM((S, D), BF),
            pltpu.VMEM((3, NC, D, T), BF),
            pltpu.VMEM((D, D), BF),
            pltpu.VMEM((NC, 3, NQ * WPAIR // 2, T), jnp.uint32),
            pltpu.VMEM((6, T, T), jnp.uint32),
            pltpu.VMEM((NC + 1, 2, 8, T), F32),
            pltpu.VMEM((2, NC, CB, T), BF),
            pltpu.VMEM((2 * NC + 1, NB, 2 * CB, T), F32),
            pltpu.VMEM((NC - 1, NB, 2 * CB, T), BF),
            pltpu.VMEM((NB, 2 * CB, T), BF),
            pltpu.VMEM((S, D), BF),
            pltpu.VMEM((S, D), BF),
            pltpu.VMEM((NQ, D, T), BF),
            pltpu.VMEM((NQ, D, T), BF),
            pltpu.VMEM((NU, UD + 16, T), F32),
            pltpu.VMEM((NU, UD + 16, T), BF),
            pltpu.VMEM((D, T), F32),
            pltpu.VMEM((3, T // 2, T), F32),
            pltpu.VMEM((L, T), BF),
            pltpu.VMEM((NQ, UH + 2, T // 2, T), jnp.uint32),
            *[pltpu.VMEM((2, NQ, UD, T), BF)] * 6,
            *[pltpu.VMEM((2, UH, NQ, 32, T), BF)] * 2,
            pltpu.VMEM((40 * T, T), F32),
            *[pltpu.VMEM((40 * T, T), BF)] * 2,
            pltpu.VMEM((NQ, UH + 2, 8, T), F32),
            pltpu.VMEM((UD, L), F32),
            pltpu.VMEM((NQ, 3 * UD, T), F32),
            pltpu.VMEM((4, D), BF),
            pltpu.VMEM((D,), BF),
            pltpu.VMEM((H,), BF),
            pltpu.SMEM((NB,), jnp.int32),
            dma((3 * NC + 1,)), dma((3,)), dma((3 * (NQ + 1),)), dma(()),
            dma((4,)), dma(()), dma(()),
        ],
        compiler_params=pltpu.CompilerParams(
            vmem_limit_bytes=100 * 1024 * 1024),
        name="h3_infini",
    )(A_q.reshape(S, D), A_k.reshape(S, D), A_v.reshape(S, D), A_shift_k.T, A_ssm_k, A_ssm_D,
      B_x.reshape(S, D), B_wq, B_wk, B_wv, B_wo, B_beta, _INVERSE_DFT)
    return out.reshape(1, S, 2 * D)
```

```python
import math

import numpy as np
import jax
import jax.numpy as jnp
from jax import lax
from jax.experimental import pallas as pl
from jax.experimental.pallas import tpu as pltpu

S, D = 2048, 640
H, DH, NSEG, L = 32, 20, 4, 512
T = 128
HALF = T // 2
NC = D // T
CB = 2 * T
NB = S // CB
NF = T // 8
NQ = L // T
UH = 4
UD = UH * DH
NU = H // UH
WPAIR = 192
BF, F32 = jnp.bfloat16, jnp.float32
LOG2E = math.log2(math.e)


def _dft_matrices():
    m = np.arange(T)[:, None]
    r = np.arange(T)[None, :]

    def rows(power):
        ang = np.pi * np.mod((4 * m + 1) * power, 1024) / 512
        f = np.stack([np.cos(ang).reshape(NF, 8, T), -np.sin(ang).reshape(NF, 8, T)], 1)
        return f.reshape(2 * T, T)

    even, odd = rows(2 * r), rows(2 * r + 1)
    lane = np.arange(T)
    even_h = even[:, lane // 2 + (T // 2) * (lane % 2)]
    odd_h = odd[:, lane // 2 + (T // 2) * (1 - lane % 2)]
    inverse = [np.concatenate([f[:T].T, f[T:].T]) / (2 * T) for f in (even, odd)]
    bits = np.stack([even, odd, even_h, odd_h] + inverse).astype(np.float32).astype(BF)
    bits = bits.view(np.uint16).astype(np.uint32)
    return (bits[:, 0::2] | (bits[:, 1::2] << 16))[4:]


_INVERSE_DFT = _dft_matrices()


def _forward_dft(which):
    row, lane = _iota((8, T), 0), _iota((8, T), 1)
    odd = which % 2
    sample = lane if which < 2 else (lane >> 1) + (T // 2) * ((lane & 1) ^ odd)
    power = 2 * sample + odd

    def unit(turn):
        angle = lambda t: (t & 1023).astype(F32) * (math.pi / 512)
        return jnp.cos(angle(turn)), jnp.cos(angle(turn + 256))

    (re, im), (step_re, step_im) = unit((4 * row + 1) * power), unit(32 * power)
    for _ in range(NF):
        yield jnp.concatenate([re, im], axis=0).astype(BF)
        re, im = re * step_re - im * step_im, re * step_im + im * step_re


def _pack(x):
    return pltpu.bitcast(x, jnp.uint32)


def _unpack(w):
    return pltpu.bitcast(w, BF)


def _halves(x):
    w = pltpu.bitcast(x, jnp.uint32)
    return (lax.bitcast_convert_type(w << 16, F32),
            lax.bitcast_convert_type(w & np.uint32(0xFFFF0000), F32))


def _interleave(even, odd):
    e, o = (lax.bitcast_convert_type(v.astype(BF).astype(F32), jnp.uint32) for v in (even, odd))
    return pltpu.bitcast((e >> 16) | o, BF)


def _dot(a, b):
    return jnp.dot(a, b, preferred_element_type=F32)


def _dot_nt(a, b):
    return lax.dot_general(a, b, (((1,), (1,)), ((), ())), preferred_element_type=F32)


def _phi(t):
    return jnp.where(t > 0, t + 1.0, jnp.exp(t))


def _iota(shape, dim):
    return lax.broadcasted_iota(jnp.int32, shape, dim)


def _head_of(z):
    return sum((z >= DH * i).astype(jnp.int32) for i in range(1, UH))


_PLANS = {
    "conv_forward": (
    ("Q30 V30 Q31 V31 P Q32 V32 Q33 V33 P X U Q20 Q21 V20 X V21 Q22 V22 P Q10 V10 Q11 X "
     "V11 V00 P X Q00 P X",
     "Q30 P V30 V31 Q31 Q32 Q33 X V32 V33 X U P Q20 X Q21 V20 V21 Q22 V22 P Q10 V10 X Q11 "
     "X V00 P V11 Q00 P"),
     (0.5, 0.8, 0.0)),
    "conv_mix": (
    ("R P Q30 Q31 V30 V31 Q32 V32 Q33 U V33 P Q20 V20 O Q21 V21 Q22 V22 P O Q10 Q11 V10 "
     "V11 V00 Q00 P P O",
     "V30 P R Q30 Q31 V31 Q32 V32 V20 Q33 V33 Q20 U P Q21 Q22 Q10 V10 Q11 V21 V22 Q00 P O "
     "P P V11 V00 O O"),
     (0.1, 0.6, 0.3)),
    "conv_inverse": (
    ("R P Q30 V30 Q31 V31 X V32 V33 Q32 Q33 P X X Q20 V20 Q21 V21 Q22 V22 P Q10 V10 X Q11 "
     "V11 O P Q00 P V00",
     "P R Q30 V30 X Q31 V31 V32 X Q32 Q33 V33 P Q20 V20 V21 Q21 V22 Q22 Q10 V10 X Q11 V11 "
     "X P Q00 P O O P V00 O O O"),
     (0.15, 0.4, 0.45)),
    "third_last": (
    ("V30 R P Q30 V31 Q31 X V32 Q32 Q33 V33 P V20 X Q20 Q21 V21 X Q22 V22 P Q10 V10 X Q11 "
     "V11 O P Q00 P V00",
     "V30 P Q30 X Q31 V31 R V32 Q32 V33 Q33 P X Q20 V20 Q21 O V21 X V22 Q22 Q10 V10 O Q11 "
     "V11 X P P Q00 O P V00 O O"),
     (0.5, 0.5, 0.0)),
    "last": (
    ("R V30 X Q30 X X X Q31 V31 X V32 Q32 V20 Q33 Q20 X X V33 X V21 Q21 X Q22 V10 Q10 V22 "
     "Q11 X V11 X X Q00 V00",
     "R D X V30 V31 X V20 V32 V33 X V21 X V22 O V10 O O O D V11 V00 O O T3 T3 D T3 T3 T3 "
     "T3 T2 T2 T2 T1 T2 T2 T1 T1 T2 T1 T1 T1 T0 T0 T0 T0 T0 T0"),
     (1.0, 1.0, 1.0)),
}
_PLANS = {name: ([half.split() for half in halves], share) for name, (halves, share) in _PLANS.items()}
_WARM_UP = ("Q30 Q31 Q32 Q33 P P Q20 Q21 W Q22 P Q10 Q11 P Q00 P".split(),
            "P Q30 Q31 Q32 Q33 P Q20 Q21 Q22 P Q10 Q11 P Q00 P".split())


def _kernel(q_hbm, k_hbm, v_hbm, shift_hbm, h_hbm, d_hbm, x_hbm, wq_hbm, wk_hbm, wv_hbm,
            wo_hbm, beta_hbm, dft_hbm, out_hbm,
            q_v, k_v, v_v, h_v, x_v, w_v, wo_v, wt_s, dft_s, kf_s, kv_s, xg_s, y_s, yl_s,
            outa_s, outb_s, ot0_s, ot1_s, mem_s, meml_s, gate_s, bias_s,
            kn_s, rq_s, pk0_s, pk1_s, pq0_s, pq1_s, vt0_s, vt1_s, va0_s, va1_s,
            s_s, p0_s, p1_s, m_s, ret_s, e_s, shift_ref, d_ref, beta_ref, zero_s,
            sem_w, sem_x, sem_a, sem_q, sem_c, sem_oa, sem_ob):
    ot_s = (ot0_s, ot1_s)
    pk_s, pq_s, vt_s = (pk0_s, pk1_s), (pq0_s, pq1_s), (vt0_s, vt1_s)
    va_s, p_s = (va0_s, va1_s), (p0_s, p1_s)

    def y_of(c):
        return yl_s if c == NC - 1 else y_s.at[c]

    def w_copy(i, t):
        cols = pl.ds(t * T, T)
        return pltpu.make_async_copy((wq_hbm, wk_hbm, wv_hbm)[i].at[:, cols], w_v.at[i, t],
                                     sem_w.at[i * NC + t])

    def wo_copy():
        return pltpu.make_async_copy(wo_hbm, wo_v, sem_w.at[3 * NC])

    def x_copy(first, count):
        rows = pl.ds(first * L, count * L)
        return pltpu.make_async_copy(x_hbm.at[rows], x_v.at[rows], sem_x.at[first])

    def conv_copies(j):
        src = pl.ds(pl.multiple_of(jnp.minimum(j, NQ - 1) * L, L), L)
        dst = pl.ds(pl.multiple_of(j * L, L), L)
        return (pltpu.make_async_copy(k_hbm.at[src], k_v.at[dst], sem_a.at[3 * j]),
                pltpu.make_async_copy(v_hbm.at[src], v_v.at[dst], sem_a.at[3 * j + 1]),
                pltpu.make_async_copy(h_hbm.at[:, src], h_v.at[j], sem_a.at[3 * j + 2]))

    def q_copy():
        return pltpu.make_async_copy(q_hbm, q_v, sem_q)

    def const_copy(i):
        src, dst = ((beta_hbm, beta_ref), (shift_hbm, shift_ref), (d_hbm, d_ref),
                    (dft_hbm, dft_s.at[4:6]))[i]
        return pltpu.make_async_copy(src, dst, sem_c.at[i])

    def oa_copy(rows, lanes):
        return pltpu.make_async_copy(outa_s.at[rows, lanes], out_hbm.at[rows, lanes], sem_oa)

    def ob_copy(rows):
        return pltpu.make_async_copy(outb_s.at[rows], out_hbm.at[rows, pl.ds(D, D)], sem_ob)

    kv_ready = []

    def gate_kv(u, half):
        src = pl.multiple_of(u * CB, CB)
        for c in range(NC):
            lanes = slice(c * T, (c + 1) * T)
            taps = [shift_ref[t:t + 1, lanes].astype(F32) for t in range(4)]
            pe, po = kf_s[c, 0], kf_s[c, 1]
            for r in range(0, T, 16):
                rows = pl.ds(pl.multiple_of(src + 2 * r, 32), 32)
                ke, ko = _halves(k_v[rows, lanes])
                ve, vo = _halves(v_v[rows, lanes])
                e1 = pltpu.roll(jnp.concatenate([pe, ke], axis=0), 1, 0)[8:24]
                odd = jnp.concatenate([po, ko], axis=0)
                o1, o2 = pltpu.roll(odd, 1, 0)[8:24], pltpu.roll(odd, 2, 0)[8:24]
                se = ke * taps[0] + o1 * taps[1] + e1 * taps[2] + o2 * taps[3]
                so = ko * taps[0] + ke * taps[1] + o1 * taps[2] + e1 * taps[3]
                kv_s[half, c, r:r + 16, :] = (se * ve).astype(BF)
                kv_s[half, c, T + r:T + r + 16, :] = (so * vo).astype(BF)
                pe, po = ke[8:16], ko[8:16]
                yield 1
            kf_s[c, 0] = pe
            kf_s[c, 1] = po
            kv_ready.append((half, c))

    def conv_forward(u, half, c):
        lanes = slice(c * T, (c + 1) * T)
        h0, h1 = (pltpu.bitcast(h_v[u // 2, lanes, (2 * half + j) * T:(2 * half + j + 1) * T], jnp.uint32)
                  for j in range(2))
        even = (_iota(h0.shape, 1) & 1) == 0
        he = pltpu.bitcast(jnp.where(even, h0, pltpu.roll(h1, 1, 1)), BF)
        ho = pltpu.bitcast(jnp.where(even, pltpu.roll(h1, T - 1, 1), h0), BF)
        for base, a, b in (
                (c, _dot(_unpack(dft_s[0]), kv_s[half, c, 0:T, :]),
                 _dot(_unpack(dft_s[1]), kv_s[half, c, T:CB, :])),
                (NC + c, _dot_nt(_unpack(dft_s[2]), he), _dot_nt(_unpack(dft_s[3]), ho))):
            xg_s[base, u, 0:CB, :] = a + b
            xg_s[base, u, CB:2 * CB, :] = a - b

    def conv_mac(items, w=2):
        skip = {c: jnp.broadcast_to(d_row(c), (8, T)) for c, _ in items}
        for c, f in items:
            for k in range(NB // w):
                outs = range(k * w, (k + 1) * w)
                r0 = pl.multiple_of((f + zero_s[k]) * 16, 16)
                plus = {}
                for sign in range(2):
                    re = pl.ds(pl.multiple_of(r0 + sign * CB, 8), 8)
                    im = pl.ds(pl.multiple_of(r0 + sign * CB + 8, 8), 8)
                    acc, g, h = {}, {}, {}

                    def filt(n):
                        if n not in g:
                            for m in (n, n - 1):
                                if m >= 0 and m not in h:
                                    h[m] = (xg_s[NC + c, m, re, :], xg_s[NC + c, m, im, :])
                            if n == 0:
                                g[n] = (h[0][0] + skip[c], h[0][1])
                            else:
                                g[n] = (h[n][0] - h[n - 1][1], h[n][1] + h[n - 1][0])
                        return g[n]

                    for b in range(max(outs) + 1):
                        xr, xi = xg_s[c, b, re, :], xg_s[c, b, im, :]
                        cost = 0
                        for a in outs:
                            if b > a:
                                continue
                            gr, gi = filt(a - b)
                            p = (xr * gr - xi * gi, xr * gi + xi * gr)
                            acc[a] = p if a not in acc else (acc[a][0] + p[0], acc[a][1] + p[1])
                            cost += 1
                            if a == b and sign == 0:
                                plus[a] = jnp.concatenate(acc[a], axis=0)
                            elif a == b:
                                minus = jnp.concatenate(acc[a], axis=0)
                                y_of(c)[a, pl.ds(r0, 16), :] = (plus[a] + minus).astype(BF)
                                y_of(c)[a, pl.ds(pl.multiple_of(r0 + CB, 16), 16), :] = (
                                    plus[a] - minus).astype(BF)
                        yield cost

    class Filler:
        def __init__(self):
            self.gen, self.credit, self.in_k = None, 0.0, False

        def pin(self, value, amount):
            if self.gen is None or amount == 0:
                return
            if self.in_k:
                k_v[S + L:S + L + 16, 0:T] = jnp.concatenate([value, value], axis=0).astype(BF)
            else:
                xg_s[2 * NC, 0, 0:8, :] = value
            self.credit += amount
            while self.gen is not None and self.credit > 0:
                cost = next(self.gen, None)
                if cost is None:
                    self.gen = None
                else:
                    self.credit -= cost

        def drain(self):
            if self.gen is not None:
                for _ in self.gen:
                    pass
            self.gen = None

    filler = Filler()

    def conv_inverse(u, c):
        r0 = pl.multiple_of(u * CB, CB)
        lanes = slice(c * T, (c + 1) * T)
        qs = _halves(q_v[pl.ds(r0, CB), lanes])
        out = []
        for j in range(2):
            inv = jnp.concatenate([_unpack(dft_s[4 + j, 0:T // 2, :]),
                                   _unpack(dft_s[4 + j, T // 2:T, :])], axis=1)
            y = _dot(inv, y_of(c)[u, j * CB:(j + 1) * CB, :])
            out.append(qs[j] * y)
        outa_s[pl.ds(r0, CB), lanes] = _interleave(*out)

    def out_proj(o, rows, amount):
        m = o[0].shape[0]
        last = NC - 1
        head = jnp.concatenate(o[0:last], axis=1)

        def pin(part):
            for r in range(0, m, 32):
                filler.pin(part[r:r + 8, 0:T], amount * 32 / (6 * m))

        edge = _dot(o[last], wo_v[last * T:D, 0:last * T])
        pin(edge)
        yield
        corner = _dot(o[last], wo_v[last * T:D, last * T:D])
        for n in reversed(range(NC)):
            part = _dot(head, wo_v[0:last * T, n * T:(n + 1) * T])
            pin(part)
            part = part + (corner if n == last else edge[:, n * T:(n + 1) * T])
            outb_s[rows, n * T:(n + 1) * T] = part.astype(BF)
            yield

    def own_rows(x, i, fill):
        low4 = _iota((8, T), 0) < 4
        full = jnp.full((8, T), fill, F32)
        g0 = 5 * (i // 2)
        if i % 2 == 0:
            body = [x[8 * g0:8 * g0 + 16], jnp.where(low4, x[8 * g0 + 16:8 * g0 + 24], fill)]
        else:
            body = [jnp.where(low4, fill, x[8 * g0 + 16:8 * g0 + 24]), x[8 * g0 + 24:8 * g0 + 40]]
        return jnp.concatenate(body + [full] if i < 2 else [full] + body, axis=0).astype(BF)

    def project(n, par, amount, need_q=True, need_k=True):
        s, u = n // NU, n % NU
        w0 = pl.multiple_of((u // 2) * (WPAIR // 2), 32) + par * (UD // 2)
        x0 = pl.multiple_of(s * L, L)
        slot = (n // 2) % 2
        pad = jnp.zeros((T - UD, T), F32)

        def finish(j, qkv):
            cols = slice(j * T, (j + 1) * T)
            qt, kt, vt = qkv[0:UD], qkv[UD:2 * UD], qkv[2 * UD:3 * UD]
            kn_s[cols, :] = jnp.concatenate([kt, pad], axis=0).T.astype(BF)
            qs = qt * (DH ** -0.5 * LOG2E)
            low4 = _iota((8, T), 0) < 4
            left = _iota((8, T), 1) < T // 2
            zero = jnp.zeros((8, T), F32)
            for pr in range(UH // 2):
                qa = [qs[40 * pr + 8 * r:40 * pr + 8 * r + 8] for r in range(3)]
                qb = [pltpu.roll(qs[40 * pr + 8 * r:40 * pr + 8 * r + 8], T // 2, 1) for r in (2, 3, 4)]
                ra = [qa[0], qa[1], jnp.where(low4, qa[2], 0.0)]
                rb = [jnp.where(low4, 0.0, qb[0]), qb[1], qb[2]]
                rh = [jnp.where(left, 0.0, qa[0]), jnp.where(left, 0.0, qa[1]),
                      jnp.where(left, rb[0], ra[2]),
                      jnp.where(left, qb[1], 0.0), jnp.where(left, qb[2], 0.0)]
                for i, rows in ((2 * pr, ra), (2 * pr + 1, rb)):
                    rows = rows + [zero] if pr == 0 else [zero] + rows
                    rq_s[j, i, 8 * i:8 * i + 16, :] = _pack(jnp.concatenate(rows, axis=0).astype(BF))
                rows = rh + [zero] if pr == 0 else [zero] + rh
                rq_s[j, UH + pr, 16 * pr:16 * pr + 24, :] = _pack(
                    jnp.concatenate(rows, axis=0).astype(BF))
            for i in range(UH):
                va_s[par][slot, i, j] = own_rows(vt, i, 1.0)
            if need_q:
                pq_s[par][slot, j] = _phi(qt).astype(BF)
            if need_k:
                pk_s[par][slot, j] = _phi(kt).astype(BF)
                vt_s[par][slot, j] = vt.astype(BF)

        w = [_unpack(jnp.concatenate(
            [wt_s[c, i, pl.ds(pl.multiple_of(w0, 8), UD // 2), :] for i in range(3)], axis=0))
             for c in range(NC)]
        part = _dot_nt(w[NC - 1], x_v[pl.ds(x0, L), (NC - 1) * T:D])
        for j in range(NQ):
            e_s[j] = part[:, j * T:(j + 1) * T]
        for r in range(0, 3 * UD, 24):
            filler.pin(part[r:r + 8, 0:T], amount / (10 * NC))
        yield
        w = jnp.concatenate(w[0:NC - 1], axis=1)
        for j in reversed(range(NQ)):
            rows = pl.ds(pl.multiple_of(x0 + j * T, T), T)
            part = _dot_nt(w, x_v[rows, 0:(NC - 1) * T])
            for r in range(0, 3 * UD, 24):
                filler.pin(part[r:r + 8], amount / (10 * NC))
            finish(j, part + e_s[j])
            yield

    def s_off(j, i, t, n=T):
        return pl.ds((2 * j * (j + 1) + i * (j + 1) + t) * T, n)

    def hi_off(j, pr):
        return pl.ds((2 * j * (j + 1) + 2 * pr * (j + 1) + j) * T + HALF, HALF)

    def sparse(j, i, first, count):
        parts = [_unpack(rq_s[j, i, first // 2:(first + count) // 2, :]),
                 jnp.zeros((T - first - count, T), BF)]
        if first:
            parts.insert(0, jnp.zeros((first, T), BF))
        return jnp.concatenate(parts, axis=0)

    def col_max(x):
        return jnp.max(x.reshape(x.shape[0] // 8, 8, T), axis=0)

    def scores(j, t, top, amount):
        rq = jnp.concatenate([sparse(j, i, 16 * i, 32) for i in range(UH)], axis=1)
        n = T if t < j else HALF
        sc = _dot(kn_s[t * T:t * T + n, :], rq)
        if t == j:
            rh = jnp.concatenate([sparse(j, UH + pr, 32 * pr, 48) for pr in range(2)], axis=1)
            hi = _dot(kn_s[t * T + HALF:(t + 1) * T, :], rh)
        for i in range(UH):
            si = sc[:, i * T:(i + 1) * T]
            if t == j:
                si = si + bias_s[i % 2]
            s_s[s_off(j, i, t, n), :] = si
            if i == 0:
                for r in range(0, n, 32):
                    filler.pin(si[r:r + 8], amount * 32 / n)
            top[i] = col_max(si) if t == 0 else jnp.maximum(top[i], col_max(si))
        if t < j:
            return
        left = _iota((8, T), 1) < HALF
        for pr in range(2):
            si = hi[:, pr * T:(pr + 1) * T] + bias_s[2]
            s_s[hi_off(j, pr), :] = si
            mh = col_max(si)
            ma = jnp.maximum(top[2 * pr], jnp.where(left, -jnp.inf, mh))
            mb = jnp.maximum(top[2 * pr + 1], jnp.where(left, mh, -jnp.inf))
            ma = jnp.broadcast_to(jnp.max(ma, axis=0, keepdims=True), (8, T))
            mb = jnp.broadcast_to(jnp.max(mb, axis=0, keepdims=True), (8, T))
            m_s[j, 2 * pr] = ma
            m_s[j, 2 * pr + 1] = mb
            m_s[j, UH + pr] = jnp.where(left, mb, ma)

    def weights(rows, j, i):
        sc = s_s[rows, :]
        m = jnp.concatenate([m_s[j, i]] * (sc.shape[0] // 8), axis=0)
        return jnp.exp2(sc - m).astype(BF)

    def softmax(par, j, t):
        n = T if t < j else HALF
        for i in range(UH):
            p_s[par][s_off(j, i, t, n), :] = weights(s_off(j, i, t, n), j, i)
        if t < j:
            return
        left = _iota((HALF // 2, T), 1) < HALF
        none = jnp.zeros((HALF // 2, T), jnp.uint32)
        for pr in range(2):
            p = pltpu.bitcast(weights(hi_off(j, pr), j, UH + pr), jnp.uint32)
            for i, part in ((2 * pr, jnp.where(left, none, p)), (2 * pr + 1, jnp.where(left, p, none))):
                p_s[par][pl.ds(s_off(j, i, t).start + HALF, HALF), :] = pltpu.bitcast(part, BF)

    def spread(a, b):
        low4 = _iota(a.shape, 0) < 4
        ar, br = pltpu.roll(a, 4, 0), pltpu.roll(b, 4, 0)
        r0, r1 = jnp.where(low4, a, ar), jnp.where(low4, ar, a)
        r2, r3 = jnp.where(low4, b, br), jnp.where(low4, br, b)
        return jnp.concatenate([r0, r0, a, r1, r1, r2, r2, b, r3, r3], axis=0)

    def retrieve(n, par):
        u, slot = n % NU, (n // 2) % 2
        zpad = jnp.zeros((T - UD, T), BF)
        pq = jnp.concatenate(
            [jnp.concatenate([pq_s[par][slot, j], zpad], axis=0) for j in range(NQ)], axis=1)
        ret = _dot(meml_s[u], pq)
        rd = 1.0 / (ret[UD:UD + 16] + 1e-6)
        ret_s[...] = ret[0:UD] * spread(rd[0:8], rd[8:16])

    def update(n, par, s):
        u, slot = n % NU, (n // 2) % 2
        zpad = jnp.zeros((T - UD, T), BF)
        va = jnp.concatenate(
            [jnp.concatenate([vt_s[par][slot, j], jnp.ones((16, T), BF)], axis=0) for j in range(NQ)],
            axis=1)
        pk = jnp.concatenate(
            [jnp.concatenate([pk_s[par][slot, j], zpad], axis=0) for j in range(NQ)], axis=1)
        mem = _dot_nt(va, pk)
        if s > 0:
            mem = mem_s[u] + mem
        if s < NSEG - 2:
            mem_s[u] = mem
        row = _iota((UD + 16, T), 0)
        row_head = jnp.where(row < UD, _head_of(row), (row - UD) >> 2)
        meml_s[u] = jnp.where(row_head == _head_of(_iota((UD + 16, T), 1)), mem, 0.0).astype(BF)

    def values(n, par, s, j, t, acc):
        u, slot = n % NU, (n // 2) % 2
        for i in range(UH):
            part = _dot(va_s[par][slot, i, t], p_s[par][s_off(j, i, t), :])
            acc[i] = part if t == 0 else acc[i] + part
        if t < j:
            return
        heads = []
        for i in range(UH):
            den = acc[i][24:32] if i < 2 else acc[i][0:8]
            val = acc[i][0:24] if i < 2 else acc[i][8:32]
            val = val * jnp.concatenate([1.0 / den] * 3, axis=0)
            heads.append(pltpu.roll(val, HALF, 1) if i % 2 else val)
        low4 = _iota((8, T), 0) < 4
        att = jnp.concatenate([
            heads[0][0:16], jnp.where(low4, heads[0][16:24], heads[1][0:8]), heads[1][8:24],
            heads[2][0:16], jnp.where(low4, heads[2][16:24], heads[3][0:8]), heads[3][8:24]], axis=0)
        rows = pl.ds(pl.multiple_of(u * UD, 16), UD)
        gt = gate_s[rows, :]
        o = (1.0 - gt) * att
        if s > 0:
            o = o + gt * ret_s[:, j * T:(j + 1) * T]
        o = o.astype(BF)
        ot_s[s % 2][j, rows, :] = o

    deliver = []

    def step(n, par, s, order, share, jobs=(), oproj=None, stages='PQSV', need_q=True, arrive=None):
        jobs = list(jobs)
        proj = project(n + 3, 1 - par, share[1], need_q=need_q, need_k=s < NSEG - 1)
        top, acc, final = [None] * UH, {}, {}
        for tok in order:
            if tok[0] == 'Q':
                j, t = int(tok[1]), int(tok[2])
                if 'S' in stages:
                    softmax(1 - par, j, t)
                if 'Q' in stages:
                    scores(j, t, top, share[0] / 10)
            elif tok[0] == 'V':
                if 'V' in stages:
                    values(n, par, s, int(tok[1]), int(tok[2]), acc.setdefault(tok[1], [None] * UH))
            elif tok == 'P':
                if 'P' in stages:
                    next(proj)
            elif tok == 'R':
                if 'V' in stages and s > 0:
                    retrieve(n, par)
            elif tok == 'U':
                if 'V' in stages and s < NSEG - 1:
                    update(n, par, s)
            elif tok[0] == 'T':
                j = int(tok[1])
                rows = pl.ds((NSEG - 1) * L + j * T, T)
                if j not in final:
                    final[j] = [out_proj(out_tiles(NSEG - 1, j), rows, 0), 0]
                next(final[j][0])
                final[j][1] += 1
                if final[j][1] == NC + 1:
                    ob_copy(rows).start()
            elif tok == 'D':
                deliver.pop(0)()
            elif tok == 'O':
                if oproj is not None:
                    next(oproj)
            elif tok == 'W':
                if arrive is not None:
                    arrive()
            elif tok == 'X':
                if jobs:
                    jobs.pop(0)()
        assert not jobs

    def out_tiles(s, j):
        return [ot_s[s % 2][j, c * T:(c + 1) * T, :].T for c in range(NC)]

    def pair_step(s, j, stages=('PQSV', 'PQSV'), mac=None, inverse=None, plan=None):
        orders, mix = _PLANS[plan or ("conv_forward", "conv_mix", "conv_mix", "conv_inverse")[s]]
        us = (2 * j, 2 * j + 1)
        oproj = None
        filler.gen, filler.credit, filler.in_k = None, 0.0, s == 0
        if s == 0:
            del kv_ready[:]
            filler.gen = (cost for half, u in enumerate(us) for cost in gate_kv(u, half))
            share = [16 * NC * v for v in mix]
        else:
            if mac is None:
                mac = [(c, 4 * j + r) for c in (2 * s - 2, 2 * s - 1) for r in range(4)]
            weight = (mix[0] * sum('Q' in st for st in stages)
                      + mix[1] * sum('P' in st for st in stages) + 2 * mix[2])
            share = [72 * len(mac) * v / weight for v in mix]
            if mac:
                filler.gen = conv_mac(mac)
            rows = pl.ds(pl.multiple_of((s - 1) * L + j * T, T), T)
            oproj = out_proj(out_tiles(s - 1, j), rows, 2 * share[2])
        for half, u in enumerate(us):
            jobs = []
            if s == 0:
                def forward(u, half, c):
                    while (half, c) not in kv_ready and filler.gen is not None:
                        if next(filler.gen, None) is None:
                            filler.gen = None
                        filler.credit -= 1
                    conv_forward(u, half, c)
                jobs = [lambda c=c, u=u, half=half: forward(u, half, c) for c in range(NC)]
            elif s == NSEG - 1:
                todo = (inverse[half] if inverse else []) + [(u, c) for c in range(NC - 1)]
                jobs = [lambda b=b, c=c: conv_inverse(b, c) for b, c in todo]
            step(s * NU + u, half, s, orders[half], share, jobs, oproj, stages[half])
        filler.drain()

    def last_mac(j, extra=None):
        return [(NC - 1, f) for f in [4 * j + r for r in range(4)] + (extra or [12 + 2 * j])]

    def transpose_weights(t):
        for i in range(3):
            for c in range(NC):
                wt = _pack(w_v[i, t, c * T:(c + 1) * T, :].T)
                for r in range(T // 16):
                    pair, off = divmod(t * T + 16 * r, 2 * UD)
                    row = (pair * WPAIR + off) // 2
                    wt_s[c, i, row:row + 8, :] = wt[8 * r:8 * r + 8]

    def d_row(c):
        return d_ref[...].astype(F32).reshape(1, D)[:, c * T:(c + 1) * T]

    def send_pair(j):
        oa_copy(pl.ds(pl.multiple_of(j * L, L), L), pl.ds(0, (NC - 1) * T)).start()
        ob_copy(pl.ds(pl.multiple_of(2 * L + j * T, T), T)).start()

    def epilogue():
        first = pl.ds(0, (NC - 1) * T)
        pair_step(3, NQ - 2, stages=('PQSV', 'QSV'), mac=last_mac(NQ - 2, [13, 15]), plan="third_last")
        send_pair(NQ - 2)

        deliver.extend([
            lambda: (oa_copy(pl.ds(0, S), pl.ds((NC - 1) * T, T)).start(),
                     oa_copy(pl.ds(S - 2 * CB, CB), first).start()),
            lambda: oa_copy(pl.ds(S - CB, CB), first).start(),
            lambda: ob_copy(pl.ds(3 * L - T, T)).start()])
        pair_step(3, NQ - 1, stages=('SV', 'V'), mac=[], plan="last",
                  inverse=[[(b, NC - 1) for b in range(NB)], []])

    for i in range(3):
        w_copy(i, 0).start()
    const_copy(0).start()
    x_copy(0, 1).start()
    key, lane = _iota((T // 2, T), 0), _iota((T // 2, T), 1)
    for b, query in enumerate((lane, lane ^ (T // 2), lane & (T // 2 - 1))):
        bias_s[b] = jnp.where(key > query, -1e9 * LOG2E, 0.0).astype(F32)
    kf_s[...] = jnp.zeros(kf_s.shape, F32)
    for k in range(NB):
        zero_s[k] = 0
    for which in range(4):
        for f, rows in enumerate(_forward_dft(which)):
            dft_s[which, 8 * f:8 * f + 8, :] = _pack(rows)
    const_copy(0).wait()
    g = jax.nn.sigmoid(beta_ref[...].astype(F32).reshape(1, H))
    rr = _iota((D, H), 0)
    hh = _iota((D, H), 1) * DH
    gate = jnp.sum(jnp.where((rr >= hh) & (rr < hh + DH), g, 0.0), axis=1, keepdims=True)
    gate_s[...] = jnp.broadcast_to(gate, (D, T))
    for i in range(3):
        w_copy(i, 0).wait()
    for i in range(3):
        w_copy(i, 1).start()
    transpose_weights(0)
    x_copy(0, 1).wait()
    for i in range(3):
        w_copy(i, 2).start()
    for _ in project(0, 0, 0, need_q=False):
        pass
    for i in range(3):
        w_copy(i, 1).wait()
    for i in range(3):
        w_copy(i, 3).start()
    const_copy(1).start()
    transpose_weights(1)

    def fetch_conv():
        for cp in conv_copies(0):
            cp.start()
    step(-2, 0, 0, _WARM_UP[0], (0, 0), stages='PQ', need_q=False, arrive=fetch_conv)
    for t in (2, 3):
        for i in range(3):
            w_copy(i, t).wait()
    for t in (2, 3):
        transpose_weights(t)
    step(-1, 1, 0, _WARM_UP[1], (0, 0), stages='PQS', need_q=False)
    const_copy(1).wait()
    for cp in conv_copies(0):
        cp.wait()
    for i in range(3):
        w_copy(i, 4).start()
    x_copy(1, 1).start()

    def seg0(j, _):
        @pl.when(j == 1)
        def _():
            for i in range(3):
                w_copy(i, 4).wait()
            x_copy(1, 1).wait()
            wo_copy().start()
            x_copy(2, 2).start()
            const_copy(2).start()
            transpose_weights(4)

        for cp in conv_copies(j + 1):
            cp.start()
        pair_step(0, j)
        for cp in conv_copies(j + 1):
            cp.wait()
    lax.fori_loop(0, NQ, seg0, None)

    const_copy(2).wait()
    const_copy(3).start()
    wo_copy().wait()
    x_copy(2, 2).wait()

    lax.fori_loop(0, NQ, lambda j, _: pair_step(1, j), None)
    ob_copy(pl.ds(0, L)).start()
    q_copy().start()
    lax.fori_loop(0, NQ, lambda j, _: pair_step(2, j), None)
    ob_copy(pl.ds(L, L)).start()
    q_copy().wait()
    const_copy(3).wait()

    def seg3(j, _):
        pair_step(3, j, mac=last_mac(j))
        send_pair(j)
    lax.fori_loop(0, NQ - 2, seg3, None)
    epilogue()

    oa_copy(pl.ds(0, S), pl.ds(0, D)).wait()
    ob_copy(pl.ds(0, S)).wait()


@jax.jit
def pallas_concat_heads__ssm_conv_h3__memory_aug_infini_attn__prompt_kernel(
    A_q, A_k, A_v, A_shift_k, A_ssm_k, A_ssm_D, B_x, B_wq, B_wk, B_wv, B_wo, B_beta,
):
    hbm = pl.BlockSpec(memory_space=pl.ANY)
    dma = pltpu.SemaphoreType.DMA
    out = pl.pallas_call(
        _kernel,
        out_shape=jax.ShapeDtypeStruct((S, 2 * D), BF),
        in_specs=[hbm] * 13,
        out_specs=hbm,
        scratch_shapes=[
            pltpu.VMEM((S, D), BF),
            pltpu.VMEM((S + L + 64, D), BF),
            pltpu.VMEM((S + L, D), BF),
            pltpu.VMEM((NQ + 1, D, L), BF),
            pltpu.VMEM((S, D), BF),
            pltpu.VMEM((3, NC, D, T), BF),
            pltpu.VMEM((D, D), BF),
            pltpu.VMEM((NC, 3, NQ * WPAIR // 2, T), jnp.uint32),
            pltpu.VMEM((6, T, T), jnp.uint32),
            pltpu.VMEM((NC + 1, 2, 8, T), F32),
            pltpu.VMEM((2, NC, CB, T), BF),
            pltpu.VMEM((2 * NC + 1, NB, 2 * CB, T), F32),
            pltpu.VMEM((NC - 1, NB, 2 * CB, T), BF),
            pltpu.VMEM((NB, 2 * CB, T), BF),
            pltpu.VMEM((S, D), BF),
            pltpu.VMEM((S, D), BF),
            pltpu.VMEM((NQ, D, T), BF),
            pltpu.VMEM((NQ, D, T), BF),
            pltpu.VMEM((NU, UD + 16, T), F32),
            pltpu.VMEM((NU, UD + 16, T), BF),
            pltpu.VMEM((D, T), F32),
            pltpu.VMEM((3, T // 2, T), F32),
            pltpu.VMEM((L, T), BF),
            pltpu.VMEM((NQ, UH + 2, T // 2, T), jnp.uint32),
            *[pltpu.VMEM((2, NQ, UD, T), BF)] * 6,
            *[pltpu.VMEM((2, UH, NQ, 32, T), BF)] * 2,
            pltpu.VMEM((40 * T, T), F32),
            *[pltpu.VMEM((40 * T, T), BF)] * 2,
            pltpu.VMEM((NQ, UH + 2, 8, T), F32),
            pltpu.VMEM((UD, L), F32),
            pltpu.VMEM((NQ, 3 * UD, T), F32),
            pltpu.VMEM((4, D), BF),
            pltpu.VMEM((D,), BF),
            pltpu.VMEM((H,), BF),
            pltpu.SMEM((NB,), jnp.int32),
            dma((3 * NC + 1,)), dma((3,)), dma((3 * (NQ + 1),)), dma(()),
            dma((4,)), dma(()), dma(()),
        ],
        compiler_params=pltpu.CompilerParams(
            vmem_limit_bytes=100 * 1024 * 1024),
        name="h3_infini",
    )(A_q.reshape(S, D), A_k.reshape(S, D), A_v.reshape(S, D), A_shift_k.T, A_ssm_k, A_ssm_D,
      B_x.reshape(S, D), B_wq, B_wk, B_wv, B_wo, B_beta, _INVERSE_DFT)
    return out.reshape(1, S, 2 * D)
```

```python
import math

import numpy as np
import jax
import jax.numpy as jnp
from jax import lax
from jax.experimental import pallas as pl
from jax.experimental.pallas import tpu as pltpu

S, D = 2048, 640
H, DH, NSEG, L = 32, 20, 4, 512
T = 128
HALF = T // 2
NC = D // T
CB = 2 * T
NB = S // CB
NF = T // 8
NQ = L // T
UH = 4
UD = UH * DH
NU = H // UH
WPAIR = 192
BF, F32 = jnp.bfloat16, jnp.float32
LOG2E = math.log2(math.e)


def _dft_matrices():
    m = np.arange(T)[:, None]
    r = np.arange(T)[None, :]

    def rows(power):
        ang = np.pi * np.mod((4 * m + 1) * power, 1024) / 512
        f = np.stack([np.cos(ang).reshape(NF, 8, T), -np.sin(ang).reshape(NF, 8, T)], 1)
        return f.reshape(2 * T, T)

    even, odd = rows(2 * r), rows(2 * r + 1)
    lane = np.arange(T)
    even_h = even[:, lane // 2 + (T // 2) * (lane % 2)]
    odd_h = odd[:, lane // 2 + (T // 2) * (1 - lane % 2)]
    inverse = [np.concatenate([f[:T].T, f[T:].T]) / (2 * T) for f in (even, odd)]
    bits = np.stack([even, odd, even_h, odd_h] + inverse).astype(np.float32).astype(BF)
    bits = bits.view(np.uint16).astype(np.uint32)
    return (bits[:, 0::2] | (bits[:, 1::2] << 16))[4:]


_INVERSE_DFT = _dft_matrices()


def _forward_dft(which):
    row, lane = _iota((8, T), 0), _iota((8, T), 1)
    odd = which % 2
    sample = lane if which < 2 else (lane >> 1) + (T // 2) * ((lane & 1) ^ odd)
    power = 2 * sample + odd

    def unit(turn):
        angle = lambda t: (t & 1023).astype(F32) * (math.pi / 512)
        return jnp.cos(angle(turn)), jnp.cos(angle(turn + 256))

    (re, im), (step_re, step_im) = unit((4 * row + 1) * power), unit(32 * power)
    for _ in range(NF):
        yield jnp.concatenate([re, im], axis=0).astype(BF)
        re, im = re * step_re - im * step_im, re * step_im + im * step_re


def _pack(x):
    return pltpu.bitcast(x, jnp.uint32)


def _unpack(w):
    return pltpu.bitcast(w, BF)


def _halves(x):
    w = pltpu.bitcast(x, jnp.uint32)
    return (lax.bitcast_convert_type(w << 16, F32),
            lax.bitcast_convert_type(w & np.uint32(0xFFFF0000), F32))


def _interleave(even, odd):
    e, o = (lax.bitcast_convert_type(v.astype(BF).astype(F32), jnp.uint32) for v in (even, odd))
    return pltpu.bitcast((e >> 16) | o, BF)


def _dot(a, b):
    return jnp.dot(a, b, preferred_element_type=F32)


def _dot_nt(a, b):
    return lax.dot_general(a, b, (((1,), (1,)), ((), ())), preferred_element_type=F32)


def _phi(t):
    return jnp.where(t > 0, t + 1.0, jnp.exp(t))


def _iota(shape, dim):
    return lax.broadcasted_iota(jnp.int32, shape, dim)


def _head_of(z):
    return sum((z >= DH * i).astype(jnp.int32) for i in range(1, UH))


_PLANS = {
    "conv_forward": (
    ("Q30 V30 Q31 V31 P Q32 V32 Q33 V33 P X U Q20 Q21 V20 X V21 Q22 V22 P Q10 V10 Q11 X "
     "V11 V00 P X Q00 P X",
     "Q30 P V30 V31 Q31 Q32 Q33 X V32 V33 X U P Q20 X Q21 V20 V21 Q22 V22 P Q10 V10 X Q11 "
     "X V00 P V11 Q00 P"),
     (0.5, 0.8, 0.0)),
    "conv_mix": (
    ("R P Q30 Q31 V30 V31 Q32 V32 Q33 U V33 P Q20 V20 O Q21 V21 Q22 V22 P O Q10 Q11 V10 "
     "V11 V00 Q00 P P O",
     "V30 P R Q30 Q31 V31 Q32 V32 V20 Q33 V33 Q20 U P Q21 Q22 Q10 V10 Q11 V21 V22 Q00 P O "
     "P P V11 V00 O O"),
     (0.1, 0.6, 0.3)),
    "conv_inverse": (
    ("R P Q30 V30 Q31 V31 X V32 V33 Q32 Q33 P X X Q20 V20 Q21 V21 Q22 V22 P Q10 V10 X Q11 "
     "V11 O P Q00 P V00",
     "P R Q30 V30 X Q31 V31 V32 X Q32 Q33 V33 P Q20 V20 V21 Q21 V22 Q22 Q10 V10 X Q11 V11 "
     "X P Q00 P O O P V00 O O O"),
     (0.15, 0.4, 0.45)),
    "third_last": (
    ("V30 R P Q30 V31 Q31 X V32 Q32 Q33 V33 P V20 X Q20 Q21 V21 X Q22 V22 P Q10 V10 X Q11 "
     "V11 O P Q00 P V00",
     "V30 P Q30 X Q31 V31 R V32 Q32 V33 Q33 P X Q20 V20 Q21 O V21 X V22 Q22 Q10 V10 O Q11 "
     "V11 X P P Q00 O P V00 O O"),
     (0.5, 0.5, 0.0)),
    "last": (
    ("R V30 X Q30 X X X Q31 V31 X V32 Q32 V20 Q33 Q20 X X V33 X V21 Q21 X Q22 V10 Q10 V22 "
     "Q11 X V11 X X Q00 V00",
     "R D X V30 V31 X V20 V32 V33 X V21 X V22 O V10 O O O D V11 V00 O O T3 T3 D T3 T3 T3 "
     "T3 T2 T2 T2 T1 T2 T2 T1 T1 T2 T1 T1 T1 T0 T0 T0 T0 T0 T0"),
     (1.0, 1.0, 1.0)),
}
_PLANS = {name: ([half.split() for half in halves], share) for name, (halves, share) in _PLANS.items()}
_WARM_UP = ("Q30 Q31 Q32 Q33 P P Q20 Q21 W Q22 P Q10 Q11 P Q00 P".split(),
            "P Q30 Q31 Q32 Q33 P Q20 Q21 Q22 P Q10 Q11 P Q00 P".split())


def _kernel(q_hbm, k_hbm, v_hbm, shift_hbm, h_hbm, d_hbm, x_hbm, wq_hbm, wk_hbm, wv_hbm,
            wo_hbm, beta_hbm, dft_hbm, out_hbm,
            q_v, k_v, v_v, h_v, x_v, w_v, wo_v, wt_s, dft_s, kf_s, kv_s, xg_s, y_s, yl_s,
            outa_s, outb_s, ot0_s, ot1_s, mem_s, meml_s, gate_s, bias_s,
            kn_s, rq_s, pk0_s, pk1_s, pq0_s, pq1_s, vt0_s, vt1_s, va0_s, va1_s,
            s_s, p0_s, p1_s, m_s, ret_s, e_s, shift_ref, d_ref, beta_ref, zero_s,
            sem_w, sem_x, sem_a, sem_q, sem_c, sem_oa, sem_ob):
    ot_s = (ot0_s, ot1_s)
    pk_s, pq_s, vt_s = (pk0_s, pk1_s), (pq0_s, pq1_s), (vt0_s, vt1_s)
    va_s, p_s = (va0_s, va1_s), (p0_s, p1_s)

    def y_of(c):
        return yl_s if c == NC - 1 else y_s.at[c]

    def w_copy(i, t):
        cols = pl.ds(t * T, T)
        return pltpu.make_async_copy((wq_hbm, wk_hbm, wv_hbm)[i].at[:, cols], w_v.at[i, t],
                                     sem_w.at[i * NC + t])

    def wo_copy():
        return pltpu.make_async_copy(wo_hbm, wo_v, sem_w.at[3 * NC])

    def x_copy(first, count):
        rows = pl.ds(first * L, count * L)
        return pltpu.make_async_copy(x_hbm.at[rows], x_v.at[rows], sem_x.at[first])

    def conv_copies(j):
        src = pl.ds(pl.multiple_of(jnp.minimum(j, NQ - 1) * L, L), L)
        dst = pl.ds(pl.multiple_of(j * L, L), L)
        return (pltpu.make_async_copy(k_hbm.at[src], k_v.at[dst], sem_a.at[3 * j]),
                pltpu.make_async_copy(v_hbm.at[src], v_v.at[dst], sem_a.at[3 * j + 1]),
                pltpu.make_async_copy(h_hbm.at[:, src], h_v.at[j], sem_a.at[3 * j + 2]))

    def q_copy():
        return pltpu.make_async_copy(q_hbm, q_v, sem_q)

    def const_copy(i):
        src, dst = ((beta_hbm, beta_ref), (shift_hbm, shift_ref), (d_hbm, d_ref),
                    (dft_hbm, dft_s.at[4:6]))[i]
        return pltpu.make_async_copy(src, dst, sem_c.at[i])

    def oa_copy(i):
        first = pl.ds(0, (NC - 1) * T)
        if not isinstance(i, int) or i < NQ - 1:
            rows, lanes = pl.ds(pl.multiple_of(i * L, L), L), first
        elif i < NQ + 1:
            rows, lanes = pl.ds(S - L + (i - NQ + 1) * CB, CB), first
        else:
            rows, lanes = pl.ds(0, S), pl.ds((NC - 1) * T, T)
        return pltpu.make_async_copy(outa_s.at[rows, lanes], out_hbm.at[rows, lanes], sem_oa.at[i])

    def ob_copy(i):
        if isinstance(i, int) and i < 2:
            rows = pl.ds(i * L, L)
        else:
            rows = pl.ds(pl.multiple_of(2 * L + (i - 2) * T, T), T)
        return pltpu.make_async_copy(outb_s.at[rows], out_hbm.at[rows, pl.ds(D, D)], sem_ob.at[i])

    kv_ready = []

    def gate_kv(u, half):
        src = pl.multiple_of(u * CB, CB)
        for c in range(NC):
            lanes = slice(c * T, (c + 1) * T)
            taps = [shift_ref[t:t + 1, lanes].astype(F32) for t in range(4)]
            pe, po = kf_s[c, 0], kf_s[c, 1]
            for r in range(0, T, 16):
                rows = pl.ds(pl.multiple_of(src + 2 * r, 32), 32)
                ke, ko = _halves(k_v[rows, lanes])
                ve, vo = _halves(v_v[rows, lanes])
                e1 = pltpu.roll(jnp.concatenate([pe, ke], axis=0), 1, 0)[8:24]
                odd = jnp.concatenate([po, ko], axis=0)
                o1, o2 = pltpu.roll(odd, 1, 0)[8:24], pltpu.roll(odd, 2, 0)[8:24]
                se = ke * taps[0] + o1 * taps[1] + e1 * taps[2] + o2 * taps[3]
                so = ko * taps[0] + ke * taps[1] + o1 * taps[2] + e1 * taps[3]
                kv_s[half, c, r:r + 16, :] = (se * ve).astype(BF)
                kv_s[half, c, T + r:T + r + 16, :] = (so * vo).astype(BF)
                pe, po = ke[8:16], ko[8:16]
                yield 1
            kf_s[c, 0] = pe
            kf_s[c, 1] = po
            kv_ready.append((half, c))

    def conv_forward(u, half, c):
        lanes = slice(c * T, (c + 1) * T)
        h0, h1 = (pltpu.bitcast(h_v[u // 2, lanes, (2 * half + j) * T:(2 * half + j + 1) * T], jnp.uint32)
                  for j in range(2))
        even = (_iota(h0.shape, 1) & 1) == 0
        he = pltpu.bitcast(jnp.where(even, h0, pltpu.roll(h1, 1, 1)), BF)
        ho = pltpu.bitcast(jnp.where(even, pltpu.roll(h1, T - 1, 1), h0), BF)
        for base, a, b in (
                (c, _dot(_unpack(dft_s[0]), kv_s[half, c, 0:T, :]),
                 _dot(_unpack(dft_s[1]), kv_s[half, c, T:CB, :])),
                (NC + c, _dot_nt(_unpack(dft_s[2]), he), _dot_nt(_unpack(dft_s[3]), ho))):
            xg_s[base, u, 0:CB, :] = a + b
            xg_s[base, u, CB:2 * CB, :] = a - b

    def conv_mac(items, w=2):
        skip = {c: jnp.broadcast_to(d_row(c), (8, T)) for c, _ in items}
        for c, f in items:
            for k in range(NB // w):
                outs = range(k * w, (k + 1) * w)
                r0 = pl.multiple_of((f + zero_s[k]) * 16, 16)
                plus = {}
                for sign in range(2):
                    re = pl.ds(pl.multiple_of(r0 + sign * CB, 8), 8)
                    im = pl.ds(pl.multiple_of(r0 + sign * CB + 8, 8), 8)
                    acc, g, h = {}, {}, {}

                    def filt(n):
                        if n not in g:
                            for m in (n, n - 1):
                                if m >= 0 and m not in h:
                                    h[m] = (xg_s[NC + c, m, re, :], xg_s[NC + c, m, im, :])
                            if n == 0:
                                g[n] = (h[0][0] + skip[c], h[0][1])
                            else:
                                g[n] = (h[n][0] - h[n - 1][1], h[n][1] + h[n - 1][0])
                        return g[n]

                    for b in range(max(outs) + 1):
                        xr, xi = xg_s[c, b, re, :], xg_s[c, b, im, :]
                        cost = 0
                        for a in outs:
                            if b > a:
                                continue
                            gr, gi = filt(a - b)
                            p = (xr * gr - xi * gi, xr * gi + xi * gr)
                            acc[a] = p if a not in acc else (acc[a][0] + p[0], acc[a][1] + p[1])
                            cost += 1
                            if a == b and sign == 0:
                                plus[a] = jnp.concatenate(acc[a], axis=0)
                            elif a == b:
                                minus = jnp.concatenate(acc[a], axis=0)
                                y_of(c)[a, pl.ds(r0, 16), :] = (plus[a] + minus).astype(BF)
                                y_of(c)[a, pl.ds(pl.multiple_of(r0 + CB, 16), 16), :] = (
                                    plus[a] - minus).astype(BF)
                        yield cost

    class Filler:
        def __init__(self):
            self.gen, self.credit, self.in_k = None, 0.0, False

        def pin(self, value, amount):
            if self.gen is None or amount == 0:
                return
            if self.in_k:
                k_v[S + L:S + L + 16, 0:T] = jnp.concatenate([value, value], axis=0).astype(BF)
            else:
                xg_s[2 * NC, 0, 0:8, :] = value
            self.credit += amount
            while self.gen is not None and self.credit > 0:
                cost = next(self.gen, None)
                if cost is None:
                    self.gen = None
                else:
                    self.credit -= cost

        def drain(self):
            if self.gen is not None:
                for _ in self.gen:
                    pass
            self.gen = None

    filler = Filler()

    def conv_inverse(u, c):
        r0 = pl.multiple_of(u * CB, CB)
        lanes = slice(c * T, (c + 1) * T)
        qs = _halves(q_v[pl.ds(r0, CB), lanes])
        out = []
        for j in range(2):
            inv = jnp.concatenate([_unpack(dft_s[4 + j, 0:T // 2, :]),
                                   _unpack(dft_s[4 + j, T // 2:T, :])], axis=1)
            y = _dot(inv, y_of(c)[u, j * CB:(j + 1) * CB, :])
            out.append(qs[j] * y)
        outa_s[pl.ds(r0, CB), lanes] = _interleave(*out)

    def out_proj(o, rows, amount):
        m = o[0].shape[0]
        last = NC - 1
        head = jnp.concatenate(o[0:last], axis=1)

        def pin(part):
            for r in range(0, m, 32):
                filler.pin(part[r:r + 8, 0:T], amount * 32 / (6 * m))

        edge = _dot(o[last], wo_v[last * T:D, 0:last * T])
        pin(edge)
        yield
        corner = _dot(o[last], wo_v[last * T:D, last * T:D])
        for n in reversed(range(NC)):
            part = _dot(head, wo_v[0:last * T, n * T:(n + 1) * T])
            pin(part)
            part = part + (corner if n == last else edge[:, n * T:(n + 1) * T])
            outb_s[rows, n * T:(n + 1) * T] = part.astype(BF)
            yield

    def own_rows(x, i, fill):
        low4 = _iota((8, T), 0) < 4
        full = jnp.full((8, T), fill, F32)
        g0 = 5 * (i // 2)
        if i % 2 == 0:
            body = [x[8 * g0:8 * g0 + 16], jnp.where(low4, x[8 * g0 + 16:8 * g0 + 24], fill)]
        else:
            body = [jnp.where(low4, fill, x[8 * g0 + 16:8 * g0 + 24]), x[8 * g0 + 24:8 * g0 + 40]]
        return jnp.concatenate(body + [full] if i < 2 else [full] + body, axis=0).astype(BF)

    def project(n, par, amount, need_q=True, need_k=True):
        s, u = n // NU, n % NU
        w0 = pl.multiple_of((u // 2) * (WPAIR // 2), 32) + par * (UD // 2)
        x0 = pl.multiple_of(s * L, L)
        slot = (n // 2) % 2
        pad = jnp.zeros((T - UD, T), F32)

        def finish(j, qkv):
            cols = slice(j * T, (j + 1) * T)
            qt, kt, vt = qkv[0:UD], qkv[UD:2 * UD], qkv[2 * UD:3 * UD]
            kn_s[cols, :] = jnp.concatenate([kt, pad], axis=0).T.astype(BF)
            qs = qt * (DH ** -0.5 * LOG2E)
            low4 = _iota((8, T), 0) < 4
            left = _iota((8, T), 1) < T // 2
            zero = jnp.zeros((8, T), F32)
            for pr in range(UH // 2):
                qa = [qs[40 * pr + 8 * r:40 * pr + 8 * r + 8] for r in range(3)]
                qb = [pltpu.roll(qs[40 * pr + 8 * r:40 * pr + 8 * r + 8], T // 2, 1) for r in (2, 3, 4)]
                ra = [qa[0], qa[1], jnp.where(low4, qa[2], 0.0)]
                rb = [jnp.where(low4, 0.0, qb[0]), qb[1], qb[2]]
                rh = [jnp.where(left, 0.0, qa[0]), jnp.where(left, 0.0, qa[1]),
                      jnp.where(left, rb[0], ra[2]),
                      jnp.where(left, qb[1], 0.0), jnp.where(left, qb[2], 0.0)]
                for i, rows in ((2 * pr, ra), (2 * pr + 1, rb)):
                    rows = rows + [zero] if pr == 0 else [zero] + rows
                    rq_s[j, i, 8 * i:8 * i + 16, :] = _pack(jnp.concatenate(rows, axis=0).astype(BF))
                rows = rh + [zero] if pr == 0 else [zero] + rh
                rq_s[j, UH + pr, 16 * pr:16 * pr + 24, :] = _pack(
                    jnp.concatenate(rows, axis=0).astype(BF))
            for i in range(UH):
                va_s[par][slot, i, j] = own_rows(vt, i, 1.0)
            if need_q:
                pq_s[par][slot, j] = _phi(qt).astype(BF)
            if need_k:
                pk_s[par][slot, j] = _phi(kt).astype(BF)
                vt_s[par][slot, j] = vt.astype(BF)

        w = [_unpack(jnp.concatenate(
            [wt_s[c, i, pl.ds(pl.multiple_of(w0, 8), UD // 2), :] for i in range(3)], axis=0))
             for c in range(NC)]
        part = _dot_nt(w[NC - 1], x_v[pl.ds(x0, L), (NC - 1) * T:D])
        for j in range(NQ):
            e_s[j] = part[:, j * T:(j + 1) * T]
        for r in range(0, 3 * UD, 24):
            filler.pin(part[r:r + 8, 0:T], amount / (10 * NC))
        yield
        w = jnp.concatenate(w[0:NC - 1], axis=1)
        for j in reversed(range(NQ)):
            rows = pl.ds(pl.multiple_of(x0 + j * T, T), T)
            part = _dot_nt(w, x_v[rows, 0:(NC - 1) * T])
            for r in range(0, 3 * UD, 24):
                filler.pin(part[r:r + 8], amount / (10 * NC))
            finish(j, part + e_s[j])
            yield

    def s_off(j, i, t, n=T):
        return pl.ds((2 * j * (j + 1) + i * (j + 1) + t) * T, n)

    def hi_off(j, pr):
        return pl.ds((2 * j * (j + 1) + 2 * pr * (j + 1) + j) * T + HALF, HALF)

    def sparse(j, i, first, count):
        parts = [_unpack(rq_s[j, i, first // 2:(first + count) // 2, :]),
                 jnp.zeros((T - first - count, T), BF)]
        if first:
            parts.insert(0, jnp.zeros((first, T), BF))
        return jnp.concatenate(parts, axis=0)

    def col_max(x):
        return jnp.max(x.reshape(x.shape[0] // 8, 8, T), axis=0)

    def scores(j, t, top, amount):
        rq = jnp.concatenate([sparse(j, i, 16 * i, 32) for i in range(UH)], axis=1)
        n = T if t < j else HALF
        sc = _dot(kn_s[t * T:t * T + n, :], rq)
        if t == j:
            rh = jnp.concatenate([sparse(j, UH + pr, 32 * pr, 48) for pr in range(2)], axis=1)
            hi = _dot(kn_s[t * T + HALF:(t + 1) * T, :], rh)
        for i in range(UH):
            si = sc[:, i * T:(i + 1) * T]
            if t == j:
                si = si + bias_s[i % 2]
            s_s[s_off(j, i, t, n), :] = si
            if i == 0:
                for r in range(0, n, 32):
                    filler.pin(si[r:r + 8], amount * 32 / n)
            top[i] = col_max(si) if t == 0 else jnp.maximum(top[i], col_max(si))
        if t < j:
            return
        left = _iota((8, T), 1) < HALF
        for pr in range(2):
            si = hi[:, pr * T:(pr + 1) * T] + bias_s[2]
            s_s[hi_off(j, pr), :] = si
            mh = col_max(si)
            ma = jnp.maximum(top[2 * pr], jnp.where(left, -jnp.inf, mh))
            mb = jnp.maximum(top[2 * pr + 1], jnp.where(left, mh, -jnp.inf))
            ma = jnp.broadcast_to(jnp.max(ma, axis=0, keepdims=True), (8, T))
            mb = jnp.broadcast_to(jnp.max(mb, axis=0, keepdims=True), (8, T))
            m_s[j, 2 * pr] = ma
            m_s[j, 2 * pr + 1] = mb
            m_s[j, UH + pr] = jnp.where(left, mb, ma)

    def weights(rows, j, i):
        sc = s_s[rows, :]
        m = jnp.concatenate([m_s[j, i]] * (sc.shape[0] // 8), axis=0)
        return jnp.exp2(sc - m).astype(BF)

    def softmax(par, j, t):
        n = T if t < j else HALF
        for i in range(UH):
            p_s[par][s_off(j, i, t, n), :] = weights(s_off(j, i, t, n), j, i)
        if t < j:
            return
        left = _iota((HALF // 2, T), 1) < HALF
        none = jnp.zeros((HALF // 2, T), jnp.uint32)
        for pr in range(2):
            p = pltpu.bitcast(weights(hi_off(j, pr), j, UH + pr), jnp.uint32)
            for i, part in ((2 * pr, jnp.where(left, none, p)), (2 * pr + 1, jnp.where(left, p, none))):
                p_s[par][pl.ds(s_off(j, i, t).start + HALF, HALF), :] = pltpu.bitcast(part, BF)

    def spread(a, b):
        low4 = _iota(a.shape, 0) < 4
        ar, br = pltpu.roll(a, 4, 0), pltpu.roll(b, 4, 0)
        r0, r1 = jnp.where(low4, a, ar), jnp.where(low4, ar, a)
        r2, r3 = jnp.where(low4, b, br), jnp.where(low4, br, b)
        return jnp.concatenate([r0, r0, a, r1, r1, r2, r2, b, r3, r3], axis=0)

    def retrieve(n, par):
        u, slot = n % NU, (n // 2) % 2
        zpad = jnp.zeros((T - UD, T), BF)
        pq = jnp.concatenate(
            [jnp.concatenate([pq_s[par][slot, j], zpad], axis=0) for j in range(NQ)], axis=1)
        ret = _dot(meml_s[u], pq)
        rd = 1.0 / (ret[UD:UD + 16] + 1e-6)
        ret_s[...] = ret[0:UD] * spread(rd[0:8], rd[8:16])

    def update(n, par, s):
        u, slot = n % NU, (n // 2) % 2
        zpad = jnp.zeros((T - UD, T), BF)
        va = jnp.concatenate(
            [jnp.concatenate([vt_s[par][slot, j], jnp.ones((16, T), BF)], axis=0) for j in range(NQ)],
            axis=1)
        pk = jnp.concatenate(
            [jnp.concatenate([pk_s[par][slot, j], zpad], axis=0) for j in range(NQ)], axis=1)
        mem = _dot_nt(va, pk)
        if s > 0:
            mem = mem_s[u] + mem
        if s < NSEG - 2:
            mem_s[u] = mem
        row = _iota((UD + 16, T), 0)
        row_head = jnp.where(row < UD, _head_of(row), (row - UD) >> 2)
        meml_s[u] = jnp.where(row_head == _head_of(_iota((UD + 16, T), 1)), mem, 0.0).astype(BF)

    def values(n, par, s, j, t, acc):
        u, slot = n % NU, (n // 2) % 2
        for i in range(UH):
            part = _dot(va_s[par][slot, i, t], p_s[par][s_off(j, i, t), :])
            acc[i] = part if t == 0 else acc[i] + part
        if t < j:
            return
        heads = []
        for i in range(UH):
            den = acc[i][24:32] if i < 2 else acc[i][0:8]
            val = acc[i][0:24] if i < 2 else acc[i][8:32]
            val = val * jnp.concatenate([1.0 / den] * 3, axis=0)
            heads.append(pltpu.roll(val, HALF, 1) if i % 2 else val)
        low4 = _iota((8, T), 0) < 4
        att = jnp.concatenate([
            heads[0][0:16], jnp.where(low4, heads[0][16:24], heads[1][0:8]), heads[1][8:24],
            heads[2][0:16], jnp.where(low4, heads[2][16:24], heads[3][0:8]), heads[3][8:24]], axis=0)
        rows = pl.ds(pl.multiple_of(u * UD, 16), UD)
        gt = gate_s[rows, :]
        o = (1.0 - gt) * att
        if s > 0:
            o = o + gt * ret_s[:, j * T:(j + 1) * T]
        o = o.astype(BF)
        ot_s[s % 2][j, rows, :] = o

    deliver = []

    def step(n, par, s, order, share, jobs=(), oproj=None, stages='PQSV', need_q=True, arrive=None):
        jobs = list(jobs)
        proj = project(n + 3, 1 - par, share[1], need_q=need_q, need_k=s < NSEG - 1)
        top, acc, final = [None] * UH, {}, {}
        for tok in order:
            if tok[0] == 'Q':
                j, t = int(tok[1]), int(tok[2])
                if 'S' in stages:
                    softmax(1 - par, j, t)
                if 'Q' in stages:
                    scores(j, t, top, share[0] / 10)
            elif tok[0] == 'V':
                if 'V' in stages:
                    values(n, par, s, int(tok[1]), int(tok[2]), acc.setdefault(tok[1], [None] * UH))
            elif tok == 'P':
                if 'P' in stages:
                    next(proj)
            elif tok == 'R':
                if 'V' in stages and s > 0:
                    retrieve(n, par)
            elif tok == 'U':
                if 'V' in stages and s < NSEG - 1:
                    update(n, par, s)
            elif tok[0] == 'T':
                j = int(tok[1])
                rows = pl.ds((NSEG - 1) * L + j * T, T)
                if j not in final:
                    final[j] = [out_proj(out_tiles(NSEG - 1, j), rows, 0), 0]
                next(final[j][0])
                final[j][1] += 1
                if final[j][1] == NC + 1:
                    ob_copy(2 + NQ + j).start()
            elif tok == 'D':
                deliver.pop(0)()
            elif tok == 'O':
                if oproj is not None:
                    next(oproj)
            elif tok == 'W':
                if arrive is not None:
                    arrive()
            elif tok == 'X':
                if jobs:
                    jobs.pop(0)()
        assert not jobs

    def out_tiles(s, j):
        return [ot_s[s % 2][j, c * T:(c + 1) * T, :].T for c in range(NC)]

    def pair_step(s, j, stages=('PQSV', 'PQSV'), mac=None, inverse=None, plan=None):
        orders, mix = _PLANS[plan or ("conv_forward", "conv_mix", "conv_mix", "conv_inverse")[s]]
        us = (2 * j, 2 * j + 1)
        oproj = None
        filler.gen, filler.credit, filler.in_k = None, 0.0, s == 0
        if s == 0:
            del kv_ready[:]
            filler.gen = (cost for half, u in enumerate(us) for cost in gate_kv(u, half))
            share = [16 * NC * v for v in mix]
        else:
            if mac is None:
                mac = [(c, 4 * j + r) for c in (2 * s - 2, 2 * s - 1) for r in range(4)]
            weight = (mix[0] * sum('Q' in st for st in stages)
                      + mix[1] * sum('P' in st for st in stages) + 2 * mix[2])
            share = [72 * len(mac) * v / weight for v in mix]
            if mac:
                filler.gen = conv_mac(mac)
            rows = pl.ds(pl.multiple_of((s - 1) * L + j * T, T), T)
            oproj = out_proj(out_tiles(s - 1, j), rows, 2 * share[2])
        for half, u in enumerate(us):
            jobs = []
            if s == 0:
                def forward(u, half, c):
                    while (half, c) not in kv_ready and filler.gen is not None:
                        if next(filler.gen, None) is None:
                            filler.gen = None
                        filler.credit -= 1
                    conv_forward(u, half, c)
                jobs = [lambda c=c, u=u, half=half: forward(u, half, c) for c in range(NC)]
            elif s == NSEG - 1:
                todo = (inverse[half] if inverse else []) + [(u, c) for c in range(NC - 1)]
                jobs = [lambda b=b, c=c: conv_inverse(b, c) for b, c in todo]
            step(s * NU + u, half, s, orders[half], share, jobs, oproj, stages[half])
        filler.drain()

    def last_mac(j, extra=None):
        return [(NC - 1, f) for f in [4 * j + r for r in range(4)] + (extra or [12 + 2 * j])]

    def transpose_weights(t):
        for i in range(3):
            for c in range(NC):
                wt = _pack(w_v[i, t, c * T:(c + 1) * T, :].T)
                for r in range(T // 16):
                    pair, off = divmod(t * T + 16 * r, 2 * UD)
                    row = (pair * WPAIR + off) // 2
                    wt_s[c, i, row:row + 8, :] = wt[8 * r:8 * r + 8]

    def d_row(c):
        return d_ref[...].astype(F32).reshape(1, D)[:, c * T:(c + 1) * T]

    def send_pair(j):
        oa_copy(j).start()
        ob_copy(2 + j).start()

    def epilogue():
        pair_step(3, NQ - 2, stages=('PQSV', 'QSV'), mac=last_mac(NQ - 2, [13, 15]), plan="third_last")
        send_pair(NQ - 2)

        deliver.extend([
            lambda: (oa_copy(NQ + 1).start(), oa_copy(NQ - 1).start()),
            lambda: oa_copy(NQ).start(),
            lambda: ob_copy(2 + NQ - 1).start()])
        pair_step(3, NQ - 1, stages=('SV', 'V'), mac=[], plan="last",
                  inverse=[[(b, NC - 1) for b in range(NB)], []])

    for i in range(3):
        w_copy(i, 0).start()
    const_copy(0).start()
    x_copy(0, 1).start()
    key, lane = _iota((T // 2, T), 0), _iota((T // 2, T), 1)
    for b, query in enumerate((lane, lane ^ (T // 2), lane & (T // 2 - 1))):
        bias_s[b] = jnp.where(key > query, -1e9 * LOG2E, 0.0).astype(F32)
    kf_s[...] = jnp.zeros(kf_s.shape, F32)
    for k in range(NB):
        zero_s[k] = 0
    for which in range(4):
        for f, rows in enumerate(_forward_dft(which)):
            dft_s[which, 8 * f:8 * f + 8, :] = _pack(rows)
    const_copy(0).wait()
    g = jax.nn.sigmoid(beta_ref[...].astype(F32).reshape(1, H))
    rr = _iota((D, H), 0)
    hh = _iota((D, H), 1) * DH
    gate = jnp.sum(jnp.where((rr >= hh) & (rr < hh + DH), g, 0.0), axis=1, keepdims=True)
    gate_s[...] = jnp.broadcast_to(gate, (D, T))
    for i in range(3):
        w_copy(i, 0).wait()
    for i in range(3):
        w_copy(i, 1).start()
    transpose_weights(0)
    x_copy(0, 1).wait()
    for i in range(3):
        w_copy(i, 2).start()
    for _ in project(0, 0, 0, need_q=False):
        pass
    for i in range(3):
        w_copy(i, 1).wait()
    for i in range(3):
        w_copy(i, 3).start()
    const_copy(1).start()
    transpose_weights(1)

    def fetch_conv():
        for cp in conv_copies(0):
            cp.start()
    step(-2, 0, 0, _WARM_UP[0], (0, 0), stages='PQ', need_q=False, arrive=fetch_conv)
    for t in (2, 3):
        for i in range(3):
            w_copy(i, t).wait()
    for t in (2, 3):
        transpose_weights(t)
    step(-1, 1, 0, _WARM_UP[1], (0, 0), stages='PQS', need_q=False)
    const_copy(1).wait()
    for cp in conv_copies(0):
        cp.wait()
    for i in range(3):
        w_copy(i, 4).start()
    x_copy(1, 1).start()

    def seg0(j, _):
        @pl.when(j == 1)
        def _():
            for i in range(3):
                w_copy(i, 4).wait()
            x_copy(1, 1).wait()
            wo_copy().start()
            x_copy(2, 2).start()
            const_copy(2).start()
            transpose_weights(4)

        for cp in conv_copies(j + 1):
            cp.start()
        pair_step(0, j)
        for cp in conv_copies(j + 1):
            cp.wait()
    lax.fori_loop(0, NQ, seg0, None)

    const_copy(2).wait()
    const_copy(3).start()
    wo_copy().wait()
    x_copy(2, 2).wait()

    lax.fori_loop(0, NQ, lambda j, _: pair_step(1, j), None)
    ob_copy(0).start()
    q_copy().start()
    lax.fori_loop(0, NQ, lambda j, _: pair_step(2, j), None)
    ob_copy(1).start()
    q_copy().wait()
    const_copy(3).wait()

    def seg3(j, _):
        pair_step(3, j, mac=last_mac(j))
        send_pair(j)
    lax.fori_loop(0, NQ - 2, seg3, None)
    epilogue()

    for i in range(NQ + 2):
        oa_copy(i).wait()
    for i in list(range(2 + NQ)) + [2 + NQ + j for j in reversed(range(NQ))]:
        ob_copy(i).wait()


@jax.jit
def pallas_concat_heads__ssm_conv_h3__memory_aug_infini_attn__prompt_kernel(
    A_q, A_k, A_v, A_shift_k, A_ssm_k, A_ssm_D, B_x, B_wq, B_wk, B_wv, B_wo, B_beta,
):
    hbm = pl.BlockSpec(memory_space=pl.ANY)
    dma = pltpu.SemaphoreType.DMA
    out = pl.pallas_call(
        _kernel,
        out_shape=jax.ShapeDtypeStruct((S, 2 * D), BF),
        in_specs=[hbm] * 13,
        out_specs=hbm,
        scratch_shapes=[
            pltpu.VMEM((S, D), BF),
            pltpu.VMEM((S + L + 64, D), BF),
            pltpu.VMEM((S + L, D), BF),
            pltpu.VMEM((NQ + 1, D, L), BF),
            pltpu.VMEM((S, D), BF),
            pltpu.VMEM((3, NC, D, T), BF),
            pltpu.VMEM((D, D), BF),
            pltpu.VMEM((NC, 3, NQ * WPAIR // 2, T), jnp.uint32),
            pltpu.VMEM((6, T, T), jnp.uint32),
            pltpu.VMEM((NC + 1, 2, 8, T), F32),
            pltpu.VMEM((2, NC, CB, T), BF),
            pltpu.VMEM((2 * NC + 1, NB, 2 * CB, T), F32),
            pltpu.VMEM((NC - 1, NB, 2 * CB, T), BF),
            pltpu.VMEM((NB, 2 * CB, T), BF),
            pltpu.VMEM((S, D), BF),
            pltpu.VMEM((S, D), BF),
            pltpu.VMEM((NQ, D, T), BF),
            pltpu.VMEM((NQ, D, T), BF),
            pltpu.VMEM((NU, UD + 16, T), F32),
            pltpu.VMEM((NU, UD + 16, T), BF),
            pltpu.VMEM((D, T), F32),
            pltpu.VMEM((3, T // 2, T), F32),
            pltpu.VMEM((L, T), BF),
            pltpu.VMEM((NQ, UH + 2, T // 2, T), jnp.uint32),
            *[pltpu.VMEM((2, NQ, UD, T), BF)] * 6,
            *[pltpu.VMEM((2, UH, NQ, 32, T), BF)] * 2,
            pltpu.VMEM((40 * T, T), F32),
            *[pltpu.VMEM((40 * T, T), BF)] * 2,
            pltpu.VMEM((NQ, UH + 2, 8, T), F32),
            pltpu.VMEM((UD, L), F32),
            pltpu.VMEM((NQ, 3 * UD, T), F32),
            pltpu.VMEM((4, D), BF),
            pltpu.VMEM((D,), BF),
            pltpu.VMEM((H,), BF),
            pltpu.SMEM((NB,), jnp.int32),
            dma((3 * NC + 1,)), dma((3,)), dma((3 * (NQ + 1),)), dma(()),
            dma((4,)), dma((NQ + 2,)), dma((2 + 2 * NQ,)),
        ],
        compiler_params=pltpu.CompilerParams(
            vmem_limit_bytes=100 * 1024 * 1024),
        name="h3_infini",
    )(A_q.reshape(S, D), A_k.reshape(S, D), A_v.reshape(S, D), A_shift_k.T, A_ssm_k, A_ssm_D,
      B_x.reshape(S, D), B_wq, B_wk, B_wv, B_wo, B_beta, _INVERSE_DFT)
    return out.reshape(1, S, 2 * D)
```
